```python
import jax
import jax.numpy as jnp

def _softmax(x, axis=-1):
    return jax.nn.softmax(x, axis=axis)

def _gelu(x):
    return jax.nn.gelu(x, approximate=True)

def _silu(x):
    return jax.nn.silu(x)

def _sigmoid(x):
    return jax.nn.sigmoid(x)

def _layernorm(x, axis=-1, eps=1e-05):
    m = jnp.mean(x, axis=axis, keepdims=True)
    v = jnp.var(x, axis=axis, keepdims=True)
    return (x - m) / jnp.sqrt(v + eps)

def _scatter_add(tgt, idx, src, axis=0):
    return tgt.at[idx].add(src)

def _segment_sum(src, seg, n):
    return jax.ops.segment_sum(src, seg, n)

class _Rng:

    def __init__(self, key):
        self._k = key

    def _next(self):
        self._k, sub = jax.random.split(self._k)
        return sub

    def normal(self, shape):
        return jax.random.normal(self._next(), shape, dtype=jnp.bfloat16)

    def randint(self, lo, hi, shape):
        return jax.random.randint(self._next(), shape, lo, hi, dtype=jnp.int32)

    def uniform(self, shape, lo=0.0, hi=1.0):
        return jax.random.uniform(self._next(), shape, jnp.bfloat16, lo, hi)

    def permutation(self, n):
        return jax.random.permutation(self._next(), n)
kernel_name = 'gated_mix__memory_aug_recurrent_mem_tr__moe_arch_mod__prompt'

def setup_inputs():
    _rng = _Rng(jax.random.key(int.from_bytes(__import__("os").urandom(4), "little")))
    _w = lambda a: (lambda t: t.astype(jnp.bfloat16) if jnp.issubdtype(t.dtype, jnp.floating) else t)(jnp.asarray(a))

    def _A_setup():
        B, S, Dm = (1, 2048, 1024)
        H, Dh = (32, 128)
        M, seg = (8, 32)
        seg = min(seg, S)
        S = S // seg * seg
        return {'x': _w((lambda *s: _rng.normal(s) * 0.05)(B, S, Dm)), 'mem0': _w((lambda *s: _rng.normal(s) * 0.05)(B, M, Dm)), 'Wq': _w((lambda *s: _rng.normal(s) * 0.05)(Dm, H, Dh) * Dm ** (-0.5)), 'Wk': _w((lambda *s: _rng.normal(s) * 0.05)(Dm, H, Dh) * Dm ** (-0.5)), 'Wv': _w((lambda *s: _rng.normal(s) * 0.05)(Dm, H, Dh) * Dm ** (-0.5)), 'Wo': _w((lambda *s: _rng.normal(s) * 0.05)(H, Dh, Dm) * (H * Dh) ** (-0.5)), 'seg_len': seg}
    _A_in = _A_setup()

    def _B_setup():
        B, S, D, F, C = (1, 2048, 1024, 3584, 8)
        return {'x': _w((lambda *s: _rng.normal(s) * 0.05)(B, S, D)), 'w_r': _w((lambda *s: _rng.normal(s) * 0.05)(D)), 'w_gate': _w((lambda *s: _rng.normal(s) * 0.05)(D, F)), 'w_up': _w((lambda *s: _rng.normal(s) * 0.05)(D, F)), 'w_down': _w((lambda *s: _rng.normal(s) * 0.05)(F, D))}
    _B_in = _B_setup()
    return {'A_x': _A_in['x'], 'A_mem0': _A_in['mem0'], 'A_Wq': _A_in['Wq'], 'A_Wk': _A_in['Wk'], 'A_Wv': _A_in['Wv'], 'A_Wo': _A_in['Wo'], 'A_seg_len': _A_in['seg_len'], 'B_x': _B_in['x'], 'B_w_r': _B_in['w_r'], 'B_w_gate': _B_in['w_gate'], 'B_w_up': _B_in['w_up'], 'B_w_down': _B_in['w_down'], 'gate_w': _w((lambda *s: _rng.normal(s) * 0.05)(1024))}

def reference(A_x, A_mem0, A_Wq, A_Wk, A_Wv, A_Wo, A_seg_len, B_x, B_w_r, B_w_gate, B_w_up, B_w_down, gate_w):

    def _A_ref(x, mem0, Wq, Wk, Wv, Wo, seg_len):
        B, S, Dm = x.shape
        H, Dh = (Wq.shape[1], Wq.shape[2])
        M = mem0.shape[1]
        scale = Dh ** (-0.5)
        n_seg = S // seg_len
        L = M + seg_len
        idx = jnp.arange(L)
        mask = (idx[:, None] < M) | (idx[:, None] >= idx[None, :])
        mem = mem0
        outs = []
        for s in range(n_seg):
            xs = x[:, s * seg_len:(s + 1) * seg_len, :].copy()
            h = jnp.concatenate([mem, xs], axis=1)
            q = jnp.einsum('btd,dhe->bhte', h, Wq)
            k = jnp.einsum('btd,dhe->bhte', h, Wk)
            v = jnp.einsum('btd,dhe->bhte', h, Wv)
            scores = jnp.einsum('bhqe,bhke->bhqk', q, k) * scale
            scores = jnp.where(mask[None, None], scores, -1000000000.0)
            p = _softmax(scores, axis=-1)
            o = jnp.einsum('bhqk,bhke->bhqe', p, v)
            o = jnp.einsum('bhte,hed->btd', o, Wo)
            mem = o[:, :M, :].copy()
            outs.append(o[:, M:, :])
        return jnp.concatenate(outs, axis=1)

    def _B_ref(x, w_r, w_gate, w_up, w_down):
        B, S, D = x.shape
        C = 8
        r = x @ w_r
        idx = jnp.argsort(-r, axis=-1)[:, :C]
        idx_e = jnp.repeat(idx.reshape(B, C, 1), D, axis=2)
        x_sel = jnp.take_along_axis(x, idx_e, axis=1)
        g = _silu(x_sel @ w_gate)
        u = x_sel @ w_up
        y = g * u @ w_down
        r_sel = _sigmoid(jnp.take_along_axis(r, idx, axis=1))
        y = y * r_sel.reshape(B, C, 1)
        b_off = (jnp.arange(B) * S).reshape(B, 1)
        flat_idx = (idx + b_off).reshape(B * C)
        zero = (x * 0.0).reshape(B * S, D)
        upd = _scatter_add(zero, flat_idx, y.reshape(B * C, D), axis=0)
        return x + upd.reshape(B, S, D)
    x = A_x
    g = _sigmoid((x * gate_w).sum(-1, keepdims=True))
    a = _A_ref(x, A_mem0, A_Wq, A_Wk, A_Wv, A_Wo, A_seg_len)
    b = _B_ref(x, B_w_r, B_w_gate, B_w_up, B_w_down)
    return g * a + (1 - g) * b
```

```python
import functools

import jax
import jax.numpy as jnp
from jax import lax
from jax.experimental import pallas as pl
from jax.experimental.pallas import tpu as pltpu

F32, BF16, U32, I32 = jnp.float32, jnp.bfloat16, jnp.uint32, jnp.int32

SEQ, DM, HEADS, HD = 2048, 1024, 32, 128
MEM, SEG, TOPK, FF = 8, 32, 8, 3584
NSEG = SEQ // SEG
NPAIR = HEADS // 2
NC = DM // 256
SROWS = NSEG * 8
UNROLL = 4
NFP = FF // 256
FF_LAG = NSEG // UNROLL - NFP
ROWS_P0 = 64
ROWS_FIN = 64
SEG_FIN = 16


def _mm(a, b):
    return jnp.dot(a, b, preferred_element_type=F32)


def _tile(i):
    return slice(i * 128, (i + 1) * 128)


def _rows(start, size):
    if isinstance(start, int):
        return pl.ds(start, size)
    return pl.ds(pl.multiple_of(start, size), size)


def _weight_blocks(b11, b12, b21, b22):
    resident = [b11, b21 - b11, b12 - b22, b22]
    alone = [b11 + b22, b11 + b12, b21 + b22]
    return resident, alone


def _resident_lhs(m1, m2, z1, z2):
    ms, zs = m1 + m2, z1 + z2
    parts = ((ms, zs[24:32], zs[0:16]), (m2, z2[24:32], z2[0:16]),
             (m1, z1[16:24], z1[0:16]), (ms, zs[16:24], zs[0:16]))
    return [jnp.concatenate(p, axis=0).astype(BF16) for p in parts]


def _alone_lhs(a11, a12, a21, a22):
    return [a11 + a22, a21 - a11, a12 - a22]


def _row_dot(x_tiles, w8):
    acc = x_tiles[0] * w8[0:1]
    for t in range(1, len(x_tiles)):
        acc = acc + x_tiles[t] * w8[t:t + 1]
    return jnp.sum(acc, axis=1, keepdims=True)


def _kernel(x_hbm, mem_hbm, wq_hbm, wk_hbm, wv_hbm, wo_hbm, wr_hbm, wg_hbm,
            wu_hbm, wd_hbm, gw_hbm, out_hbm,
            xbuf, mem_v, wr_v, gw_v, wres_u, wores_u, woalone_u, dbuf, xsel,
            rsel, idx_s):
    wres = wres_u.bitcast(BF16)
    wores = wores_u.bitcast(BF16)
    woalone = woalone_u.bitcast(BF16)

    def prologue(stage, wo_raw, xl_u, rkey, sem_w, sem_x, sem_o, sem_s):
        xl = xl_u.bitcast(BF16)
        stage32 = stage.bitcast(U32)
        w_hbm = (wq_hbm, wk_hbm, wv_hbm)
        crows = 256 * HEADS

        def w_copy(w, c):
            return pltpu.make_async_copy(
                w_hbm[w].at[_rows(c * crows, crows)], stage.at[w], sem_w.at[w])

        def xs_copy(c):
            sl = (slice(None), pl.ds(16, 16), _rows(c * 256, 256))
            return pltpu.make_async_copy(x_hbm.at[sl], xbuf.at[sl], sem_x.at[c])

        def xp_copy(h):
            sl = (_rows(h * (NSEG // 2), NSEG // 2), pl.ds(0, 16), slice(None))
            return pltpu.make_async_copy(x_hbm.at[sl], xbuf.at[sl], sem_x.at[NC + h])

        def wo_copy(p):
            sl = _rows(p * 512, 512)
            return pltpu.make_async_copy(wo_hbm.at[sl], wo_raw.at[sl], sem_o.at[p])

        small = [pltpu.make_async_copy(s, d, sem_s.at[i]) for i, (s, d) in enumerate(
            ((mem_hbm, mem_v), (wr_hbm, wr_v), (gw_hbm, gw_v)))]

        def x_blocks(c, sp):
            got = []
            for s in (2 * sp, 2 * sp + 1):
                z = xbuf[s, 16:32, _rows(c * 256, 256)].astype(F32)
                got.append(_alone_lhs(z[0:8, :128], z[0:8, 128:], z[8:16, :128], z[8:16, 128:]))
            for t in range(3):
                xl.at[c][_rows(sp * 16, 16), _tile(t)] = jnp.concatenate(
                    [got[0][t], got[1][t]], axis=0).astype(BF16)

        def qkv_unit(w, c, j):
            h1 = stage32[w, pl.ds(j, 128, stride=NPAIR), :]
            h2 = stage32[w, pl.ds(128 * NPAIR + j, 128, stride=NPAIR), :]
            even = lambda z: pltpu.bitcast(z << 16, F32)
            odd = lambda z: pltpu.bitcast((z >> 16) << 16, F32)
            resident, alone = _weight_blocks(even(h1), odd(h1), even(h2), odd(h2))
            u = w * NPAIR + j
            for t in range(4):
                wres.at[u][_rows(c * 128, 128), _tile(t)] = resident[t].astype(BF16)
            alone = [a.astype(BF16) for a in alone]
            for r in range(0, SROWS, ROWS_P0):
                rows = pl.ds(r, ROWS_P0)
                m1, m6, m7 = [_mm(xl.at[c][rows, _tile(t)], alone[t]) for t in range(3)]
                for t, d in enumerate((m1 + m7, m1 + m6)):
                    old = dbuf[u, rows, _tile(t)]
                    if not isinstance(c, int):
                        old = jnp.where(c > 0, old, 0.0)
                    dbuf[u, rows, _tile(t)] = d + old

        def wo_unit(j, c):
            top = wo_raw[j * 256:j * 256 + 128, c * 256:(c + 1) * 256].astype(F32)
            bot = wo_raw[j * 256 + 128:(j + 1) * 256, c * 256:(c + 1) * 256].astype(F32)
            resident, alone = _weight_blocks(top[:, :128], top[:, 128:], bot[:, :128], bot[:, 128:])
            for t in range(4):
                wores.at[c][_tile(j), _tile(t)] = resident[t].astype(BF16)
            for t in range(3):
                woalone.at[c][_tile(j), _tile(t)] = alone[t].astype(BF16)

        lane = lax.broadcasted_iota(I32, (8, 128), 1)
        sub = lax.broadcasted_iota(I32, (8, 128), 0)

        def router_scores(s, acc):
            xs = [xbuf[s, :, _tile(t)].astype(F32) for t in range(DM // 128)]
            r = _row_dot(xs, wr_v[...].astype(F32))
            for i in range(SEG // 8):
                acc = jnp.where(lane == (4 * s + i) % 128, r[8 * i:8 * i + 8], acc)
            return acc

        def router_keys(h, r):
            r = r.astype(BF16).astype(F32)
            bits = pltpu.bitcast(jnp.where(r == 0.0, 0.0, r), I32) >> 16
            order = jnp.where(bits < 0, ~bits, bits + 0x8000)
            order = jnp.where(r != r, 0, order)
            token = (h * 128 + lane) * 8 + sub
            return pltpu.bitcast((1 << 29) + (order << 11) + (SEQ - 1 - token), F32)

        def select_tokens():
            keys = [rkey[0], rkey[1]]
            row16 = lax.broadcasted_iota(I32, (16, DM), 0)
            row8 = lax.broadcasted_iota(I32, (8, DM), 0)
            picked = jnp.zeros((8, DM), F32)
            for i in range(TOPK):
                top = jnp.max(jnp.maximum(keys[0], keys[1]), axis=0, keepdims=True)
                top = jnp.max(top, axis=1, keepdims=True)
                keys = [jnp.where(k == top, 0.0, k) for k in keys]
                token = SEQ - 1 - (pltpu.bitcast(jnp.broadcast_to(top, (8, 128)), I32)[0, 0] & (SEQ - 1))
                idx_s[i] = token
                blk = xbuf[token >> 5, _rows(token & 16, 16), :].astype(F32)
                row = jnp.sum(jnp.where(row16 == (token & 15), blk, 0.0), axis=0, keepdims=True)
                picked = jnp.where(row8 == i, row, picked)
            xsel[...] = picked
            r = _row_dot([picked[:, _tile(t)] for t in range(DM // 128)], wr_v[...].astype(F32))
            rsel[...] = jnp.broadcast_to(jax.nn.sigmoid(r), (8, 128))

        xs_copy(0).start()
        for w in range(3):
            w_copy(w, 0).start()
        xs_copy(1).start()
        for cp in small:
            cp.start()
        xs_copy(0).wait()
        for sp in range(NSEG // 2):
            x_blocks(0, sp)

        def early(c, carry):
            for w in range(3):
                w_copy(w, c).wait()
                if w == 1:
                    xs_copy(c + 1).wait()
                for j in range(NPAIR):
                    qkv_unit(w, c, j)
                    if w >= 1:
                        x_blocks(c + 1, (w - 1) * NPAIR + j)
                w_copy(w, c + 1).start()
                if w == 0:
                    @pl.when(c < 2)
                    def _():
                        xs_copy(c + 2).start()
                        xp_copy(c).start()

                    @pl.when(c == 2)
                    def _():
                        wo_copy(4).start()
                        wo_copy(5).start()
                else:
                    wo_copy(jnp.where(c < 2, 2 * c, 6) + w - 1).start()
            return carry

        lax.fori_loop(0, NC - 1, early, 0)

        for cp in small:
            cp.wait()
        wo_first = (0, 6, 12, NPAIR)
        for w in range(3):
            w_copy(w, NC - 1).wait()
            if w < 2:
                xp_copy(w).wait()
            wo_todo = [(j, c) for j in range(wo_first[w], wo_first[w + 1]) for c in range(NC)]
            per = -(-len(wo_todo) // NPAIR)
            for p in range(wo_first[w] // 2, wo_first[w + 1] // 2):
                wo_copy(p).wait()
            scores = jnp.zeros((8, 128), F32)
            for j in range(NPAIR):
                qkv_unit(w, NC - 1, j)
                for jc in wo_todo[j * per:(j + 1) * per]:
                    wo_unit(*jc)
                if w < 2:
                    for s in (2 * j, 2 * j + 1):
                        scores = router_scores(w * (NSEG // 2) + s, scores)
                elif j == 0:
                    select_tokens()
            if w < 2:
                rkey[w] = router_keys(w, scores)

    pl.run_scoped(
        prologue,
        pltpu.VMEM((3, 256 * HEADS, HD), BF16),
        pltpu.VMEM((HEADS * HD, DM), BF16),
        pltpu.VMEM((NC, SROWS // 2, 3 * 128), U32),
        pltpu.VMEM((2, 8, 128), F32),
        pltpu.SemaphoreType.DMA((3,)),
        pltpu.SemaphoreType.DMA((NC + 2,)),
        pltpu.SemaphoreType.DMA((8,)),
        pltpu.SemaphoreType.DMA((3,)),
    )

    def main(lhs_u, olhs_u, oalone_u, apart, gate, wg_v, wu_v, wd_v, sem_f, sem_out):
        lhs = lhs_u.bitcast(BF16)
        olhs = olhs_u.bitcast(BF16)
        oalone = oalone_u.bitcast(BF16)

        ff_copies = []
        for t in range(FF // 128):
            ff_copies.append(pltpu.make_async_copy(wg_hbm.at[:, _tile(t)], wg_v.at[t], sem_f))
            ff_copies.append(pltpu.make_async_copy(wu_hbm.at[:, _tile(t)], wu_v.at[t], sem_f))
        for t in range(DM // 128):
            ff_copies.append(pltpu.make_async_copy(
                wd_hbm.at[:, _tile(t)], wd_v.at[t, pl.ds(0, FF)], sem_f))
        for cp in ff_copies:
            cp.start()
        for t in (2 * NFP, 2 * NFP + 1):
            wg_v[t] = jnp.zeros((DM, 128), BF16)
            wu_v[t] = jnp.zeros((DM, 128), BF16)
        for t in range(DM // 128):
            wd_v[t, FF:FF + 256, :] = jnp.zeros((256, 128), BF16)

        qi = lax.broadcasted_iota(I32, (MEM + SEG, MEM + SEG), 0)
        ki = lax.broadcasted_iota(I32, (MEM + SEG, MEM + SEG), 1)
        visible = (qi < MEM) | (qi >= ki)

        def attend(q, k):
            sc = lax.dot_general(q, k, (((1,), (1,)), ((), ())), preferred_element_type=F32)
            sc = jnp.where(visible, sc * HD ** -0.5, -1000000000.0)
            e = jnp.exp(sc - jnp.max(sc, axis=1, keepdims=True))
            return e / jnp.sum(e, axis=1, keepdims=True)

        def segment(s, mem, held):
            r8, r32 = _rows(s * 8, 8), _rows(s * SEG, SEG)
            xs = [xbuf[s, :, _tile(t)].astype(F32) for t in range(DM // 128)]
            for c in range(NC):
                ops = _resident_lhs(mem[2 * c], mem[2 * c + 1], xs[2 * c], xs[2 * c + 1])
                for t in range(4):
                    lhs.at[t][:, _tile(c)] = ops[t]
            gate[r32, :] = jnp.broadcast_to(
                jax.nn.sigmoid(_row_dot(xs, gw_v[...].astype(F32))), (SEG, 128))

            def project(w, j):
                u = w * NPAIR + j
                m2, m4, m3, m5 = [_mm(lhs[t], wres.at[u][:, _tile(t)]) for t in range(4)]
                left, right = m2 + m4, m3 + m5
                c11 = m4[8:16] - m5[8:16] + dbuf[u, r8, _tile(0)]
                c22 = m3[8:16] - m2[8:16] + dbuf[u, r8, _tile(1)]
                return (jnp.concatenate([left[0:8], left[16:32], c11, left[8:16]], axis=0),
                        jnp.concatenate([right[0:8], right[16:32], right[8:16], c22], axis=0))

            keep = {}

            def values(j, p, v):
                oe, oo = _mm(p[0], v[0]), _mm(p[1], v[1])
                ops = _resident_lhs(oe[0:8], oo[0:8], oe[8:40], oo[8:40])
                for t in range(4):
                    olhs.at[t][:, _tile(j)] = ops[t]
                alone = _alone_lhs(oe[24:32], oo[24:32], oe[32:40], oo[32:40])
                if held is None:
                    keep[j] = alone
                else:
                    for t in range(3):
                        oalone.at[t][_rows((s - 1) * 8, 16), _tile(j)] = jnp.concatenate(
                            [held[j][t], alone[t]], axis=0).astype(BF16)

            def out_proj(c, j0, j1):
                k = slice(j0 * 128, j1 * 128)
                return [_mm(olhs.at[t][:, k], wores.at[c][k, _tile(t)]) for t in range(4)]

            new_mem = [None] * (2 * NC)

            def out_done(c, ms):
                m2, m4, m3, m5 = ms
                left, right = m2 + m4, m3 + m5
                new_mem[2 * c], new_mem[2 * c + 1] = left[0:8], right[0:8]
                apart[r32, _tile(2 * c)] = jnp.concatenate(
                    [left[16:32], m4[8:16] - m5[8:16], left[8:16]], axis=0)
                apart[r32, _tile(2 * c + 1)] = jnp.concatenate(
                    [right[16:32], right[8:16], m3[8:16] - m2[8:16]], axis=0)

            pending = None
            for j in range(0, NPAIR, 2):
                q0, k0 = project(0, j), project(1, j)
                q1, k1 = project(0, j + 1), project(1, j + 1)
                if pending is not None:
                    values(j - 2, *pending[0])
                    values(j - 1, *pending[1])
                v0 = project(2, j)
                p0 = [attend(q0[0], k0[0]), attend(q0[1], k0[1])]
                p1 = [attend(q1[0], k1[0]), attend(q1[1], k1[1])]
                v1 = project(2, j + 1)
                pending = ((p0, v0), (p1, v1))
            split = NPAIR - 4
            head0 = out_proj(0, 0, split)
            values(NPAIR - 2, *pending[0])
            values(NPAIR - 1, *pending[1])
            head1 = out_proj(1, 0, split)
            for c, head in enumerate((head0, head1)):
                out_done(c, [tail + h for tail, h in zip(out_proj(c, split, NPAIR), head)])
            for c in range(2, NC):
                out_done(c, out_proj(c, 0, NPAIR))
            return new_mem, keep

        def trip(i, carry):
            mem, y = list(carry[0]), carry[1]

            @pl.when(i == FF_LAG)
            def _():
                for cp in ff_copies:
                    cp.wait()

            f = jnp.where(i < FF_LAG, NFP, i - FF_LAG)
            mem, held = segment(i * UNROLL, mem, None)
            ff_g = [_mm(xsel[...], wg_v[2 * f + h]) for h in range(2)]
            mem, _ = segment(i * UNROLL + 1, mem, held)
            ff_u = [_mm(xsel[...], wu_v[2 * f + h]) for h in range(2)]
            mem, held = segment(i * UNROLL + 2, mem, None)
            act = jnp.concatenate([jax.nn.silu(g) * u for g, u in zip(ff_g, ff_u)], axis=1)
            y = tuple(_mm(act, wd_v[t, _rows(f * 256, 256), :]) + y[t] for t in range(DM // 128))
            mem, _ = segment(i * UNROLL + 3, mem, held)
            return tuple(mem), y

        mem0 = tuple(mem_v[:, _tile(t)].astype(F32) for t in range(DM // 128))
        y0 = tuple(jnp.zeros((8, 128), F32) for _ in range(DM // 128))
        _, y = lax.fori_loop(0, NSEG // UNROLL, trip, (mem0, y0))

        row16 = lax.broadcasted_iota(I32, (16, DM), 0)
        y = jnp.concatenate([yt * rsel[...] for yt in y], axis=1)
        for i in range(TOPK):
            token = idx_s[i]
            where = (token >> 5, _rows(token & 16, 16), slice(None))
            upd = jnp.where(row16 == (token & 15), y[i:i + 1], 0.0)
            xbuf[where] = (xbuf[where].astype(F32) + upd).astype(BF16)

        def out_copy(n, c):
            sl = (_rows(n * SEG_FIN, SEG_FIN), slice(None), pl.ds(c * 256, 256))
            return pltpu.make_async_copy(xbuf.at[sl], out_hbm.at[sl], sem_out)

        def finish(n, carry):
            for c in range(NC):
                for r in range(0, SEG_FIN * 8, ROWS_FIN):
                    rows = _rows(n * SEG_FIN * 8 + r, ROWS_FIN)
                    m1, m6, m7 = [_mm(oalone.at[t][rows, :], woalone.at[c][:, _tile(t)])
                                  for t in range(3)]
                    d11, d22 = m1 + m7, m1 + m6
                    for i in range(ROWS_FIN // 8):
                        s = n * SEG_FIN + r // 8 + i
                        r32 = _rows(s * SEG, SEG)
                        g = gate[r32, :]
                        al, ar = apart[r32, _tile(2 * c)], apart[r32, _tile(2 * c + 1)]
                        al = jnp.concatenate(
                            [al[0:16], al[16:24] + d11[8 * i:8 * i + 8], al[24:32]], axis=0)
                        ar = jnp.concatenate(
                            [ar[0:24], ar[24:32] + d22[8 * i:8 * i + 8]], axis=0)
                        for t, a in ((2 * c, al), (2 * c + 1, ar)):
                            b = xbuf[s, :, _tile(t)].astype(F32)
                            xbuf[s, :, _tile(t)] = (g * a + (1.0 - g) * b).astype(BF16)
                out_copy(n, c).start()
            return carry

        lax.fori_loop(0, NSEG // SEG_FIN, finish, 0)
        for n in range(NSEG // SEG_FIN):
            for c in range(NC):
                out_copy(n, c).wait()

    pl.run_scoped(
        main,
        pltpu.VMEM((4, 16, NC * 128), U32),
        pltpu.VMEM((4, 16, NPAIR * 128), U32),
        pltpu.VMEM((3, SROWS // 2, NPAIR * 128), U32),
        pltpu.VMEM((SEQ, DM), F32),
        pltpu.VMEM((SEQ, 128), F32),
        pltpu.VMEM((2 * NFP + 2, DM, 128), BF16),
        pltpu.VMEM((2 * NFP + 2, DM, 128), BF16),
        pltpu.VMEM((DM // 128, FF + 256, 128), BF16),
        pltpu.SemaphoreType.DMA,
        pltpu.SemaphoreType.DMA,
    )


@functools.partial(jax.jit, static_argnames=("A_seg_len",))
def pallas_gated_mix__memory_aug_recurrent_mem_tr__moe_arch_mod__prompt_kernel(
    A_x: jax.Array,
    A_mem0: jax.Array,
    A_Wq: jax.Array,
    A_Wk: jax.Array,
    A_Wv: jax.Array,
    A_Wo: jax.Array,
    A_seg_len: int,
    B_x: jax.Array,
    B_w_r: jax.Array,
    B_w_gate: jax.Array,
    B_w_up: jax.Array,
    B_w_down: jax.Array,
    gate_w: jax.Array,
):
    del B_x
    assert A_seg_len == SEG and A_x.shape == (1, SEQ, DM) and A_mem0.shape == (1, MEM, DM)
    assert A_Wq.shape == (DM, HEADS, HD) and B_w_gate.shape == (DM, FF)

    hbm = pl.BlockSpec(memory_space=pl.ANY)
    out = pl.pallas_call(
        _kernel,
        out_shape=jax.ShapeDtypeStruct((NSEG, SEG, DM), BF16),
        in_specs=[hbm] * 11,
        out_specs=hbm,
        scratch_shapes=[
            pltpu.VMEM((NSEG, SEG, DM), BF16),
            pltpu.VMEM((MEM, DM), BF16),
            pltpu.VMEM((8, 128), BF16),
            pltpu.VMEM((8, 128), BF16),
            pltpu.VMEM((3 * NPAIR, 256, 4 * 128), U32),
            pltpu.VMEM((NC, NPAIR * 64, 4 * 128), U32),
            pltpu.VMEM((NC, NPAIR * 64, 3 * 128), U32),
            pltpu.VMEM((3 * NPAIR, SROWS, 2 * 128), F32),
            pltpu.VMEM((TOPK, DM), F32),
            pltpu.VMEM((TOPK, 128), F32),
            pltpu.SMEM((TOPK,), I32),
        ],
        compiler_params=pltpu.CompilerParams(vmem_limit_bytes=122 * 1024 * 1024),
    )(
        A_x.reshape(NSEG, SEG, DM),
        A_mem0.reshape(MEM, DM),
        A_Wq.reshape(DM * HEADS, HD),
        A_Wk.reshape(DM * HEADS, HD),
        A_Wv.reshape(DM * HEADS, HD),
        A_Wo.reshape(HEADS * HD, DM),
        B_w_r.reshape(8, 128),
        B_w_gate,
        B_w_up,
        B_w_down,
        gate_w.reshape(8, 128),
    )
    return out.reshape(1, SEQ, DM)
```

```python
import functools

import jax
import jax.numpy as jnp
import numpy as np
from jax import lax
from jax.experimental import pallas as pl
from jax.experimental.pallas import tpu as pltpu

F32, BF16, U32, I32 = jnp.float32, jnp.bfloat16, jnp.uint32, jnp.int32

SEQ, DM, HEADS, HD = 2048, 1024, 32, 128
MEM, SEG, TOPK, FF = 8, 32, 8, 3584
NSEG = SEQ // SEG
NPAIR = HEADS // 2
NC = DM // 256
SROWS = NSEG * 8
UNROLL = 4
NFP = FF // 256
ROWS_P0 = 64
ROWS_FIN = 64
SEG_FIN = 16


def _mm(a, b):
    return jnp.dot(a, b, preferred_element_type=F32)


def _tile(i):
    return slice(i * 128, (i + 1) * 128)


def _rows(start, size):
    if isinstance(start, int):
        return pl.ds(start, size)
    return pl.ds(pl.multiple_of(start, size), size)


def _window(first, count, unit):
    start = first * unit
    return pl.ds(start if isinstance(start, int) else pl.multiple_of(start, unit), count * unit)


def _weight_blocks(b11, b12, b21, b22):
    resident = [b11, b21 - b11, b12 - b22, b22]
    alone = [b11 + b22, b11 + b12, b21 + b22]
    return resident, alone


def _resident_lhs(m1, m2, z1, z2):
    ms, zs = m1 + m2, z1 + z2
    parts = ((ms, zs[24:32], zs[0:16]), (m2, z2[24:32], z2[0:16]),
             (m1, z1[16:24], z1[0:16]), (ms, zs[16:24], zs[0:16]))
    return [jnp.concatenate(p, axis=0).astype(BF16) for p in parts]


def _alone_lhs(a11, a12, a21, a22):
    return [a11 + a22, a21 - a11, a12 - a22]


def _row_dot(x_tiles, w8):
    acc = x_tiles[0] * w8[0:1]
    for t in range(1, len(x_tiles)):
        acc = acc + x_tiles[t] * w8[t:t + 1]
    return jnp.sum(acc, axis=1, keepdims=True)


def _kernel(x_hbm, mem_hbm, wq_hbm, wk_hbm, wv_hbm, wo_hbm, wr_hbm, wg_hbm,
            wu_hbm, wd_hbm, gw_hbm, out_hbm,
            xbuf, mem_v, wr_v, gw_v, stage, wo_raw, xl_u, wres_u, wores_u,
            woalone_u, dbuf, lhs_u, olhs_u, oalone_u, apart, gate, ffw, idx_s,
            sem_w, sem_x, sem_o, sem_s, sem_f, sem_out):
    xl = xl_u.bitcast(BF16)
    wres = wres_u.bitcast(BF16)
    wores = wores_u.bitcast(BF16)
    woalone = woalone_u.bitcast(BF16)
    lhs = lhs_u.bitcast(BF16)
    olhs = olhs_u.bitcast(BF16)
    oalone = oalone_u.bitcast(BF16)
    stage32 = stage.bitcast(U32)

    lane = lax.broadcasted_iota(I32, (8, 128), 1)
    sub = lax.broadcasted_iota(I32, (8, 128), 0)
    row16 = lax.broadcasted_iota(I32, (16, DM), 0)

    def w_start(w, c):
        for g in range(HEADS // 8):
            pltpu.make_async_copy(
                (wq_hbm, wk_hbm, wv_hbm)[w].at[_rows(c * 2048, 2048), _tile(g)],
                stage.at[w, g], sem_w.at[w]).start()

    def w_wait(w):
        pltpu.make_async_copy(stage.at[w], stage.at[w], sem_w.at[w]).wait()

    def xs_copy(c):
        sl = (slice(None), pl.ds(16, 16), _rows(c * 256, 256))
        return pltpu.make_async_copy(x_hbm.at[sl], xbuf.at[sl], sem_x.at[c])

    def xp_copy():
        sl = (slice(None), pl.ds(0, 16), slice(None))
        return pltpu.make_async_copy(x_hbm.at[sl], xbuf.at[sl], sem_x.at[NC])

    def wo_copy(p):
        sl = _rows(p * 512, 512)
        return pltpu.make_async_copy(wo_hbm.at[sl], wo_raw.at[sl], sem_o.at[p])

    def ff_start(f):
        for h in range(2):
            cols = _rows(f * 256 + h * 128, 128)
            for n, src in enumerate((wg_hbm, wu_hbm)):
                pltpu.make_async_copy(
                    src.at[:, cols], ffw.at[f, pl.ds((2 * n + h) * DM, DM)], sem_f.at[f]).start()
        for t in range(DM // 128):
            pltpu.make_async_copy(
                wd_hbm.at[_rows(f * 256, 256), _tile(t)],
                ffw.at[f, pl.ds(4 * DM + t * 256, 256)], sem_f.at[f]).start()

    def ff_wait(f):
        pltpu.make_async_copy(ffw.at[f], ffw.at[f], sem_f.at[f]).wait()

    small = [pltpu.make_async_copy(s, d, sem_s.at[i]) for i, (s, d) in enumerate(
        ((mem_hbm, mem_v), (wr_hbm, wr_v), (gw_hbm, gw_v)))]

    def x_blocks(c, first, count):
        src = xbuf.at[pl.ds(2 * first, 2 * count), :, _rows(c * 256, 256)]
        dst = xl.at[c, _window(first, count, 16)]
        for n in range(count):
            got = []
            for s in (2 * n, 2 * n + 1):
                z = src[s, 16:32, :].astype(F32)
                got.append(_alone_lhs(z[0:8, :128], z[0:8, 128:], z[8:16, :128], z[8:16, 128:]))
            for t in range(3):
                dst[pl.ds(n * 16, 16), _tile(t)] = jnp.concatenate(
                    [got[0][t], got[1][t]], axis=0).astype(BF16)

    def qkv_blocks(w, c, j):
        raw = stage32.at[w, j // 4]
        res = wres.at[pl.ds(w * NPAIR, NPAIR), _rows(c * 128, 128)]
        even = lambda z: pltpu.bitcast(z << 16, F32)
        odd = lambda z: pltpu.bitcast(z & np.uint32(0xFFFF0000), F32)
        rest = []
        for r in range(112, -16, -16):
            h1 = raw[pl.ds(4 * r + j % 4, 16, stride=4), :]
            h2 = raw[pl.ds(4 * (128 + r) + j % 4, 16, stride=4), :]
            resident, alone = _weight_blocks(even(h1), odd(h1), even(h2), odd(h2))
            res.at[j][pl.ds(r, 16), :] = jnp.concatenate(resident, axis=1).astype(BF16)
            rest.insert(0, alone)
        return tuple(jnp.concatenate(a, axis=0).astype(BF16) for a in zip(*rest))

    def wo_blocks(views, j, c, r, pace):
        raw, res, rest = views
        top = raw[pl.ds(j * 256 + r, 16), c * 256:(c + 1) * 256].astype(F32)
        bot = raw[pl.ds(j * 256 + 128 + r, 16), c * 256:(c + 1) * 256].astype(F32)
        resident, alone = _weight_blocks(
            pace(top[:, :128]), top[:, 128:], bot[:, :128], bot[:, 128:])
        res.at[c][pl.ds(j * 128 + r, 16), :] = jnp.concatenate(resident, axis=1).astype(BF16)
        rest.at[c][pl.ds(j * 128 + r, 16), :] = jnp.concatenate(alone, axis=1).astype(BF16)

    def router_scores(s, half, scores, pace):
        xs = [xbuf[s, 16 * half:16 * half + 16, _tile(t)].astype(F32) for t in range(DM // 128)]
        r = _row_dot([pace(xs[0])] + xs[1:], wr_v[...].astype(F32))
        for i in range(2):
            scores = [jnp.where(lane == 4 * s + 2 * half + i - 128 * h, r[8 * i:8 * i + 8], acc)
                      for h, acc in enumerate(scores)]
        return scores

    def qkv_chunk(w, c, extra):
        sums = dbuf.at[pl.ds(w * NPAIR, NPAIR)]
        alone = qkv_blocks(w, c, 0)
        for j in range(NPAIR):
            ahead = qkv_blocks(w, c, j + 1) if j + 1 < NPAIR else None
            for r in range(0, SROWS, ROWS_P0):
                rows = pl.ds(r, ROWS_P0)
                ops = [xl.at[c][rows, _tile(t)] for t in range(3)]
                if ahead is not None:
                    n = 128 - 16 * min((r + ROWS_P0) * 8 // SROWS + 1, 8)
                    ops[0] = jnp.concatenate(
                        [jnp.where(w < 0, ahead[0][n:n + 16], ops[0][:16]), ops[0][16:]], axis=0)
                m1, m6, m7 = [_mm(ops[t], alone[t]) for t in range(3)]
                for t, d in enumerate((m1 + m7, m1 + m6)):
                    old = sums[j, rows, _tile(t)]
                    if not isinstance(c, int):
                        old = jnp.where(c > 0, old, 0.0)
                    sums[j, rows, _tile(t)] = d + old
                extra((j * SROWS + r) // ROWS_P0, m1)
            alone = ahead

    xs_copy(0).start()
    w_start(0, 0)
    w_start(1, 0)
    xs_copy(1).start()
    w_start(2, 0)
    for cp in small:
        cp.start()
    xs_copy(0).wait()
    x_blocks(0, 0, NSEG // 2)

    def early(i, carry):
        c, w = i // 3, i % 3
        w_wait(w)

        @pl.when(w == 1)
        def _():
            xs_copy(c + 1).wait()

        qkv_chunk(w, c, lambda n, m: None)
        x_blocks(jnp.where(w == 0, c, c + 1), jnp.where(w == 2, NSEG // 4, 0), NSEG // 4)
        for n in range(3):
            @pl.when(w == n)
            def _():
                w_start(n, c + 1)

        @pl.when((i == 0) | (i == 3))
        def _():
            xs_copy(c + 2).start()

        @pl.when(i == 0)
        def _():
            xp_copy().start()

        @pl.when(i > 0)
        def _():
            wo_copy(i - 1).start()

        return carry

    lax.fori_loop(0, 3 * (NC - 1), early, 0)

    for cp in small:
        cp.wait()
    xp_copy().wait()
    ff_start(0)

    def last(w, scores):
        scores = list(scores)
        w_wait(w)
        for n in range(3):
            @pl.when(3 * w + n < 8)
            def _():
                wo_copy(jnp.minimum(3 * w + n, 7)).wait()

        j0 = jnp.minimum(6 * w, NPAIR - 6)
        s0 = jnp.minimum(22 * w, NSEG - 22)
        wo_todo = [(j, c, r) for j in range(6) for c in range(NC) for r in range(0, 128, 16)]
        slots = (NPAIR * SROWS - 128) // ROWS_P0
        views = (wo_raw.at[_window(j0, 6, 256)], wores.at[:, _window(j0, 6, 128)],
                 woalone.at[:, _window(j0, 6, 128)])

        def extra(n, m):
            pace = lambda z: jnp.where(w < 0, m[:z.shape[0]], z)
            for item in wo_todo[len(wo_todo) * n // slots:len(wo_todo) * (n + 1) // slots]:
                wo_blocks(views, *item, pace)
            for g in range(44 * n // slots, min(44 * (n + 1) // slots, 44)):
                scores[:] = router_scores(s0 + g // 2, g % 2, scores, pace)

        qkv_chunk(w, NC - 1, extra)
        return tuple(scores)

    zero = jnp.zeros((8, 128), F32)
    scores = lax.fori_loop(0, 3, last, (zero, zero))

    keys = []
    for h, r in enumerate(scores):
        r = r.astype(BF16).astype(F32)
        bits = pltpu.bitcast(jnp.where(r == 0.0, 0.0, r), I32) >> 16
        order = jnp.where(r != r, 0, jnp.where(bits < 0, ~bits, bits + 0x8000))
        token = (h * 128 + lane) * 8 + sub
        keys.append(pltpu.bitcast((1 << 29) + (order << 11) + (SEQ - 1 - token), F32))
    row8 = lax.broadcasted_iota(I32, (8, DM), 0)
    xsel = jnp.zeros((8, DM), F32)
    for i in range(TOPK):
        top = jnp.max(jnp.maximum(keys[0], keys[1]), axis=0, keepdims=True)
        top = jnp.max(top, axis=1, keepdims=True)
        keys = [jnp.where(k == top, 0.0, k) for k in keys]
        token = SEQ - 1 - (pltpu.bitcast(jnp.broadcast_to(top, (8, 128)), I32)[0, 0] & (SEQ - 1))
        idx_s[i] = token
        blk = xbuf[token >> 5, _rows(token & 16, 16), :].astype(F32)
        row = jnp.sum(jnp.where(row16 == (token & 15), blk, 0.0), axis=0, keepdims=True)
        xsel = jnp.where(row8 == i, row, xsel)

    qi = lax.broadcasted_iota(I32, (MEM + SEG, MEM + SEG), 0)
    ki = lax.broadcasted_iota(I32, (MEM + SEG, MEM + SEG), 1)
    visible = (qi < MEM) | (qi >= ki)

    def attend(q, k):
        sc = lax.dot_general(q, k, (((1,), (1,)), ((), ())), preferred_element_type=F32)
        sc = jnp.where(visible, sc * HD ** -0.5, -1000000000.0)
        e = jnp.exp(sc - jnp.max(sc, axis=1, keepdims=True))
        return e / jnp.sum(e, axis=1, keepdims=True)

    def segment(s, mem, held):
        r8, r32 = _rows(s * 8, 8), _rows(s * SEG, SEG)
        xs = [xbuf[s, :, _tile(t)].astype(F32) for t in range(DM // 128)]
        for c in range(NC):
            ops = _resident_lhs(mem[2 * c], mem[2 * c + 1], xs[2 * c], xs[2 * c + 1])
            for t in range(4):
                lhs.at[t][:, _tile(c)] = ops[t]
        gate[r32, :] = jnp.broadcast_to(
            jax.nn.sigmoid(_row_dot(xs, gw_v[...].astype(F32))), (SEG, 128))

        def project(w, j):
            u = w * NPAIR + j
            m2, m4, m3, m5 = [_mm(lhs[t], wres.at[u][:, _tile(t)]) for t in range(4)]
            left, right = m2 + m4, m3 + m5
            c11 = m4[8:16] - m5[8:16] + dbuf[u, r8, _tile(0)]
            c22 = m3[8:16] - m2[8:16] + dbuf[u, r8, _tile(1)]
            return (jnp.concatenate([left[0:8], left[16:32], c11, left[8:16]], axis=0),
                    jnp.concatenate([right[0:8], right[16:32], right[8:16], c22], axis=0))

        keep = {}

        def values(j, p, v):
            oe, oo = _mm(p[0], v[0]), _mm(p[1], v[1])
            ops = _resident_lhs(oe[0:8], oo[0:8], oe[8:40], oo[8:40])
            for t in range(4):
                olhs.at[t][:, _tile(j)] = ops[t]
            alone = _alone_lhs(oe[24:32], oo[24:32], oe[32:40], oo[32:40])
            if held is None:
                keep[j] = alone
            else:
                for t in range(3):
                    oalone.at[t][_rows((s - 1) * 8, 16), _tile(j)] = jnp.concatenate(
                        [held[j][t], alone[t]], axis=0).astype(BF16)

        def out_proj(c, j0, j1):
            k = slice(j0 * 128, j1 * 128)
            return [_mm(olhs.at[t][:, k], wores.at[c][k, _tile(t)]) for t in range(4)]

        new_mem = [None] * (2 * NC)

        def out_done(c, ms):
            m2, m4, m3, m5 = ms
            left, right = m2 + m4, m3 + m5
            new_mem[2 * c], new_mem[2 * c + 1] = left[0:8], right[0:8]
            apart[r32, _tile(2 * c)] = jnp.concatenate(
                [left[16:32], m4[8:16] - m5[8:16], left[8:16]], axis=0)
            apart[r32, _tile(2 * c + 1)] = jnp.concatenate(
                [right[16:32], right[8:16], m3[8:16] - m2[8:16]], axis=0)

        pending = None
        for j in range(0, NPAIR, 2):
            q0, k0 = project(0, j), project(1, j)
            q1, k1 = project(0, j + 1), project(1, j + 1)
            if pending is not None:
                values(j - 2, *pending[0])
                values(j - 1, *pending[1])
            v0 = project(2, j)
            p0 = [attend(q0[0], k0[0]), attend(q0[1], k0[1])]
            p1 = [attend(q1[0], k1[0]), attend(q1[1], k1[1])]
            v1 = project(2, j + 1)
            pending = ((p0, v0), (p1, v1))
        split = NPAIR - 4
        head0 = out_proj(0, 0, split)
        values(NPAIR - 2, *pending[0])
        values(NPAIR - 1, *pending[1])
        head1 = out_proj(1, 0, split)
        for c, head in enumerate((head0, head1)):
            out_done(c, [tail + h for tail, h in zip(out_proj(c, split, NPAIR), head)])
        for c in range(2, NC):
            out_done(c, out_proj(c, 0, NPAIR))
        return new_mem, keep

    def trip(i, carry):
        mem, y = list(carry[0]), carry[1]
        f = jnp.minimum(i, NFP - 1)

        @pl.when(i < NFP)
        def _():
            ff_wait(f)

        @pl.when(i + 1 < NFP)
        def _():
            ff_start(jnp.minimum(i + 1, NFP - 1))

        mem, held = segment(i * UNROLL, mem, None)
        ff_g = [_mm(xsel, ffw[f, pl.ds(h * DM, DM), :]) for h in range(2)]
        mem, _ = segment(i * UNROLL + 1, mem, held)
        ff_u = [_mm(xsel, ffw[f, pl.ds((2 + h) * DM, DM), :]) for h in range(2)]
        mem, held = segment(i * UNROLL + 2, mem, None)
        act = jnp.concatenate([jax.nn.silu(g) * u for g, u in zip(ff_g, ff_u)], axis=1)
        y = tuple(y[t] + jnp.where(i < NFP, _mm(act, ffw[f, pl.ds(4 * DM + t * 256, 256), :]), 0.0)
                  for t in range(DM // 128))
        mem, _ = segment(i * UNROLL + 3, mem, held)
        return tuple(mem), y

    mem0 = tuple(mem_v[:, _tile(t)].astype(F32) for t in range(DM // 128))
    _, y = lax.fori_loop(0, NSEG // UNROLL, trip, (mem0, (zero,) * (DM // 128)))

    r_sel = _row_dot([xsel[:, _tile(t)] for t in range(DM // 128)], wr_v[...].astype(F32))
    y = jnp.concatenate(y, axis=1) * jax.nn.sigmoid(r_sel)
    for i in range(TOPK):
        token = idx_s[i]
        where = (token >> 5, _rows(token & 16, 16), slice(None))
        upd = jnp.where(row16 == (token & 15), y[i:i + 1], 0.0)
        xbuf[where] = (xbuf[where].astype(F32) + upd).astype(BF16)

    def out_copy(n, c):
        sl = (_rows(n * SEG_FIN, SEG_FIN), slice(None), pl.ds(c * 256, 256))
        return pltpu.make_async_copy(xbuf.at[sl], out_hbm.at[sl], sem_out)

    def finish(n, carry):
        ops = oalone.at[:, _rows(n * SEG_FIN * 8, SEG_FIN * 8)]
        xs = xbuf.at[_rows(n * SEG_FIN, SEG_FIN)]
        att = apart.at[_rows(n * SEG_FIN * SEG, SEG_FIN * SEG)]
        gates = gate.at[_rows(n * SEG_FIN * SEG, SEG_FIN * SEG)]
        for c in range(NC):
            for r in range(0, SEG_FIN * 8, ROWS_FIN):
                m1, m6, m7 = [_mm(ops.at[t][pl.ds(r, ROWS_FIN), :], woalone.at[c][:, _tile(t)])
                              for t in range(3)]
                d11, d22 = m1 + m7, m1 + m6
                for i in range(ROWS_FIN // 8):
                    s = r // 8 + i
                    r32 = pl.ds(s * SEG, SEG)
                    g = gates[r32, :]
                    al, ar = att[r32, _tile(2 * c)], att[r32, _tile(2 * c + 1)]
                    al = jnp.concatenate(
                        [al[0:16], al[16:24] + d11[8 * i:8 * i + 8], al[24:32]], axis=0)
                    ar = jnp.concatenate(
                        [ar[0:24], ar[24:32] + d22[8 * i:8 * i + 8]], axis=0)
                    for t, a in ((2 * c, al), (2 * c + 1, ar)):
                        b = xs[s, :, _tile(t)].astype(F32)
                        xs[s, :, _tile(t)] = (g * a + (1.0 - g) * b).astype(BF16)
            out_copy(n, c).start()
        return carry

    lax.fori_loop(0, NSEG // SEG_FIN, finish, 0)
    pltpu.make_async_copy(xbuf, out_hbm, sem_out).wait()


def _by_head_group(w):
    return w.reshape(DM, HEADS // 8, 8, HD).transpose(0, 2, 1, 3).reshape(DM * 8, HEADS // 8 * HD)


@functools.partial(jax.jit, static_argnames=("A_seg_len",))
def pallas_gated_mix__memory_aug_recurrent_mem_tr__moe_arch_mod__prompt_kernel(
    A_x: jax.Array,
    A_mem0: jax.Array,
    A_Wq: jax.Array,
    A_Wk: jax.Array,
    A_Wv: jax.Array,
    A_Wo: jax.Array,
    A_seg_len: int,
    B_x: jax.Array,
    B_w_r: jax.Array,
    B_w_gate: jax.Array,
    B_w_up: jax.Array,
    B_w_down: jax.Array,
    gate_w: jax.Array,
):
    del B_x
    assert A_seg_len == SEG and A_x.shape == (1, SEQ, DM) and A_mem0.shape == (1, MEM, DM)
    assert A_Wq.shape == (DM, HEADS, HD) and B_w_gate.shape == (DM, FF)

    hbm = pl.BlockSpec(memory_space=pl.ANY)
    out = pl.pallas_call(
        _kernel,
        out_shape=jax.ShapeDtypeStruct((NSEG, SEG, DM), BF16),
        in_specs=[hbm] * 11,
        out_specs=hbm,
        scratch_shapes=[
            pltpu.VMEM((NSEG, SEG, DM), BF16),
            pltpu.VMEM((MEM, DM), BF16),
            pltpu.VMEM((8, 128), BF16),
            pltpu.VMEM((8, 128), BF16),
            pltpu.VMEM((3, HEADS // 8, 2048, HD), BF16),
            pltpu.VMEM((HEADS * HD, DM), BF16),
            pltpu.VMEM((NC, SROWS // 2, 3 * 128), U32),
            pltpu.VMEM((3 * NPAIR, 256, 4 * 128), U32),
            pltpu.VMEM((NC, NPAIR * 64, 4 * 128), U32),
            pltpu.VMEM((NC, NPAIR * 64, 3 * 128), U32),
            pltpu.VMEM((3 * NPAIR, SROWS, 2 * 128), F32),
            pltpu.VMEM((4, 16, NC * 128), U32),
            pltpu.VMEM((4, 16, NPAIR * 128), U32),
            pltpu.VMEM((3, SROWS // 2, NPAIR * 128), U32),
            pltpu.VMEM((SEQ, DM), F32),
            pltpu.VMEM((SEQ, 128), F32),
            pltpu.VMEM((NFP, 6 * DM, 128), BF16),
            pltpu.SMEM((TOPK,), I32),
            pltpu.SemaphoreType.DMA((3,)),
            pltpu.SemaphoreType.DMA((NC + 1,)),
            pltpu.SemaphoreType.DMA((8,)),
            pltpu.SemaphoreType.DMA((3,)),
            pltpu.SemaphoreType.DMA((NFP,)),
            pltpu.SemaphoreType.DMA,
        ],
        compiler_params=pltpu.CompilerParams(
            vmem_limit_bytes=126 * 1024 * 1024, disable_bounds_checks=True),
    )(
        A_x.reshape(NSEG, SEG, DM),
        A_mem0.reshape(MEM, DM),
        _by_head_group(A_Wq),
        _by_head_group(A_Wk),
        _by_head_group(A_Wv),
        A_Wo.reshape(HEADS * HD, DM),
        B_w_r.reshape(8, 128),
        B_w_gate,
        B_w_up,
        B_w_down,
        gate_w.reshape(8, 128),
    )
    return out.reshape(1, SEQ, DM)
```

```python
import functools

import jax
import jax.numpy as jnp
import numpy as np
from jax import lax
from jax.experimental import pallas as pl
from jax.experimental.pallas import tpu as pltpu

F32, BF16, U32, I32 = jnp.float32, jnp.bfloat16, jnp.uint32, jnp.int32

SEQ, DM, HEADS, HD = 2048, 1024, 32, 128
MEM, SEG, TOPK, FF = 8, 32, 8, 3584
NSEG = SEQ // SEG
NPAIR = HEADS // 2
NGROUP = HEADS // 8
NC = DM // 256
SROWS = NSEG * 8
ORDER = "kKqQfPpVSsv"
SPLIT = 14
UNROLL_FIN = 0
UNROLL_LAST = 0
EXP2 = 1
LOG2E = 1.4426950408889634
UNROLL = 4
NFP = FF // 256
ROWS_P0 = 64
ROWS_FIN = 64
SEG_FIN = 16


def _mm(a, b):
    return jnp.dot(a, b, preferred_element_type=F32)


def _repeat(n, body, carry, unroll):
    return lax.fori_loop(0, n, body, carry, unroll=bool(unroll))


def _tile(i):
    return slice(i * 128, (i + 1) * 128)


def _rows(start, size):
    if isinstance(start, int):
        return pl.ds(start, size)
    return pl.ds(pl.multiple_of(start, size), size)


def _window(first, count, unit):
    start = first * unit
    return pl.ds(start if isinstance(start, int) else pl.multiple_of(start, unit), count * unit)


def _weight_blocks(b11, b12, b21, b22):
    resident = [b11, b21 - b11, b12 - b22, b22]
    alone = [b11 + b22, b11 + b12, b21 + b22]
    return resident, alone


def _resident_lhs(m1, m2, z1, z2):
    ms, zs = m1 + m2, z1 + z2
    parts = ((ms, zs[24:32], zs[0:16]), (m2, z2[24:32], z2[0:16]),
             (m1, z1[16:24], z1[0:16]), (ms, zs[16:24], zs[0:16]))
    return [jnp.concatenate(p, axis=0).astype(BF16) for p in parts]


def _alone_lhs(a11, a12, a21, a22):
    return [a11 + a22, a21 - a11, a12 - a22]


def _row_dot(x_tiles, w8):
    acc = x_tiles[0] * w8[0:1]
    for t in range(1, len(x_tiles)):
        acc = acc + x_tiles[t] * w8[t:t + 1]
    return jnp.sum(acc, axis=1, keepdims=True)


def _kernel(x_hbm, mem_hbm, wq_hbm, wk_hbm, wv_hbm, wo_hbm, wr_hbm, wg_hbm,
            wu_hbm, wd_hbm, gw_hbm, out_hbm,
            vecs, xbuf, mem_v, stage, wo_raw, xl_u, wres_u, wores_u,
            woalone_u, dbuf, lhs_u, olhs_u, oalone_u, apart, gate, ffw, out_v, chosen,
            sem_w, sem_g, sem_x, sem_o, sem_s, sem_f, sem_out):
    xl = xl_u.bitcast(BF16)
    wres = wres_u.bitcast(BF16)
    wores = wores_u.bitcast(BF16)
    woalone = woalone_u.bitcast(BF16)
    lhs = lhs_u.bitcast(BF16)
    olhs = olhs_u.bitcast(BF16)
    oalone = oalone_u.bitcast(BF16)
    stage32 = stage.bitcast(U32)

    wr_v, gw_v = vecs.at[0:8], vecs.at[16:24]
    zero = jnp.zeros((8, 128), F32)
    lane = lax.broadcasted_iota(I32, (8, 128), 1)
    sub = lax.broadcasted_iota(I32, (8, 128), 0)

    def w_start(w, c, sems=None):
        for g in range(NGROUP):
            pltpu.make_async_copy(
                (wq_hbm, wk_hbm, wv_hbm)[w].at[_rows(c * 2048, 2048), _tile(g)],
                stage.at[w, g], sem_w.at[w] if sems is None else sems.at[g]).start()

    def w_wait(w):
        pltpu.make_async_copy(stage.at[w], stage.at[w], sem_w.at[w]).wait()

    def x_copies(c, rows, sem):
        return [pltpu.make_async_copy(x_hbm.at[:, rows, _tile(t)], xbuf.at[t, :, rows], sem)
                for t in (2 * c, 2 * c + 1)]

    def x_wait(c):
        whole = xbuf.at[_rows(2 * c, 2)]
        pltpu.make_async_copy(whole, whole, sem_x.at[c]).wait()

    def wo_start(p):
        rows = _rows(p * 512, 512)
        for t in range(DM // 128):
            pltpu.make_async_copy(
                wo_hbm.at[rows, _tile(t)], wo_raw.at[t, rows], sem_o.at[p]).start()

    def wo_wait(p):
        piece = wo_raw.at[:, _rows(p * 512, 512)]
        pltpu.make_async_copy(piece, piece, sem_o.at[p]).wait()

    def ff_start(f):
        dst, sem = ffw.at[f % 2], sem_f.at[f % 2]
        for h in range(2):
            cols = _rows(f * 256 + h * 128, 128)
            for n, src in enumerate((wg_hbm, wu_hbm)):
                pltpu.make_async_copy(
                    src.at[:, cols], dst.at[pl.ds((2 * n + h) * DM, DM)], sem).start()
        for t in range(DM // 128):
            pltpu.make_async_copy(wd_hbm.at[_rows(f * 256, 256), _tile(t)],
                                  dst.at[pl.ds(4 * DM + t * 256, 256)], sem).start()

    def ff_wait(f):
        pltpu.make_async_copy(ffw.at[f % 2], ffw.at[f % 2], sem_f.at[f % 2]).wait()

    small = [pltpu.make_async_copy(s, d, sem_s.at[i]) for i, (s, d) in enumerate(
        ((mem_hbm, mem_v), (wr_hbm, wr_v), (gw_hbm, gw_v)))]

    def x_blocks(c, first, count):
        src = xbuf.at[_rows(2 * c, 2), pl.ds(2 * first, 2 * count)]
        dst = xl.at[c, _window(first, count, 16)]
        for n in range(count):
            got = []
            for s in (2 * n, 2 * n + 1):
                z1, z2 = [src[h, s, 16:32, :].astype(F32) for h in range(2)]
                got.append(_alone_lhs(z1[0:8], z2[0:8], z1[8:16], z2[8:16]))
            for t in range(3):
                dst[pl.ds(n * 16, 16), _tile(t)] = jnp.concatenate(
                    [got[0][t], got[1][t]], axis=0).astype(BF16)

    def qkv_blocks(raw, res, j):
        raw = raw.at[j // 4]
        even = lambda z: pltpu.bitcast(z << 16, F32)
        odd = lambda z: pltpu.bitcast(z & np.uint32(0xFFFF0000), F32)
        rest = []
        for r in range(112, -16, -16):
            h1 = raw[pl.ds(4 * r + j % 4, 16, stride=4), :]
            h2 = raw[pl.ds(4 * (128 + r) + j % 4, 16, stride=4), :]
            resident, alone = _weight_blocks(even(h1), odd(h1), even(h2), odd(h2))
            res.at[j][pl.ds(r, 16), :] = jnp.concatenate(resident, axis=1).astype(BF16)
            rest.insert(0, alone)
        return tuple(jnp.concatenate(a, axis=0).astype(BF16) for a in zip(*rest))

    def wo_blocks(views, j, c, r, pace):
        raw, res, rest = views
        b11, b12, b21, b22 = [
            raw[2 * c + h, pl.ds(j * 256 + half + r, 16), :].astype(F32)
            for half in (0, 128) for h in range(2)]
        resident, alone = _weight_blocks(pace(b11), b12, b21, b22)
        res.at[c][pl.ds(j * 128 + r, 16), :] = jnp.concatenate(resident, axis=1).astype(BF16)
        rest.at[c][pl.ds(j * 128 + r, 16), :] = jnp.concatenate(alone, axis=1).astype(BF16)

    def router_scores(x_v, s, half, scores, pace):
        xs = [x_v[t, s, 16 * half:16 * half + 16, :].astype(F32) for t in range(DM // 128)]
        r = _row_dot([pace(xs[0])] + xs[1:], wr_v[...].astype(F32))
        for i in range(2):
            scores = jnp.where(lane == 4 * s + 2 * half + i, r[8 * i:8 * i + 8], scores)
        return scores

    def select_tokens(scores):
        keys = []
        for h, r in enumerate(scores):
            r = r.astype(BF16).astype(F32)
            bits = pltpu.bitcast(jnp.where(r == 0.0, 0.0, r), I32) >> 16
            order = jnp.where(r != r, 0, jnp.where(bits < 0, ~bits, bits + 0x8000))
            token = (h * 128 + lane) * 8 + sub
            keys.append(pltpu.bitcast((1 << 29) + (order << 11) + (SEQ - 1 - token), F32))
        words, tiles = xbuf.bitcast(U32), [zero] * (DM // 128)
        for n in range(TOPK):
            top = jnp.max(jnp.maximum(keys[0], keys[1]), axis=0, keepdims=True)
            top = jnp.max(top, axis=1, keepdims=True)
            keys = [jnp.where(k == top, 0.0, k) for k in keys]
            low = pltpu.bitcast(jnp.broadcast_to(top, (8, 128)), I32)[0, 0] & (SEQ - 1)
            token = SEQ - 1 - low
            chosen[n] = token
            for t in range(DM // 128):
                z = words[t, token >> 5, pl.ds((token >> 1) & 15, 1), :]
                z = jnp.broadcast_to(z, (8, 128))
                z = jnp.where((token & 1) == 0, z << 16, z & np.uint32(0xFFFF0000))
                tiles[t] = jnp.where(sub == n, pltpu.bitcast(z, F32), tiles[t])
        r, g = [jax.nn.sigmoid(_row_dot(tiles, v[...].astype(F32))) for v in (wr_v, gw_v)]
        return jnp.concatenate(tiles, axis=1), jnp.broadcast_to(r * (1.0 - g), (8, 128))

    def qkv_chunk(w, c, group, groups, never, extra=None):
        pairs = pl.ds(w * NPAIR + 4 * group, 4 * groups)
        raw = stage32.at[w, pl.ds(group, groups)]
        res, sums = wres.at[pairs, _rows(c * 128, 128)], dbuf.at[pairs]
        alone = qkv_blocks(raw, res, 0)
        for j in range(4 * groups):
            ahead = qkv_blocks(raw, res, j + 1) if j + 1 < 4 * groups else None
            for r in range(0, SROWS, ROWS_P0):
                rows = pl.ds(r, ROWS_P0)
                ops = [xl.at[c][rows, _tile(t)] for t in range(3)]
                if ahead is not None:
                    n = 128 - 16 * min((r + ROWS_P0) * 8 // SROWS + 1, 8)
                    ops[0] = jnp.concatenate(
                        [jnp.where(never, ahead[0][n:n + 16], ops[0][:16]), ops[0][16:]], axis=0)
                m1, m6, m7 = [_mm(ops[t], alone[t]) for t in range(3)]
                for t, d in enumerate((m1 + m7, m1 + m6)):
                    if not isinstance(c, int):
                        d = d + jnp.where(c > 0, sums[j, rows, _tile(t)], 0.0)
                    elif c > 0:
                        d = d + sums[j, rows, _tile(t)]
                    sums[j, rows, _tile(t)] = d
                if extra is not None:
                    extra((j * SROWS + r) // ROWS_P0, m1)
            alone = ahead

    x_first = x_copies(0, pl.ds(16, 16), sem_x.at[0])
    x_rest = x_copies(0, pl.ds(0, 16), sem_x.at[NC])
    for cp in x_first:
        cp.start()
    w_start(0, 0, sem_g)
    w_start(1, 0)
    for cp in x_copies(1, slice(None), sem_x.at[1]):
        cp.start()
    w_start(2, 0)
    for cp in x_rest + small:
        cp.start()
    for cp in x_first:
        cp.wait()
    x_blocks(0, 0, NSEG // 2)

    def first(g, carry):
        pltpu.make_async_copy(stage.at[0, g], stage.at[0, g], sem_g.at[g]).wait()
        qkv_chunk(0, 0, g, 1, g < 0)
        return carry

    lax.fori_loop(0, NGROUP, first, 0)
    w_start(0, 1)

    def early(i, carry):
        c, w = i // 3, i % 3
        w_wait(w)

        @pl.when(w == 1)
        def _():
            x_wait(c + 1)

        qkv_chunk(w, c, 0, NGROUP, i < 0)
        x_blocks(jnp.where(w == 0, c, c + 1), jnp.where(w == 2, NSEG // 4, 0), NSEG // 4)
        for n in range(3):
            @pl.when(w == n)
            def _():
                w_start(n, c + 1)

        for n in (2, 3):
            @pl.when(i == 3 * n - 5)
            def _():
                for cp in x_copies(n, slice(None), sem_x.at[n]):
                    cp.start()

        wo_start(i - 1)
        return carry

    lax.fori_loop(1, 3 * (NC - 1), early, 0)

    for cp in x_rest + small:
        cp.wait()
    ff_start(0)

    def last(w, carry):
        scores, fresh = carry[0], [zero]
        w_wait(w)
        for n in range(3):
            @pl.when(3 * w + n < 8)
            def _():
                wo_wait(jnp.minimum(3 * w + n, 7))

        j0 = jnp.minimum(6 * w, NPAIR - 6)
        x_v = xbuf.at[:, _rows(jnp.minimum(w, 1) * (NSEG // 2), NSEG // 2)]
        wo_todo = [(j, c, r) for j in range(6) for c in range(NC) for r in range(0, 128, 16)]
        slots = (NPAIR * SROWS - 128) // ROWS_P0
        views = (wo_raw.at[:, _window(j0, 6, 256)], wores.at[:, _window(j0, 6, 128)],
                 woalone.at[:, _window(j0, 6, 128)])

        def extra(n, m):
            pace = lambda z: jnp.where(w < 0, m[:z.shape[0]], z)
            for item in wo_todo[len(wo_todo) * n // slots:len(wo_todo) * (n + 1) // slots]:
                wo_blocks(views, *item, pace)
            for g in range(NSEG * n // slots, min(NSEG * (n + 1) // slots, NSEG)):
                fresh[0] = router_scores(x_v, g // 2, g % 2, fresh[0], pace)

        picked = select_tokens(scores)
        qkv_chunk(w, NC - 1, 0, NGROUP, w < 0, extra)
        return (jnp.where(w == 0, fresh[0], scores[0]), fresh[0]), picked

    _, (xsel, weight) = _repeat(
        3, last, ((zero, zero), (jnp.zeros((8, DM), F32), zero)), UNROLL_LAST)

    qi = lax.broadcasted_iota(I32, (MEM + SEG, MEM + SEG), 0)
    ki = lax.broadcasted_iota(I32, (MEM + SEG, MEM + SEG), 1)
    visible = (qi < MEM) | (qi >= ki)

    def attend(q, k):
        sc = lax.dot_general(q, k, (((1,), (1,)), ((), ())), preferred_element_type=F32)
        if EXP2:
            sc = jnp.where(visible, sc * (HD ** -0.5 * LOG2E), -1000000000.0 * LOG2E)
            e = jnp.exp2(sc - jnp.max(sc, axis=1, keepdims=True))
        else:
            sc = jnp.where(visible, sc * HD ** -0.5, -1000000000.0)
            e = jnp.exp(sc - jnp.max(sc, axis=1, keepdims=True))
        total = jnp.sum(e, axis=1, keepdims=True)
        inv = pltpu.reciprocal(total, approx=True)
        return e, inv * (2.0 - total * inv)

    def segment(views, s, mem, held, filler, never):
        x_v, sums, ops_out, mix, gates = views
        r8, r32 = pl.ds(s * 8, 8), pl.ds(s * SEG, SEG)
        xs = [jnp.where(never, 1.0, x_v[t, s].astype(F32)) for t in range(DM // 128)]
        for c in range(NC):
            ops = _resident_lhs(mem[2 * c], mem[2 * c + 1], xs[2 * c], xs[2 * c + 1])
            for t in range(4):
                lhs.at[t][:, _tile(c)] = ops[t]
        g = jnp.broadcast_to(jax.nn.sigmoid(_row_dot(xs, gw_v[...].astype(F32))), (SEG, 128))
        gates[pl.ds(s * 16, 16), :] = g[16:32]

        def products(w, j, k):
            return [_mm(lhs.at[t][:, k], wres.at[w * NPAIR + j][k, _tile(t)]) for t in range(4)]

        def project(w, j, head=None):
            u = w * NPAIR + j
            if head is None:
                m2, m4, m3, m5 = products(w, j, slice(0, NC * 128))
            else:
                m2, m4, m3, m5 = [b + a for a, b in zip(head, products(w, j, _tile(NC - 1)))]
            left, right = m2 + m4, m3 + m5
            c11 = m4[8:16] - m5[8:16] + sums[u, r8, _tile(0)]
            c22 = m3[8:16] - m2[8:16] + sums[u, r8, _tile(1)]
            return (jnp.concatenate([left[0:8], left[16:32], c11, left[8:16]], axis=0),
                    jnp.concatenate([right[0:8], right[16:32], right[8:16], c22], axis=0))

        keep = {}

        def values(j, p, v):
            oe, oo = [_mm(e, vh) * inv for (e, inv), vh in zip(p, v)]
            ops = _resident_lhs(oe[0:8], oo[0:8], oe[8:40], oo[8:40])
            for t in range(4):
                olhs.at[t][:, _tile(j)] = ops[t]
            alone = _alone_lhs(oe[24:32], oo[24:32], oe[32:40], oo[32:40])
            if held is None:
                keep[j] = alone
            else:
                for t in range(3):
                    ops_out.at[t][pl.ds((s - 1) * 8, 16), _tile(j)] = jnp.concatenate(
                        [held[j][t], alone[t]], axis=0).astype(BF16)

        def out_proj(c, j0, j1):
            k = slice(j0 * 128, j1 * 128)
            return [_mm(olhs.at[t][:, k], wores.at[c][k, _tile(t)]) for t in range(4)]

        new_mem = [None] * (2 * NC)

        def out_done(c, ms):
            m2, m4, m3, m5 = ms
            left, right = m2 + m4, m3 + m5
            new_mem[2 * c], new_mem[2 * c + 1] = left[0:8], right[0:8]
            parts = ((left[16:32], m4[8:16] - m5[8:16], left[8:16]),
                     (right[16:32], right[8:16], m3[8:16] - m2[8:16]))
            for t, a in zip((2 * c, 2 * c + 1), parts):
                mix[r32, _tile(t)] = (g * jnp.concatenate(a, axis=0)
                                      + (1.0 - g) * x_v[t, s].astype(F32))

        first = [("qkv".index(op.lower()), int(op.isupper()))
                 for op in ORDER if op in "qkvQKV"][:2]
        heads = {wj: products(*wj, slice(0, (NC - 1) * 128)) for wj in first}
        got = {}
        for pair in range(0, NPAIR, 2):
            for op in ORDER:
                j = pair + op.isupper()
                if op in "qkvQKV":
                    w = "qkv".index(op.lower())
                    got[w, j] = project(w, j, heads.get((w, j)))
                elif op in "sS":
                    got["p", j] = [attend(q, k) for q, k in zip(got[0, j], got[1, j])]
                elif op in "pP" and pair > 0:
                    values(j - 2, got["p", j - 2], got[2, j - 2])
                elif op == "f" and pair > 0:
                    filler(pair // 2)
        split = SPLIT
        head0 = out_proj(0, 0, split)
        for j in (NPAIR - 2, NPAIR - 1):
            values(j, got["p", j], got[2, j])
        head1 = out_proj(1, 0, split)
        for c, head in enumerate((head0, head1)):
            out_done(c, [tail + h for tail, h in zip(out_proj(c, split, NPAIR), head)])
        for c in range(2, NC):
            out_done(c, out_proj(c, 0, NPAIR))
        return new_mem, keep or None

    def trip(i, carry):
        mem, y = list(carry[0]), list(carry[1])

        f = jnp.minimum(i, NFP - 1)

        @pl.when(i < NFP)
        def _():
            ff_wait(f)

        @pl.when(i + 1 < NFP)
        def _():
            ff_start(jnp.minimum(i + 1, NFP - 1))

        weights, hidden = ffw.at[f % 2], {}

        def ff_in(m):
            def fill(n):
                if n <= 4:
                    u, k = 2 * m + (n - 1) // 2, (n - 1) % 2 * 512
                    part = _mm(xsel[:, k:k + 512], weights[pl.ds(u * DM + k, 512), :])
                    hidden[u] = part if k == 0 else part + hidden[u]
            return fill

        def ff_out(n):
            if n <= 4:
                act = jnp.concatenate(
                    [jax.nn.silu(hidden[h]) * hidden[2 + h] for h in range(2)], axis=1)
                for t in (2 * n - 2, 2 * n - 1):
                    part = _mm(act, weights[pl.ds(4 * DM + t * 256, 256), :])
                    y[t] = y[t] + jnp.where(i < NFP, part, 0.0)

        views = (xbuf.at[:, _rows(i * UNROLL, UNROLL)], dbuf.at[:, _rows(i * UNROLL * 8, UNROLL * 8)],
                 oalone.at[:, _rows(i * UNROLL * 8, UNROLL * 8)],
                 apart.at[_rows(i * UNROLL * SEG, UNROLL * SEG)],
                 gate.at[_rows(i * UNROLL * 16, UNROLL * 16)])
        held = None
        for s, fill in enumerate((lambda n: None, ff_in(0), ff_in(1), ff_out)):
            mem, held = segment(views, s, mem, held, fill, i < 0)
        return tuple(mem), tuple(y)

    mem0 = tuple(mem_v[:, _tile(t)].astype(F32) for t in range(DM // 128))
    _, y = lax.fori_loop(0, NSEG // UNROLL, trip, (mem0, (zero,) * (DM // 128)))
    y = jnp.concatenate([part * weight for part in y], axis=1)
    for n in range(TOPK):
        apart[pl.ds(chosen[n], 1), :] += y[n:n + 1]

    def finish(n, carry):
        ops = oalone.at[:, _rows(n * SEG_FIN * 8, SEG_FIN * 8)]
        mix = apart.at[_rows(n * SEG_FIN * SEG, SEG_FIN * SEG)]
        gates = gate.at[_rows(n * SEG_FIN * 16, SEG_FIN * 16)]
        outs = out_v.at[_rows(n * SEG_FIN * SEG, SEG_FIN * SEG)]
        done = []
        for c in range(NC):
            for r in range(0, SEG_FIN * 8, ROWS_FIN):
                left = [ops.at[t][pl.ds(r, ROWS_FIN), :] for t in range(3)]
                if done:
                    late = jnp.concatenate(done[::len(done) // (2 * NPAIR)], axis=1)
                    for t, part in ((2, late[:, :NPAIR * 128]), (1, late[:, NPAIR * 128:])):
                        left[t] = jnp.concatenate(
                            [jnp.where(n < 0, part, left[t][:16]), left[t][16:]], axis=0)
                done = []
                m1, m7, m6 = [_mm(left[t], woalone.at[c][:, _tile(t)]) for t in (0, 2, 1)]
                d11, d22 = m1 + m7, m1 + m6
                for i in range(ROWS_FIN // 8):
                    s = r // 8 + i
                    r32 = pl.ds(s * SEG, SEG)
                    g = gates[pl.ds(s * 16, 16), :]
                    zl, zr = mix[r32, _tile(2 * c)], mix[r32, _tile(2 * c + 1)]
                    zl = [zl[0:16], zl[16:24] + g[0:8] * d11[8 * i:8 * i + 8], zl[24:32]]
                    zr = [zr[0:24], zr[24:32] + g[8:16] * d22[8 * i:8 * i + 8]]
                    for t, z in ((2 * c, zl), (2 * c + 1, zr)):
                        z = jnp.concatenate(z, axis=0).astype(BF16)
                        outs[r32, _tile(t)] = z
                        done += [z[16:], z[:16]]
                sl = (_window(n * SEG_FIN + r // 8, ROWS_FIN // 8, SEG), pl.ds(c * 256, 256))
                pltpu.make_async_copy(out_v.at[sl], out_hbm.at[sl], sem_out).start()
        return carry

    _repeat(NSEG // SEG_FIN, finish, 0, UNROLL_FIN)
    pltpu.make_async_copy(out_v, out_hbm, sem_out).wait()


def _by_head_group(w):
    return w.reshape(DM, HEADS // 8, 8, HD).transpose(0, 2, 1, 3).reshape(DM * 8, HEADS // 8 * HD)


@functools.partial(jax.jit, static_argnames=("A_seg_len",))
def pallas_gated_mix__memory_aug_recurrent_mem_tr__moe_arch_mod__prompt_kernel(
    A_x: jax.Array,
    A_mem0: jax.Array,
    A_Wq: jax.Array,
    A_Wk: jax.Array,
    A_Wv: jax.Array,
    A_Wo: jax.Array,
    A_seg_len: int,
    B_x: jax.Array,
    B_w_r: jax.Array,
    B_w_gate: jax.Array,
    B_w_up: jax.Array,
    B_w_down: jax.Array,
    gate_w: jax.Array,
):
    del B_x
    assert A_seg_len == SEG and A_x.shape == (1, SEQ, DM) and A_mem0.shape == (1, MEM, DM)
    assert A_Wq.shape == (DM, HEADS, HD) and B_w_gate.shape == (DM, FF)

    hbm = pl.BlockSpec(memory_space=pl.ANY)
    out = pl.pallas_call(
        _kernel,
        out_shape=jax.ShapeDtypeStruct((SEQ, DM), BF16),
        in_specs=[hbm] * 11,
        out_specs=hbm,
        scratch_shapes=[
            pltpu.VMEM((48, 128), BF16),
            pltpu.VMEM((DM // 128, NSEG, SEG, 128), BF16),
            pltpu.VMEM((MEM, DM), BF16),
            pltpu.VMEM((3, HEADS // 8, 2048, HD), BF16),
            pltpu.VMEM((DM // 128, HEADS * HD, 128), BF16),
            pltpu.VMEM((NC, SROWS // 2, 3 * 128), U32),
            pltpu.VMEM((3 * NPAIR, 256, 4 * 128), U32),
            pltpu.VMEM((NC, NPAIR * 64, 4 * 128), U32),
            pltpu.VMEM((NC, NPAIR * 64, 3 * 128), U32),
            pltpu.VMEM((3 * NPAIR, SROWS, 2 * 128), F32),
            pltpu.VMEM((4, 16, NC * 128), U32),
            pltpu.VMEM((4, 16, NPAIR * 128), U32),
            pltpu.VMEM((3, SROWS // 2, NPAIR * 128), U32),
            pltpu.VMEM((SEQ, DM), F32),
            pltpu.VMEM((SEQ // 2, 128), F32),
            pltpu.VMEM((2, 6 * DM, 128), BF16),
            pltpu.VMEM((SEQ, DM), BF16),
            pltpu.SMEM((TOPK,), I32),
            pltpu.SemaphoreType.DMA((3,)),
            pltpu.SemaphoreType.DMA((NGROUP,)),
            pltpu.SemaphoreType.DMA((NC + 1,)),
            pltpu.SemaphoreType.DMA((8,)),
            pltpu.SemaphoreType.DMA((3,)),
            pltpu.SemaphoreType.DMA((2,)),
            pltpu.SemaphoreType.DMA,
        ],
        compiler_params=pltpu.CompilerParams(
            vmem_limit_bytes=126 * 1024 * 1024, disable_bounds_checks=True),
    )(
        A_x.reshape(NSEG, SEG, DM),
        A_mem0.reshape(MEM, DM),
        _by_head_group(A_Wq),
        _by_head_group(A_Wk),
        _by_head_group(A_Wv),
        A_Wo.reshape(HEADS * HD, DM),
        B_w_r.reshape(8, 128),
        B_w_gate,
        B_w_up,
        B_w_down,
        gate_w.reshape(8, 128),
    )
    return out.reshape(1, SEQ, DM)
```

```python
import functools

import jax
import jax.numpy as jnp
import numpy as np
from jax import lax
from jax.experimental import pallas as pl
from jax.experimental.pallas import tpu as pltpu

F32, BF16, U32, I32 = jnp.float32, jnp.bfloat16, jnp.uint32, jnp.int32

SEQ, DM, HEADS, HD = 2048, 1024, 32, 128
MEM, SEG, TOPK, FF = 8, 32, 8, 3584
NSEG = SEQ // SEG
NPAIR = HEADS // 2
NGROUP = HEADS // 8
NC = DM // 256
SROWS = NSEG * 8
ORDER = "kKqQfPpVSsv"
SPLIT = 14
UNROLL_FIN = 0
UNROLL_LAST = 0
EXP2 = 1
LOG2E = 1.4426950408889634
UNROLL = 4
NFP = FF // 256
ROWS_P0 = 64
ROWS_FIN = 64
SEG_FIN = 16


def _mm(a, b):
    return jnp.dot(a, b, preferred_element_type=F32)


def _repeat(n, body, carry, unroll):
    return lax.fori_loop(0, n, body, carry, unroll=bool(unroll))


def _tile(i):
    return slice(i * 128, (i + 1) * 128)


def _rows(start, size):
    if isinstance(start, int):
        return pl.ds(start, size)
    return pl.ds(pl.multiple_of(start, size), size)


def _window(first, count, unit):
    start = first * unit
    return pl.ds(start if isinstance(start, int) else pl.multiple_of(start, unit), count * unit)


def _weight_blocks(b11, b12, b21, b22):
    resident = [b11, b21 - b11, b12 - b22, b22]
    alone = [b11 + b22, b11 + b12, b21 + b22]
    return resident, alone


def _resident_lhs(m1, m2, z1, z2):
    ms, zs = m1 + m2, z1 + z2
    parts = ((ms, zs[24:32], zs[0:16]), (m2, z2[24:32], z2[0:16]),
             (m1, z1[16:24], z1[0:16]), (ms, zs[16:24], zs[0:16]))
    return [jnp.concatenate(p, axis=0).astype(BF16) for p in parts]


def _alone_lhs(a11, a12, a21, a22):
    return [a11 + a22, a21 - a11, a12 - a22]


def _row_dot(x_tiles, w8):
    acc = x_tiles[0] * w8[0:1]
    for t in range(1, len(x_tiles)):
        acc = acc + x_tiles[t] * w8[t:t + 1]
    return jnp.sum(acc, axis=1, keepdims=True)


def _kernel(x_hbm, mem_hbm, wq_hbm, wk_hbm, wv_hbm, wo_hbm, wr_hbm, wg_hbm,
            wu_hbm, wd_hbm, gw_hbm, out_hbm,
            vecs, xbuf, mem_v, stage, wo_raw, xl_u, wres_u, wores_u,
            woalone_u, dbuf, lhs_u, olhs_u, oalone_u, apart, gate, ffw, out_v, chosen,
            sem_w, sem_g, sem_x, sem_o, sem_s, sem_f, sem_out):
    xl = xl_u.bitcast(BF16)
    wres = wres_u.bitcast(BF16)
    wores = wores_u.bitcast(BF16)
    woalone = woalone_u.bitcast(BF16)
    lhs = lhs_u.bitcast(BF16)
    olhs = olhs_u.bitcast(BF16)
    oalone = oalone_u.bitcast(BF16)
    stage32 = stage.bitcast(U32)

    wr_v, gw_v = vecs.at[0:8], vecs.at[16:24]
    zero = jnp.zeros((8, 128), F32)
    lane = lax.broadcasted_iota(I32, (8, 128), 1)
    sub = lax.broadcasted_iota(I32, (8, 128), 0)

    def w_start(w, c, sems=None):
        for g in range(NGROUP):
            pltpu.make_async_copy(
                (wq_hbm, wk_hbm, wv_hbm)[w].at[_rows(c * 2048, 2048), _tile(g)],
                stage.at[w, g], sem_w.at[w] if sems is None else sems.at[g]).start()

    def w_wait(w):
        pltpu.make_async_copy(stage.at[w], stage.at[w], sem_w.at[w]).wait()

    def x_copy(n, segs, rows, cols):
        return pltpu.make_async_copy(
            x_hbm.at[segs, rows, cols], xbuf.at[segs, rows, cols], sem_x.at[n])

    every = slice(None)
    x_first = x_copy(0, every, pl.ds(16, 16), pl.ds(0, 256))
    x_rest = x_copy(1, every, pl.ds(0, 16), pl.ds(0, 256))
    x_second = x_copy(2, every, every, pl.ds(256, 256))

    def x_right(h):
        return x_copy(3 + h, _rows(h * (NSEG // 2), NSEG // 2), every, pl.ds(512, 512))

    def wo_copy(p, pairs=3):
        rows = _window(3 * p, pairs, 256)
        return pltpu.make_async_copy(wo_hbm.at[rows], wo_raw.at[rows], sem_o.at[p])

    def ff_start(f):
        dst, sem = ffw.at[f % 2], sem_f.at[f % 2]
        for h in range(2):
            cols = _rows(f * 256 + h * 128, 128)
            for n, src in enumerate((wg_hbm, wu_hbm)):
                pltpu.make_async_copy(
                    src.at[:, cols], dst.at[pl.ds((2 * n + h) * DM, DM)], sem).start()
        for t in range(DM // 128):
            pltpu.make_async_copy(wd_hbm.at[_rows(f * 256, 256), _tile(t)],
                                  dst.at[pl.ds(4 * DM + t * 256, 256)], sem).start()

    def ff_wait(f):
        pltpu.make_async_copy(ffw.at[f % 2], ffw.at[f % 2], sem_f.at[f % 2]).wait()

    small = [pltpu.make_async_copy(s, d, sem_s.at[i]) for i, (s, d) in enumerate(
        ((mem_hbm, mem_v), (wr_hbm, wr_v), (gw_hbm, gw_v)))]

    def x_blocks(c):
        src, dst = xbuf.at[:, :, _rows(c * 256, 256)], xl.at[c]
        for n in range(NSEG // 2):
            got = []
            for s in (2 * n, 2 * n + 1):
                z1, z2 = [src[s, 16:32, _tile(h)].astype(F32) for h in range(2)]
                got.append(_alone_lhs(z1[0:8], z2[0:8], z1[8:16], z2[8:16]))
            for t in range(3):
                dst[pl.ds(n * 16, 16), _tile(t)] = jnp.concatenate(
                    [got[0][t], got[1][t]], axis=0).astype(BF16)

    def qkv_blocks(raw, res, j):
        raw = raw.at[j // 4]
        even = lambda z: pltpu.bitcast(z << 16, F32)
        odd = lambda z: pltpu.bitcast(z & np.uint32(0xFFFF0000), F32)
        rest = []
        for r in range(112, -16, -16):
            h1 = raw[pl.ds(4 * r + j % 4, 16, stride=4), :]
            h2 = raw[pl.ds(4 * (128 + r) + j % 4, 16, stride=4), :]
            resident, alone = _weight_blocks(even(h1), odd(h1), even(h2), odd(h2))
            res.at[j][pl.ds(r, 16), :] = jnp.concatenate(resident, axis=1).astype(BF16)
            rest.insert(0, alone)
        return tuple(jnp.concatenate(a, axis=0).astype(BF16) for a in zip(*rest))

    def wo_blocks(views, j, c, r, pace):
        raw, res, rest = views
        b11, b12, b21, b22 = [
            raw[pl.ds(j * 256 + half + r, 16), _tile(2 * c + h)].astype(F32)
            for half in (0, 128) for h in range(2)]
        resident, alone = _weight_blocks(pace(b11), b12, b21, b22)
        res.at[c][pl.ds(j * 128 + r, 16), :] = jnp.concatenate(resident, axis=1).astype(BF16)
        rest.at[c][pl.ds(j * 128 + r, 16), :] = jnp.concatenate(alone, axis=1).astype(BF16)

    def router_scores(x_v, s, half, scores, pace):
        xs = [x_v[s, 16 * half:16 * half + 16, _tile(t)].astype(F32) for t in range(DM // 128)]
        r = _row_dot([pace(xs[0])] + xs[1:], wr_v[...].astype(F32))
        for i in range(2):
            scores = jnp.where(lane == 4 * s + 2 * half + i, r[8 * i:8 * i + 8], scores)
        return scores

    def select_tokens(scores):
        keys = []
        for h, r in enumerate(scores):
            r = r.astype(BF16).astype(F32)
            bits = pltpu.bitcast(jnp.where(r == 0.0, 0.0, r), I32) >> 16
            order = jnp.where(r != r, 0, jnp.where(bits < 0, ~bits, bits + 0x8000))
            token = (h * 128 + lane) * 8 + sub
            keys.append(pltpu.bitcast((1 << 29) + (order << 11) + (SEQ - 1 - token), F32))
        tiles = [zero] * (DM // 128)
        for n in range(TOPK):
            top = jnp.max(jnp.maximum(keys[0], keys[1]), axis=0, keepdims=True)
            top = jnp.max(top, axis=1, keepdims=True)
            keys = [jnp.where(k == top, 0.0, k) for k in keys]
            low = pltpu.bitcast(jnp.broadcast_to(top, (8, 128)), I32)[0, 0] & (SEQ - 1)
            token = SEQ - 1 - low
            chosen[n] = token
            rows = xbuf[token >> 5, _rows(token & 24, 8), :].astype(F32)
            rows = pltpu.roll(rows, (n - token) & 7, 0)
            tiles = [jnp.where(sub == n, rows[:, _tile(t)], z) for t, z in enumerate(tiles)]
        r, g = [jax.nn.sigmoid(_row_dot(tiles, v[...].astype(F32))) for v in (wr_v, gw_v)]
        return jnp.concatenate(tiles, axis=1), jnp.broadcast_to(r * (1.0 - g), (8, 128))

    def qkv_chunk(w, c, group, groups, never, extra=None):
        pairs = pl.ds(w * NPAIR + 4 * group, 4 * groups)
        raw = stage32.at[w, pl.ds(group, groups)]
        res, sums = wres.at[pairs, _rows(c * 128, 128)], dbuf.at[pairs]
        alone = qkv_blocks(raw, res, 0)
        for j in range(4 * groups):
            ahead = qkv_blocks(raw, res, j + 1) if j + 1 < 4 * groups else None
            for r in range(0, SROWS, ROWS_P0):
                rows = pl.ds(r, ROWS_P0)
                ops = [xl.at[c][rows, _tile(t)] for t in range(3)]
                if ahead is not None:
                    n = 128 - 16 * min((r + ROWS_P0) * 8 // SROWS + 1, 8)
                    ops[0] = jnp.concatenate(
                        [jnp.where(never, ahead[0][n:n + 16], ops[0][:16]), ops[0][16:]], axis=0)
                m1, m6, m7 = [_mm(ops[t], alone[t]) for t in range(3)]
                for t, d in enumerate((m1 + m7, m1 + m6)):
                    if not isinstance(c, int):
                        d = d + jnp.where(c > 0, sums[j, rows, _tile(t)], 0.0)
                    elif c > 0:
                        d = d + sums[j, rows, _tile(t)]
                    sums[j, rows, _tile(t)] = d
                if extra is not None:
                    extra((j * SROWS + r) // ROWS_P0, m1)
            alone = ahead

    x_first.start()
    w_start(0, 0, sem_g)
    w_start(1, 0)
    w_start(2, 0)
    x_first.wait()
    for cp in [x_second, x_rest] + small:
        cp.start()
    x_blocks(0)

    def first(g, carry):
        pltpu.make_async_copy(stage.at[0, g], stage.at[0, g], sem_g.at[g]).wait()
        qkv_chunk(0, 0, g, 1, g < 0)
        return carry

    lax.fori_loop(0, NGROUP, first, 0)
    w_start(0, 1)

    def early(i, carry):
        c, w = i // 3, i % 3
        w_wait(w)

        @pl.when(i == 3)
        def _():
            x_second.wait()

        @pl.when(i == 6)
        def _():
            x_right(0).wait()
            x_right(1).wait()

        @pl.when((i == 2) | (i == 3))
        def _():
            x_right(jnp.clip(i - 2, 0, 1)).start()

        @pl.when(i >= 4)
        def _():
            wo_copy(jnp.maximum(i - 4, 0)).start()

        @pl.when(w == 0)
        def _():
            x_blocks(c)

        qkv_chunk(w, c, 0, NGROUP, i < 0)
        for n in range(3):
            @pl.when(w == n)
            def _():
                w_start(n, c + 1)

        return carry

    lax.fori_loop(1, 3 * (NC - 1), early, 0)

    for cp in [x_rest, wo_copy(0)] + small:
        cp.wait()
    wo_copy(5, 1).start()
    ff_start(0)
    x_blocks(NC - 1)

    def wo_views(first, pairs):
        return (wo_raw.at[_window(first, pairs, 256)], wores.at[:, _window(first, pairs, 128)],
                woalone.at[:, _window(first, pairs, 128)])

    def last(w, carry):
        scores, fresh = carry[0], [zero]
        w_wait(w)
        wo_copy(jnp.minimum(w + 1, 2) + w).wait()

        @pl.when(w == 1)
        def _():
            wo_copy(2).wait()

        x_v = xbuf.at[_rows(jnp.minimum(w, 1) * (NSEG // 2), NSEG // 2)]
        wo_todo = [(j, c, r) for j in range(5) for c in range(NC) for r in range(0, 128, 16)]
        slots = (NPAIR * SROWS - 128) // ROWS_P0
        views = wo_views(5 * w, 5)

        def extra(n, m):
            pace = lambda z: jnp.where(w < 0, m[:z.shape[0]], z)
            for item in wo_todo[len(wo_todo) * n // slots:len(wo_todo) * (n + 1) // slots]:
                wo_blocks(views, *item, pace)
            for g in range(NSEG * n // slots, min(NSEG * (n + 1) // slots, NSEG)):
                fresh[0] = router_scores(x_v, g // 2, g % 2, fresh[0], pace)

        picked = select_tokens(scores)
        qkv_chunk(w, NC - 1, 0, NGROUP, w < 0, extra)
        return (jnp.where(w == 0, fresh[0], scores[0]), fresh[0]), picked

    _, (xsel, weight) = _repeat(
        3, last, ((zero, zero), (jnp.zeros((8, DM), F32), zero)), UNROLL_LAST)

    wo_copy(5, 1).wait()
    for c in range(NC):
        for r in range(0, 128, 16):
            wo_blocks(wo_views(NPAIR - 1, 1), 0, c, r, lambda z: z)

    qi = lax.broadcasted_iota(I32, (MEM + SEG, MEM + SEG), 0)
    ki = lax.broadcasted_iota(I32, (MEM + SEG, MEM + SEG), 1)
    visible = (qi < MEM) | (qi >= ki)

    def attend(q, k):
        sc = lax.dot_general(q, k, (((1,), (1,)), ((), ())), preferred_element_type=F32)
        if EXP2:
            sc = jnp.where(visible, sc * (HD ** -0.5 * LOG2E), -1000000000.0 * LOG2E)
            e = jnp.exp2(sc - jnp.max(sc, axis=1, keepdims=True))
        else:
            sc = jnp.where(visible, sc * HD ** -0.5, -1000000000.0)
            e = jnp.exp(sc - jnp.max(sc, axis=1, keepdims=True))
        total = jnp.sum(e, axis=1, keepdims=True)
        inv = pltpu.reciprocal(total, approx=True)
        return e, inv * (2.0 - total * inv)

    def segment(views, s, mem, held, filler, never):
        x_v, sums, ops_out, mix, gates = views
        r8, r32 = pl.ds(s * 8, 8), pl.ds(s * SEG, SEG)
        xs = [jnp.where(never, 1.0, x_v[s, :, _tile(t)].astype(F32)) for t in range(DM // 128)]
        for c in range(NC):
            ops = _resident_lhs(mem[2 * c], mem[2 * c + 1], xs[2 * c], xs[2 * c + 1])
            for t in range(4):
                lhs.at[t][:, _tile(c)] = ops[t]
        g = jnp.broadcast_to(jax.nn.sigmoid(_row_dot(xs, gw_v[...].astype(F32))), (SEG, 128))
        gates[pl.ds(s * 16, 16), :] = g[16:32]

        def products(w, j, k):
            return [_mm(lhs.at[t][:, k], wres.at[w * NPAIR + j][k, _tile(t)]) for t in range(4)]

        def project(w, j, head=None):
            u = w * NPAIR + j
            if head is None:
                m2, m4, m3, m5 = products(w, j, slice(0, NC * 128))
            else:
                m2, m4, m3, m5 = [b + a for a, b in zip(head, products(w, j, _tile(NC - 1)))]
            left, right = m2 + m4, m3 + m5
            c11 = m4[8:16] - m5[8:16] + sums[u, r8, _tile(0)]
            c22 = m3[8:16] - m2[8:16] + sums[u, r8, _tile(1)]
            return (jnp.concatenate([left[0:8], left[16:32], c11, left[8:16]], axis=0),
                    jnp.concatenate([right[0:8], right[16:32], right[8:16], c22], axis=0))

        keep = {}

        def values(j, p, v):
            oe, oo = [_mm(e, vh) * inv for (e, inv), vh in zip(p, v)]
            ops = _resident_lhs(oe[0:8], oo[0:8], oe[8:40], oo[8:40])
            for t in range(4):
                olhs.at[t][:, _tile(j)] = ops[t]
            alone = _alone_lhs(oe[24:32], oo[24:32], oe[32:40], oo[32:40])
            if held is None:
                keep[j] = alone
            else:
                for t in range(3):
                    ops_out.at[t][pl.ds((s - 1) * 8, 16), _tile(j)] = jnp.concatenate(
                        [held[j][t], alone[t]], axis=0).astype(BF16)

        def out_proj(c, j0, j1):
            k = slice(j0 * 128, j1 * 128)
            return [_mm(olhs.at[t][:, k], wores.at[c][k, _tile(t)]) for t in range(4)]

        new_mem = [None] * (2 * NC)

        def out_done(c, ms):
            m2, m4, m3, m5 = ms
            left, right = m2 + m4, m3 + m5
            new_mem[2 * c], new_mem[2 * c + 1] = left[0:8], right[0:8]
            parts = ((left[16:32], m4[8:16] - m5[8:16], left[8:16]),
                     (right[16:32], right[8:16], m3[8:16] - m2[8:16]))
            for t, a in zip((2 * c, 2 * c + 1), parts):
                mix[r32, _tile(t)] = (g * jnp.concatenate(a, axis=0)
                                      + (1.0 - g) * x_v[s, :, _tile(t)].astype(F32))

        first = [("qkv".index(op.lower()), int(op.isupper()))
                 for op in ORDER if op in "qkvQKV"][:2]
        heads = {wj: products(*wj, slice(0, (NC - 1) * 128)) for wj in first}
        got = {}
        for pair in range(0, NPAIR, 2):
            for op in ORDER:
                j = pair + op.isupper()
                if op in "qkvQKV":
                    w = "qkv".index(op.lower())
                    got[w, j] = project(w, j, heads.get((w, j)))
                elif op in "sS":
                    got["p", j] = [attend(q, k) for q, k in zip(got[0, j], got[1, j])]
                elif op in "pP" and pair > 0:
                    values(j - 2, got["p", j - 2], got[2, j - 2])
                elif op == "f" and pair > 0:
                    filler(pair // 2)
        split = SPLIT
        head0 = out_proj(0, 0, split)
        for j in (NPAIR - 2, NPAIR - 1):
            values(j, got["p", j], got[2, j])
        head1 = out_proj(1, 0, split)
        for c, head in enumerate((head0, head1)):
            out_done(c, [tail + h for tail, h in zip(out_proj(c, split, NPAIR), head)])
        for c in range(2, NC):
            out_done(c, out_proj(c, 0, NPAIR))
        return new_mem, keep or None

    def trip(i, carry):
        mem, y = list(carry[0]), list(carry[1])

        f = jnp.minimum(i, NFP - 1)

        @pl.when(i < NFP)
        def _():
            ff_wait(f)

        @pl.when(i + 1 < NFP)
        def _():
            ff_start(jnp.minimum(i + 1, NFP - 1))

        weights, hidden = ffw.at[f % 2], {}

        def ff_in(m):
            def fill(n):
                if n <= 4:
                    u, k = 2 * m + (n - 1) // 2, (n - 1) % 2 * 512
                    part = _mm(xsel[:, k:k + 512], weights[pl.ds(u * DM + k, 512), :])
                    hidden[u] = part if k == 0 else part + hidden[u]
            return fill

        def ff_out(n):
            if n <= 4:
                act = jnp.concatenate(
                    [jax.nn.silu(hidden[h]) * hidden[2 + h] for h in range(2)], axis=1)
                for t in (2 * n - 2, 2 * n - 1):
                    part = _mm(act, weights[pl.ds(4 * DM + t * 256, 256), :])
                    y[t] = y[t] + jnp.where(i < NFP, part, 0.0)

        views = (xbuf.at[_rows(i * UNROLL, UNROLL)], dbuf.at[:, _rows(i * UNROLL * 8, UNROLL * 8)],
                 oalone.at[:, _rows(i * UNROLL * 8, UNROLL * 8)],
                 apart.at[_rows(i * UNROLL * SEG, UNROLL * SEG)],
                 gate.at[_rows(i * UNROLL * 16, UNROLL * 16)])
        held = None
        for s, fill in enumerate((lambda n: None, ff_in(0), ff_in(1), ff_out)):
            mem, held = segment(views, s, mem, held, fill, i < 0)
        return tuple(mem), tuple(y)

    mem0 = tuple(mem_v[:, _tile(t)].astype(F32) for t in range(DM // 128))
    _, y = lax.fori_loop(0, NSEG // UNROLL, trip, (mem0, (zero,) * (DM // 128)))
    y = jnp.concatenate([part * weight for part in y], axis=1)
    for n in range(TOPK):
        apart[pl.ds(chosen[n], 1), :] += y[n:n + 1]

    def finish(n, carry):
        ops = oalone.at[:, _rows(n * SEG_FIN * 8, SEG_FIN * 8)]
        mix = apart.at[_rows(n * SEG_FIN * SEG, SEG_FIN * SEG)]
        gates = gate.at[_rows(n * SEG_FIN * 16, SEG_FIN * 16)]
        outs = out_v.at[_rows(n * SEG_FIN * SEG, SEG_FIN * SEG)]
        done = []
        for c in range(NC):
            for r in range(0, SEG_FIN * 8, ROWS_FIN):
                left = [ops.at[t][pl.ds(r, ROWS_FIN), :] for t in range(3)]
                if done:
                    late = jnp.concatenate(done[::len(done) // (2 * NPAIR)], axis=1)
                    for t, part in ((2, late[:, :NPAIR * 128]), (1, late[:, NPAIR * 128:])):
                        left[t] = jnp.concatenate(
                            [jnp.where(n < 0, part, left[t][:16]), left[t][16:]], axis=0)
                done = []
                m1, m7, m6 = [_mm(left[t], woalone.at[c][:, _tile(t)]) for t in (0, 2, 1)]
                d11, d22 = m1 + m7, m1 + m6
                for i in range(ROWS_FIN // 8):
                    s = r // 8 + i
                    r32 = pl.ds(s * SEG, SEG)
                    g = gates[pl.ds(s * 16, 16), :]
                    zl, zr = mix[r32, _tile(2 * c)], mix[r32, _tile(2 * c + 1)]
                    zl = [zl[0:16], zl[16:24] + g[0:8] * d11[8 * i:8 * i + 8], zl[24:32]]
                    zr = [zr[0:24], zr[24:32] + g[8:16] * d22[8 * i:8 * i + 8]]
                    for t, z in ((2 * c, zl), (2 * c + 1, zr)):
                        z = jnp.concatenate(z, axis=0).astype(BF16)
                        outs[r32, _tile(t)] = z
                        done += [z[16:], z[:16]]
                sl = (_window(n * SEG_FIN + r // 8, ROWS_FIN // 8, SEG), pl.ds(c * 256, 256))
                pltpu.make_async_copy(out_v.at[sl], out_hbm.at[sl], sem_out).start()
        return carry

    _repeat(NSEG // SEG_FIN, finish, 0, UNROLL_FIN)
    pltpu.make_async_copy(out_v, out_hbm, sem_out).wait()


def _by_head_group(w):
    return w.reshape(DM, HEADS // 8, 8, HD).transpose(0, 2, 1, 3).reshape(DM * 8, HEADS // 8 * HD)


@functools.partial(jax.jit, static_argnames=("A_seg_len",))
def pallas_gated_mix__memory_aug_recurrent_mem_tr__moe_arch_mod__prompt_kernel(
    A_x: jax.Array,
    A_mem0: jax.Array,
    A_Wq: jax.Array,
    A_Wk: jax.Array,
    A_Wv: jax.Array,
    A_Wo: jax.Array,
    A_seg_len: int,
    B_x: jax.Array,
    B_w_r: jax.Array,
    B_w_gate: jax.Array,
    B_w_up: jax.Array,
    B_w_down: jax.Array,
    gate_w: jax.Array,
):
    del B_x
    assert A_seg_len == SEG and A_x.shape == (1, SEQ, DM) and A_mem0.shape == (1, MEM, DM)
    assert A_Wq.shape == (DM, HEADS, HD) and B_w_gate.shape == (DM, FF)

    hbm = pl.BlockSpec(memory_space=pl.ANY)
    out = pl.pallas_call(
        _kernel,
        out_shape=jax.ShapeDtypeStruct((SEQ, DM), BF16),
        in_specs=[hbm] * 11,
        out_specs=hbm,
        scratch_shapes=[
            pltpu.VMEM((48, 128), BF16),
            pltpu.VMEM((NSEG, SEG, DM), BF16),
            pltpu.VMEM((MEM, DM), BF16),
            pltpu.VMEM((3, HEADS // 8, 2048, HD), BF16),
            pltpu.VMEM((HEADS * HD, DM), BF16),
            pltpu.VMEM((NC, SROWS // 2, 3 * 128), U32),
            pltpu.VMEM((3 * NPAIR, 256, 4 * 128), U32),
            pltpu.VMEM((NC, NPAIR * 64, 4 * 128), U32),
            pltpu.VMEM((NC, NPAIR * 64, 3 * 128), U32),
            pltpu.VMEM((3 * NPAIR, SROWS, 2 * 128), F32),
            pltpu.VMEM((4, 16, NC * 128), U32),
            pltpu.VMEM((4, 16, NPAIR * 128), U32),
            pltpu.VMEM((3, SROWS // 2, NPAIR * 128), U32),
            pltpu.VMEM((SEQ, DM), F32),
            pltpu.VMEM((SEQ // 2, 128), F32),
            pltpu.VMEM((2, 6 * DM, 128), BF16),
            pltpu.VMEM((SEQ, DM), BF16),
            pltpu.SMEM((TOPK,), I32),
            pltpu.SemaphoreType.DMA((3,)),
            pltpu.SemaphoreType.DMA((NGROUP,)),
            pltpu.SemaphoreType.DMA((NC + 1,)),
            pltpu.SemaphoreType.DMA((6,)),
            pltpu.SemaphoreType.DMA((3,)),
            pltpu.SemaphoreType.DMA((2,)),
            pltpu.SemaphoreType.DMA,
        ],
        compiler_params=pltpu.CompilerParams(
            vmem_limit_bytes=126 * 1024 * 1024, disable_bounds_checks=True),
    )(
        A_x.reshape(NSEG, SEG, DM),
        A_mem0.reshape(MEM, DM),
        _by_head_group(A_Wq),
        _by_head_group(A_Wk),
        _by_head_group(A_Wv),
        A_Wo.reshape(HEADS * HD, DM),
        B_w_r.reshape(8, 128),
        B_w_gate,
        B_w_up,
        B_w_down,
        gate_w.reshape(8, 128),
    )
    return out.reshape(1, SEQ, DM)
```

```python
import functools

import jax
import jax.numpy as jnp
import numpy as np
from jax import lax
from jax.experimental import pallas as pl
from jax.experimental.pallas import tpu as pltpu

F32, BF16, U32, I32 = jnp.float32, jnp.bfloat16, jnp.uint32, jnp.int32

SEQ, DM, HEADS, HD = 2048, 1024, 32, 128
MEM, SEG, TOPK, FF = 8, 32, 8, 3584
NSEG = SEQ // SEG
NPAIR = HEADS // 2
NGROUP = HEADS // 8
NC = DM // 256
SROWS = NSEG * 8
ORDER = "kKqQfPpVSsv"
SPLIT = 14
PACE = 4
PER = 3
NORM = 1
KV16 = 6
SLOTS = (2,3,5,6)
FLAGS = None
UNROLL_FIN = 0
UNROLL_LAST = 0
EXP2 = 1
LOG2E = 1.4426950408889634
UNROLL = 4
NFP = FF // 256
ROWS_P0 = 64
ROWS_FIN = 64
SEG_FIN = 32


def _mm(a, b):
    return jnp.dot(a, b, preferred_element_type=F32)


def _repeat(n, body, carry, unroll):
    return lax.fori_loop(0, n, body, carry, unroll=bool(unroll))


def _tile(i):
    return slice(i * 128, (i + 1) * 128)


def _rows(start, size):
    if isinstance(start, int):
        return pl.ds(start, size)
    return pl.ds(pl.multiple_of(start, size), size)


def _window(first, count, unit):
    start = first * unit
    return pl.ds(start if isinstance(start, int) else pl.multiple_of(start, unit), count * unit)


def _weight_blocks(b11, b12, b21, b22):
    resident = [b11, b21 - b11, b12 - b22, b22]
    alone = [b11 + b22, b11 + b12, b21 + b22]
    return resident, alone


def _resident_lhs(m1, m2, z1, z2):
    ms, zs = m1 + m2, z1 + z2
    parts = ((ms, zs[24:32], zs[0:16]), (m2, z2[24:32], z2[0:16]),
             (m1, z1[16:24], z1[0:16]), (ms, zs[16:24], zs[0:16]))
    return [jnp.concatenate(p, axis=0).astype(BF16) for p in parts]


def _alone_lhs(a11, a12, a21, a22):
    return [a11 + a22, a21 - a11, a12 - a22]


def _row_dot(x_tiles, w8):
    acc = x_tiles[0] * w8[0:1]
    for t in range(1, len(x_tiles)):
        acc = acc + x_tiles[t] * w8[t:t + 1]
    return jnp.sum(acc, axis=1, keepdims=True)


def _kernel(x_hbm, mem_hbm, wq_hbm, wk_hbm, wv_hbm, wo_hbm, wr_hbm, wg_hbm,
            wu_hbm, wd_hbm, gw_hbm, out_hbm,
            vecs, xbuf, mem_v, stage, wo_raw, xl_u, wres_u, wores_u,
            woalone_u, dbuf, lhs_u, olhs_u, oalone_u, apart, gate, ffw, out_v, chosen,
            sem_w, sem_g, sem_x, sem_o, sem_s, sem_f, sem_out):
    xl = xl_u.bitcast(BF16)
    wres = wres_u.bitcast(BF16)
    wores = wores_u.bitcast(BF16)
    woalone = woalone_u.bitcast(BF16)
    lhs = lhs_u.bitcast(BF16)
    olhs = olhs_u.bitcast(BF16)
    oalone = oalone_u.bitcast(BF16)
    stage32 = stage.bitcast(U32)

    wr_v, gw_v = vecs.at[0:8], vecs.at[16:24]
    zero = jnp.zeros((8, 128), F32)
    lane = lax.broadcasted_iota(I32, (8, 128), 1)
    sub = lax.broadcasted_iota(I32, (8, 128), 0)

    def w_start(w, c, sems=None):
        for g in range(NGROUP):
            pltpu.make_async_copy(
                (wq_hbm, wk_hbm, wv_hbm)[w].at[_rows(c * 2048, 2048), _tile(g)],
                stage.at[w, g], sem_w.at[w] if sems is None else sems.at[g]).start()

    def w_wait(w):
        pltpu.make_async_copy(stage.at[w], stage.at[w], sem_w.at[w]).wait()

    def x_copy(n, segs, rows, cols):
        return pltpu.make_async_copy(
            x_hbm.at[segs, rows, cols], xbuf.at[segs, rows, cols], sem_x.at[n])

    every = slice(None)
    x_first = x_copy(0, every, pl.ds(16, 16), pl.ds(0, 256))
    x_rest = x_copy(1, every, pl.ds(0, 16), pl.ds(0, 256))
    x_second = x_copy(2, every, every, pl.ds(256, 256))

    def x_right(h):
        return x_copy(3 + h, _rows(h * (NSEG // 2), NSEG // 2), every, pl.ds(512, 512))

    def wo_copy(p, pairs=3):
        rows = _window(3 * p, pairs, 256)
        return pltpu.make_async_copy(wo_hbm.at[rows], wo_raw.at[rows], sem_o.at[p])

    def ff_start(f):
        dst, sem = ffw.at[f & 1], sem_f.at[f & 1]
        for h in range(2):
            cols = _rows(f * 256 + h * 128, 128)
            for n, src in enumerate((wg_hbm, wu_hbm)):
                pltpu.make_async_copy(
                    src.at[:, cols], dst.at[pl.ds((2 * n + h) * DM, DM)], sem).start()
        for t in range(DM // 128):
            pltpu.make_async_copy(wd_hbm.at[_rows(f * 256, 256), _tile(t)],
                                  dst.at[pl.ds(4 * DM + t * 256, 256)], sem).start()

    def ff_wait(f):
        pltpu.make_async_copy(ffw.at[f & 1], ffw.at[f & 1], sem_f.at[f & 1]).wait()

    small = [pltpu.make_async_copy(s, d, sem_s.at[i]) for i, (s, d) in enumerate(
        ((mem_hbm, mem_v), (wr_hbm, wr_v), (gw_hbm, gw_v)))]

    def x_blocks(c):
        src, dst = xbuf.at[:, :, _rows(c * 256, 256)], xl.at[c]
        for n in range(NSEG // 2):
            got = []
            for s in (2 * n, 2 * n + 1):
                z1, z2 = [src[s, 16:32, _tile(h)].astype(F32) for h in range(2)]
                got.append(_alone_lhs(z1[0:8], z2[0:8], z1[8:16], z2[8:16]))
            for t in range(3):
                dst[pl.ds(n * 16, 16), _tile(t)] = jnp.concatenate(
                    [got[0][t], got[1][t]], axis=0).astype(BF16)

    def qkv_blocks(raw, res, j):
        raw = raw.at[j // 4]
        even = lambda z: pltpu.bitcast(z << 16, F32)
        odd = lambda z: pltpu.bitcast(z & np.uint32(0xFFFF0000), F32)
        rest = []
        for r in range(112, -16, -16):
            h1 = raw[pl.ds(4 * r + j % 4, 16, stride=4), :]
            h2 = raw[pl.ds(4 * (128 + r) + j % 4, 16, stride=4), :]
            resident, alone = _weight_blocks(even(h1), odd(h1), even(h2), odd(h2))
            res.at[j][pl.ds(r, 16), :] = jnp.concatenate(resident, axis=1).astype(BF16)
            rest.insert(0, alone)
        return tuple(jnp.concatenate(a, axis=0).astype(BF16) for a in zip(*rest))

    def wo_blocks(views, j, c, r, pace):
        raw, res, rest = views
        b11, b12, b21, b22 = [
            raw[pl.ds(j * 256 + half + r, 16), _tile(2 * c + h)].astype(F32)
            for half in (0, 128) for h in range(2)]
        resident, alone = _weight_blocks(pace(b11), b12, b21, b22)
        res.at[c][pl.ds(j * 128 + r, 16), :] = jnp.concatenate(resident, axis=1).astype(BF16)
        rest.at[c][pl.ds(j * 128 + r, 16), :] = jnp.concatenate(alone, axis=1).astype(BF16)

    def router_scores(x_v, s, half, scores, pace):
        xs = [x_v[s, 16 * half:16 * half + 16, _tile(t)].astype(F32) for t in range(DM // 128)]
        r = _row_dot([pace(xs[0])] + xs[1:], wr_v[...].astype(F32))
        for i in range(2):
            scores = jnp.where(lane == 4 * s + 2 * half + i, r[8 * i:8 * i + 8], scores)
        return scores

    def select_tokens(scores):
        keys = []
        for h, r in enumerate(scores):
            r = r.astype(BF16).astype(F32)
            bits = pltpu.bitcast(jnp.where(r == 0.0, 0.0, r), I32) >> 16
            order = jnp.where(r != r, 0, jnp.where(bits < 0, ~bits, bits + 0x8000))
            token = (h * 128 + lane) * 8 + sub
            keys.append(pltpu.bitcast((1 << 29) + (order << 11) + (SEQ - 1 - token), F32))
        tiles = [zero] * (DM // 128)
        for n in range(TOPK):
            top = jnp.max(jnp.maximum(keys[0], keys[1]), axis=0, keepdims=True)
            top = jnp.max(top, axis=1, keepdims=True)
            keys = [jnp.where(k == top, 0.0, k) for k in keys]
            low = pltpu.bitcast(jnp.broadcast_to(top, (8, 128)), I32)[0, 0] & (SEQ - 1)
            token = SEQ - 1 - low
            chosen[n] = token
            rows = xbuf[token >> 5, _rows(token & 24, 8), :].astype(F32)
            rows = pltpu.roll(rows, (n - token) & 7, 0)
            tiles = [jnp.where(sub == n, rows[:, _tile(t)], z) for t, z in enumerate(tiles)]
        r, g = [jax.nn.sigmoid(_row_dot(tiles, v[...].astype(F32))) for v in (wr_v, gw_v)]
        return jnp.concatenate(tiles, axis=1), jnp.broadcast_to(r * (1.0 - g), (8, 128))

    def qkv_chunk(w, c, group, groups, never, extra=None):
        pairs = pl.ds(w * NPAIR + 4 * group, 4 * groups)
        raw = stage32.at[w, pl.ds(group, groups)]
        res, sums = wres.at[pairs, _rows(c * 128, 128)], dbuf.at[pairs]
        alone = qkv_blocks(raw, res, 0)
        for j in range(4 * groups):
            ahead = qkv_blocks(raw, res, j + 1) if j + 1 < 4 * groups else None
            for r in range(0, SROWS, ROWS_P0):
                rows = pl.ds(r, ROWS_P0)
                ops = [xl.at[c][rows, _tile(t)] for t in range(3)]
                if ahead is not None:
                    n = 128 - 16 * min((r + ROWS_P0) * 8 // SROWS + 1, 8)
                    ops[0] = jnp.concatenate(
                        [jnp.where(never, ahead[0][n:n + 16], ops[0][:16]), ops[0][16:]], axis=0)
                m1, m6, m7 = [_mm(ops[t], alone[t]) for t in range(3)]
                for t, d in enumerate((m1 + m7, m1 + m6)):
                    if not isinstance(c, int):
                        d = d + jnp.where(c > 0, sums[j, rows, _tile(t)], 0.0)
                    elif c > 0:
                        d = d + sums[j, rows, _tile(t)]
                    sums[j, rows, _tile(t)] = d
                if extra is not None:
                    extra((j * SROWS + r) // ROWS_P0, m1)
            alone = ahead

    x_first.start()
    w_start(0, 0, sem_g)
    w_start(1, 0)
    w_start(2, 0)
    x_first.wait()
    for cp in [x_second, x_rest] + small:
        cp.start()
    x_blocks(0)

    def first(g, carry):
        pltpu.make_async_copy(stage.at[0, g], stage.at[0, g], sem_g.at[g]).wait()
        qkv_chunk(0, 0, g, 1, g < 0)
        return carry

    lax.fori_loop(0, NGROUP, first, 0)
    w_start(0, 1)

    def early(i, carry):
        c, w = carry
        w_wait(w)

        @pl.when(i == 3)
        def _():
            x_second.wait()

        @pl.when(i == 6)
        def _():
            x_right(0).wait()
            x_right(1).wait()

        @pl.when((i == 2) | (i == 3))
        def _():
            x_right(jnp.clip(i - 2, 0, 1)).start()

        @pl.when(i >= 4)
        def _():
            wo_copy(jnp.maximum(i - 4, 0)).start()

        @pl.when(w == 0)
        def _():
            x_blocks(c)

        qkv_chunk(w, c, 0, NGROUP, i < 0)
        for n in range(3):
            @pl.when(w == n)
            def _():
                w_start(n, c + 1)

        return jnp.where(w == 2, c + 1, c), jnp.where(w == 2, 0, w + 1)

    lax.fori_loop(1, 3 * (NC - 1), early, (0, 1))

    for cp in [x_rest, wo_copy(0)] + small:
        cp.wait()
    wo_copy(5, 1).start()
    ff_start(0)
    x_blocks(NC - 1)

    def wo_views(first, pairs):
        return (wo_raw.at[_window(first, pairs, 256)], wores.at[:, _window(first, pairs, 128)],
                woalone.at[:, _window(first, pairs, 128)])

    def last(w, carry):
        scores, fresh = carry[0], [zero]
        w_wait(w)
        wo_copy(jnp.minimum(w + 1, 2) + w).wait()

        @pl.when(w == 1)
        def _():
            wo_copy(2).wait()

        x_v = xbuf.at[_rows(jnp.minimum(w, 1) * (NSEG // 2), NSEG // 2)]
        wo_todo = [(j, c, r) for j in range(5) for c in range(NC) for r in range(0, 128, 16)]
        slots = (NPAIR * SROWS - 128) // ROWS_P0
        views = wo_views(5 * w, 5)

        def extra(n, m):
            pace = lambda z: jnp.where(w < 0, m[:z.shape[0]], z)
            for item in wo_todo[len(wo_todo) * n // slots:len(wo_todo) * (n + 1) // slots]:
                wo_blocks(views, *item, pace)
            for g in range(NSEG * n // slots, min(NSEG * (n + 1) // slots, NSEG)):
                fresh[0] = router_scores(x_v, g // 2, g % 2, fresh[0], pace)

        picked = select_tokens(scores)
        qkv_chunk(w, NC - 1, 0, NGROUP, w < 0, extra)
        return (jnp.where(w == 0, fresh[0], scores[0]), fresh[0]), picked

    _, (xsel, weight) = _repeat(
        3, last, ((zero, zero), (jnp.zeros((8, DM), F32), zero)), UNROLL_LAST)

    wo_copy(5, 1).wait()
    ff_wait(0)
    for c in range(NC):
        for r in range(0, 128, 16):
            wo_blocks(wo_views(NPAIR - 1, 1), 0, c, r, lambda z: z)

    qi = lax.broadcasted_iota(I32, (MEM + SEG, MEM + SEG), 0)
    ki = lax.broadcasted_iota(I32, (MEM + SEG, MEM + SEG), 1)
    visible = (qi < MEM) | (qi >= ki)

    def attend(q, k):
        sc = lax.dot_general(q, k, (((1,), (1,)), ((), ())), preferred_element_type=F32)
        if EXP2:
            sc = jnp.where(visible, sc * (HD ** -0.5 * LOG2E), -1000000000.0 * LOG2E)
            e = jnp.exp2(sc - jnp.max(sc, axis=1, keepdims=True))
        else:
            sc = jnp.where(visible, sc * HD ** -0.5, -1000000000.0)
            e = jnp.exp(sc - jnp.max(sc, axis=1, keepdims=True))
        total = jnp.sum(e, axis=1, keepdims=True)
        inv = pltpu.reciprocal(total, approx=True)
        return e, inv * (2.0 - total * inv)

    def segment(views, s, mem, held, filler, never, ready):
        x_v, sums, ops_out, mix, gates = views
        r8, r32 = pl.ds(s * 8, 8), pl.ds(s * SEG, SEG)
        xs = [jnp.where(never, 1.0, x_v[s, :, _tile(t)].astype(F32)) for t in range(DM // 128)]
        for c in range(NC):
            ops = _resident_lhs(mem[2 * c], mem[2 * c + 1], xs[2 * c], xs[2 * c + 1])
            for t in range(4):
                lhs.at[t][:, _tile(c)] = ops[t]
        g = jnp.broadcast_to(jax.nn.sigmoid(_row_dot(xs, gw_v[...].astype(F32))), (SEG, 128))
        gates[pl.ds(s * 16, 16), :] = g[16:32]

        def products(w, j, k):
            return [_mm(lhs.at[t][:, k], wres.at[w * NPAIR + j][k, _tile(t)]) for t in range(4)]

        due = []

        def on_time(z):
            for _ in range(min(len(due), PER)):
                z = jnp.where(never, due.pop(0), z)
            return z

        def project(w, j, head=None):
            u = w * NPAIR + j
            if head is None:
                m2, m4, m3, m5 = products(w, j, slice(0, NC * 128))
            else:
                m2, m4, m3, m5 = [b + a for a, b in zip(head, products(w, j, _tile(NC - 1)))]
            left, right = m2 + m4, m3 + m5
            c11 = m4[8:16] - m5[8:16] + on_time(sums[u, r8, _tile(0)])
            c22 = m3[8:16] - m2[8:16] + on_time(sums[u, r8, _tile(1)])
            return (jnp.concatenate([left[0:8], left[16:32], c11, left[8:16]], axis=0),
                    jnp.concatenate([right[0:8], right[16:32], right[8:16], c22], axis=0))

        keep = {}

        def values(j, p, v):
            oe, oo = [_mm(e * inv, vh) if NORM else _mm(e, vh) * inv for (e, inv), vh in zip(p, v)]
            ops = _resident_lhs(oe[0:8], oo[0:8], oe[8:40], oo[8:40])
            for t in range(4):
                olhs.at[t][:, _tile(j)] = ops[t]
            if PACE & 1:
                ready.extend((oe + oo)[n:n + 8] for n in range(0, MEM + SEG, 8))
            alone = _alone_lhs(oe[24:32], oo[24:32], oe[32:40], oo[32:40])
            if PACE & 2:
                ready.extend(alone)
            if held is None:
                keep[j] = alone
            else:
                for t in range(3):
                    ops_out.at[t][pl.ds((s - 1) * 8, 16), _tile(j)] = jnp.concatenate(
                        [held[j][t], alone[t]], axis=0).astype(BF16)

        def out_proj(c, j0, j1):
            k = slice(j0 * 128, j1 * 128)
            return [_mm(olhs.at[t][:, k], wores.at[c][k, _tile(t)]) for t in range(4)]

        new_mem = [None] * (2 * NC)

        acc = {}

        def out_part(c, j0, j1):
            m2, m4, m3, m5 = out_proj(c, j0, j1)
            new = [m2 + m4, m3 + m5, m4[8:16] - m5[8:16], m3[8:16] - m2[8:16]]
            acc[c] = [a + b for a, b in zip(acc[c], new)] if c in acc else new

        def out_done(c):
            left, right, c11, c22 = acc[c]
            new_mem[2 * c], new_mem[2 * c + 1] = left[0:8], right[0:8]
            parts = ((left[16:32], c11, left[8:16]), (right[16:32], right[8:16], c22))
            for t, a in zip((2 * c, 2 * c + 1), parts):
                z = g * jnp.concatenate(a, axis=0) + (1.0 - g) * x_v[s, :, _tile(t)].astype(F32)
                mix[r32, _tile(t)] = z
                if PACE & 4:
                    ready.extend(z[n:n + 8] for n in range(0, SEG, 8))

        first = [("qkv".index(op.lower()), int(op.isupper()))
                 for op in ORDER if op in "qkvQKV"][:2]
        heads = {wj: products(*wj, slice(0, (NC - 1) * 128)) for wj in first}
        got = {}
        for pair in range(0, NPAIR, 2):
            due.extend(ready)
            ready.clear()
            for op in ORDER:
                j = pair + op.isupper()
                if op in "qkvQKV":
                    w = "qkv".index(op.lower())
                    got[w, j] = project(w, j, heads.get((w, j)))
                    if KV16 >> w & 1:
                        got[w, j] = [z.astype(BF16) for z in got[w, j]]
                elif op in "sS":
                    got["p", j] = [attend(q, k) for q, k in zip(got[0, j], got[1, j])]
                elif op in "pP" and pair > 0:
                    values(j - 2, got["p", j - 2], got[2, j - 2])
                elif op == "f" and pair // 2 in SLOTS:
                    filler(SLOTS.index(pair // 2) + 1)
        out_part(0, 0, SPLIT)
        for j in (NPAIR - 2, NPAIR - 1):
            values(j, got["p", j], got[2, j])
        out_part(1, 0, SPLIT)
        for c in range(NC):
            out_part(c, SPLIT if c < 2 else 0, NPAIR)
            out_done(c)
        return new_mem, keep or None

    def trip(i, carry):
        mem, y = list(carry[0]), list(carry[1])

        f = jnp.minimum(i, NFP - 1)

        @pl.when(i + 1 < NFP)
        def _():
            ff_start(jnp.minimum(i + 1, NFP - 1))

        weights, hidden = ffw.at[f & 1], {}

        def ff_in(m):
            def fill(n):
                if n <= 4:
                    u, k = 2 * m + (n - 1) // 2, (n - 1) % 2 * 512
                    part = _mm(xsel[:, k:k + 512], weights[pl.ds(u * DM + k, 512), :])
                    hidden[u] = part if k == 0 else part + hidden[u]
            return fill

        def ff_out(n):
            if n <= 4:
                act = jnp.concatenate(
                    [jax.nn.silu(hidden[h]) * hidden[2 + h] for h in range(2)], axis=1)
                for t in (2 * n - 2, 2 * n - 1):
                    part = _mm(act, weights[pl.ds(4 * DM + t * 256, 256), :])
                    y[t] = y[t] + jnp.where(i < NFP, part, 0.0)

        views = (xbuf.at[_rows(i * UNROLL, UNROLL)], dbuf.at[:, _rows(i * UNROLL * 8, UNROLL * 8)],
                 oalone.at[:, _rows(i * UNROLL * 8, UNROLL * 8)],
                 apart.at[_rows(i * UNROLL * SEG, UNROLL * SEG)],
                 gate.at[_rows(i * UNROLL * 16, UNROLL * 16)])
        held, ready = None, []
        for s, fill in enumerate((lambda n: None, ff_in(0), ff_in(1), ff_out)):
            mem, held = segment(views, s, mem, held, fill, i < 0, ready)

        @pl.when(i + 1 < NFP)
        def _():
            ff_wait(i + 1)

        return tuple(mem), tuple(y)

    mem0 = tuple(mem_v[:, _tile(t)].astype(F32) for t in range(DM // 128))
    _, y = lax.fori_loop(0, NSEG // UNROLL, trip, (mem0, (zero,) * (DM // 128)))
    y = jnp.concatenate([part * weight for part in y], axis=1)
    for n in range(TOPK):
        apart[pl.ds(chosen[n], 1), :] += y[n:n + 1]

    def finish(n, carry):
        ops = oalone.at[:, _rows(n * SEG_FIN * 8, SEG_FIN * 8)]
        mix = apart.at[_rows(n * SEG_FIN * SEG, SEG_FIN * SEG)]
        gates = gate.at[_rows(n * SEG_FIN * 16, SEG_FIN * 16)]
        outs = out_v.at[_rows(n * SEG_FIN * SEG, SEG_FIN * SEG)]
        done = []
        for c in range(NC):
            for r in range(0, SEG_FIN * 8, ROWS_FIN):
                left = [ops.at[t][pl.ds(r, ROWS_FIN), :] for t in range(3)]
                if done:
                    late = jnp.concatenate(done[::len(done) // (2 * NPAIR)], axis=1)
                    for t, part in ((2, late[:, :NPAIR * 128]), (1, late[:, NPAIR * 128:])):
                        left[t] = jnp.concatenate(
                            [jnp.where(n < 0, part, left[t][:16]), left[t][16:]], axis=0)
                done = []
                m1, m7, m6 = [_mm(left[t], woalone.at[c][:, _tile(t)]) for t in (0, 2, 1)]
                d11, d22 = m1 + m7, m1 + m6
                for i in range(ROWS_FIN // 8):
                    s = r // 8 + i
                    r32 = pl.ds(s * SEG, SEG)
                    g = gates[pl.ds(s * 16, 16), :]
                    zl, zr = mix[r32, _tile(2 * c)], mix[r32, _tile(2 * c + 1)]
                    zl = [zl[0:16], zl[16:24] + g[0:8] * d11[8 * i:8 * i + 8], zl[24:32]]
                    zr = [zr[0:24], zr[24:32] + g[8:16] * d22[8 * i:8 * i + 8]]
                    for t, z in ((2 * c, zl), (2 * c + 1, zr)):
                        z = jnp.concatenate(z, axis=0).astype(BF16)
                        outs[r32, _tile(t)] = z
                        done += [z[16:], z[:16]]
                sl = (_window(n * SEG_FIN + r // 8, ROWS_FIN // 8, SEG), pl.ds(c * 256, 256))
                pltpu.make_async_copy(out_v.at[sl], out_hbm.at[sl], sem_out).start()
        return carry

    _repeat(NSEG // SEG_FIN, finish, 0, UNROLL_FIN)
    pltpu.make_async_copy(out_v, out_hbm, sem_out).wait()


def _by_head_group(w):
    return w.reshape(DM, HEADS // 8, 8, HD).transpose(0, 2, 1, 3).reshape(DM * 8, HEADS // 8 * HD)


@functools.partial(jax.jit, static_argnames=("A_seg_len",))
def pallas_gated_mix__memory_aug_recurrent_mem_tr__moe_arch_mod__prompt_kernel(
    A_x: jax.Array,
    A_mem0: jax.Array,
    A_Wq: jax.Array,
    A_Wk: jax.Array,
    A_Wv: jax.Array,
    A_Wo: jax.Array,
    A_seg_len: int,
    B_x: jax.Array,
    B_w_r: jax.Array,
    B_w_gate: jax.Array,
    B_w_up: jax.Array,
    B_w_down: jax.Array,
    gate_w: jax.Array,
):
    del B_x
    assert A_seg_len == SEG and A_x.shape == (1, SEQ, DM) and A_mem0.shape == (1, MEM, DM)
    assert A_Wq.shape == (DM, HEADS, HD) and B_w_gate.shape == (DM, FF)

    hbm = pl.BlockSpec(memory_space=pl.ANY)
    out = pl.pallas_call(
        _kernel,
        out_shape=jax.ShapeDtypeStruct((SEQ, DM), BF16),
        in_specs=[hbm] * 11,
        out_specs=hbm,
        scratch_shapes=[
            pltpu.VMEM((48, 128), BF16),
            pltpu.VMEM((NSEG, SEG, DM), BF16),
            pltpu.VMEM((MEM, DM), BF16),
            pltpu.VMEM((3, HEADS // 8, 2048, HD), BF16),
            pltpu.VMEM((HEADS * HD, DM), BF16),
            pltpu.VMEM((NC, SROWS // 2, 3 * 128), U32),
            pltpu.VMEM((3 * NPAIR, 256, 4 * 128), U32),
            pltpu.VMEM((NC, NPAIR * 64, 4 * 128), U32),
            pltpu.VMEM((NC, NPAIR * 64, 3 * 128), U32),
            pltpu.VMEM((3 * NPAIR, SROWS, 2 * 128), F32),
            pltpu.VMEM((4, 16, NC * 128), U32),
            pltpu.VMEM((4, 16, NPAIR * 128), U32),
            pltpu.VMEM((3, SROWS // 2, NPAIR * 128), U32),
            pltpu.VMEM((SEQ, DM), F32),
            pltpu.VMEM((SEQ // 2, 128), F32),
            pltpu.VMEM((2, 6 * DM, 128), BF16),
            pltpu.VMEM((SEQ, DM), BF16),
            pltpu.SMEM((TOPK,), I32),
            pltpu.SemaphoreType.DMA((3,)),
            pltpu.SemaphoreType.DMA((NGROUP,)),
            pltpu.SemaphoreType.DMA((NC + 1,)),
            pltpu.SemaphoreType.DMA((6,)),
            pltpu.SemaphoreType.DMA((3,)),
            pltpu.SemaphoreType.DMA((2,)),
            pltpu.SemaphoreType.DMA,
        ],
        compiler_params=pltpu.CompilerParams(
            vmem_limit_bytes=126 * 1024 * 1024, disable_bounds_checks=True, flags=FLAGS),
    )(
        A_x.reshape(NSEG, SEG, DM),
        A_mem0.reshape(MEM, DM),
        _by_head_group(A_Wq),
        _by_head_group(A_Wk),
        _by_head_group(A_Wv),
        A_Wo.reshape(HEADS * HD, DM),
        B_w_r.reshape(8, 128),
        B_w_gate,
        B_w_up,
        B_w_down,
        gate_w.reshape(8, 128),
    )
    return out.reshape(1, SEQ, DM)
```

```python
import functools

import jax
import jax.numpy as jnp
import numpy as np
from jax import lax
from jax.experimental import pallas as pl
from jax.experimental.pallas import tpu as pltpu

F32, BF16, U32, I32 = jnp.float32, jnp.bfloat16, jnp.uint32, jnp.int32

SEQ, DM, HEADS, HD = 2048, 1024, 32, 128
MEM, SEG, TOPK, FF = 8, 32, 8, 3584
NSEG = SEQ // SEG
NPAIR = HEADS // 2
NGROUP = HEADS // 8
NC = DM // 256
SROWS = NSEG * 8
ORDER = 'kKfpPqQvsSV'
SPLIT = 10
PACE = 4
PER = 3
TPERM = (2,3,0,1)
OPERM = (1,0,2,3)
FIRST0 = 1
NORM = 1
KV16 = 6
SLOTS = (1,2,4,6)
FLAGS = None
UNROLL_FIN = 0
UNROLL_LAST = 0
EXP2 = 0
LOG2E = 1.4426950408889634
UNROLL = 4
NFP = FF // 256
ROWS_P0 = 64
ROWS_FIN = 64
SEG_FIN = 32


def _mm(a, b):
    return jnp.dot(a, b, preferred_element_type=F32)


def _repeat(n, body, carry, unroll):
    return lax.fori_loop(0, n, body, carry, unroll=bool(unroll))


def _tile(i):
    return slice(i * 128, (i + 1) * 128)


def _rows(start, size):
    if isinstance(start, int):
        return pl.ds(start, size)
    return pl.ds(pl.multiple_of(start, size), size)


def _window(first, count, unit):
    start = first * unit
    return pl.ds(start if isinstance(start, int) else pl.multiple_of(start, unit), count * unit)


def _weight_blocks(b11, b12, b21, b22):
    resident = [b11, b21 - b11, b12 - b22, b22]
    alone = [b11 + b22, b11 + b12, b21 + b22]
    return resident, alone


def _resident_lhs(m1, m2, z1, z2):
    ms, zs = m1 + m2, z1 + z2
    parts = ((ms, zs[24:32], zs[0:16]), (m2, z2[24:32], z2[0:16]),
             (m1, z1[16:24], z1[0:16]), (ms, zs[16:24], zs[0:16]))
    return [jnp.concatenate(p, axis=0).astype(BF16) for p in parts]


def _alone_lhs(a11, a12, a21, a22):
    return [a11 + a22, a21 - a11, a12 - a22]


def _row_dot(x_tiles, w8):
    acc = x_tiles[0] * w8[0:1]
    for t in range(1, len(x_tiles)):
        acc = acc + x_tiles[t] * w8[t:t + 1]
    return jnp.sum(acc, axis=1, keepdims=True)


def _kernel(x_hbm, mem_hbm, wq_hbm, wk_hbm, wv_hbm, wo_hbm, wr_hbm, wg_hbm,
            wu_hbm, wd_hbm, gw_hbm, out_hbm,
            vecs, xbuf, mem_v, stage, wo_raw, xl_u, wres_u, wores_u,
            woalone_u, dbuf, lhs_u, olhs_u, oalone_u, apart, gate, ffw, out_v, chosen,
            sem_w, sem_g, sem_x, sem_o, sem_s, sem_f, sem_out):
    xl = xl_u.bitcast(BF16)
    wres = wres_u.bitcast(BF16)
    wores = wores_u.bitcast(BF16)
    woalone = woalone_u.bitcast(BF16)
    lhs = lhs_u.bitcast(BF16)
    olhs = olhs_u.bitcast(BF16)
    oalone = oalone_u.bitcast(BF16)
    stage32 = stage.bitcast(U32)

    wr_v, gw_v = vecs.at[0:8], vecs.at[16:24]
    zero = jnp.zeros((8, 128), F32)
    lane = lax.broadcasted_iota(I32, (8, 128), 1)
    sub = lax.broadcasted_iota(I32, (8, 128), 0)

    staged = stage.at[:, :, pl.ds(0, 2048)]

    def w_start(w, c, sems=None):
        for g in range(NGROUP):
            pltpu.make_async_copy(
                (wq_hbm, wk_hbm, wv_hbm)[w].at[_rows(c * 2048, 2048), _tile(g)],
                staged.at[w, g], sem_w.at[w] if sems is None else sems.at[g]).start()

    def w_wait(w):
        pltpu.make_async_copy(staged.at[w], staged.at[w], sem_w.at[w]).wait()

    def x_copy(n, segs, rows, cols):
        return pltpu.make_async_copy(
            x_hbm.at[segs, rows, cols], xbuf.at[segs, rows, cols], sem_x.at[n])

    every = slice(None)
    x_first = x_copy(0, every, pl.ds(16, 16), pl.ds(0, 256))
    x_rest = x_copy(1, every, pl.ds(0, 16), pl.ds(0, 256))
    x_second = x_copy(2, every, every, pl.ds(256, 256))

    def x_right(h):
        return x_copy(3 + h, _rows(h * (NSEG // 2), NSEG // 2), every, pl.ds(512, 512))

    def wo_copy(p, pairs=3):
        rows = _window(3 * p, pairs, 256)
        return pltpu.make_async_copy(wo_hbm.at[rows], wo_raw.at[rows], sem_o.at[p])

    def ff_start(f):
        dst, sem = ffw.at[f & 1], sem_f.at[f & 1]
        for h in range(2):
            cols = _rows(f * 256 + h * 128, 128)
            for n, src in enumerate((wg_hbm, wu_hbm)):
                pltpu.make_async_copy(
                    src.at[:, cols], dst.at[pl.ds((2 * n + h) * DM, DM)], sem).start()
        for t in range(DM // 128):
            pltpu.make_async_copy(wd_hbm.at[_rows(f * 256, 256), _tile(t)],
                                  dst.at[pl.ds(4 * DM + t * 256, 256)], sem).start()

    def ff_wait(f):
        pltpu.make_async_copy(ffw.at[f & 1], ffw.at[f & 1], sem_f.at[f & 1]).wait()

    small = [pltpu.make_async_copy(s, d, sem_s.at[i]) for i, (s, d) in enumerate(
        ((mem_hbm, mem_v), (wr_hbm, wr_v), (gw_hbm, gw_v)))]

    def x_blocks(c):
        src, dst = xbuf.at[:, :, _rows(c * 256, 256)], xl.at[c]
        for n in range(NSEG // 2):
            got = []
            for s in (2 * n, 2 * n + 1):
                z1, z2 = [src[s, 16:32, _tile(h)].astype(F32) for h in range(2)]
                got.append(_alone_lhs(z1[0:8], z2[0:8], z1[8:16], z2[8:16]))
            for t in range(3):
                dst[pl.ds(n * 16, 16), _tile(t)] = jnp.concatenate(
                    [got[0][t], got[1][t]], axis=0).astype(BF16)

    def qkv_blocks(raw, res, j):
        raw = raw.at[j // 4]
        even = lambda z: pltpu.bitcast(z << 16, F32)
        odd = lambda z: pltpu.bitcast(z & np.uint32(0xFFFF0000), F32)
        rest = []
        for r in range(112, -16, -16):
            h1 = raw[pl.ds(4 * r + j % 4, 16, stride=4), :]
            h2 = raw[pl.ds(4 * (128 + r) + j % 4, 16, stride=4), :]
            resident, alone = _weight_blocks(even(h1), odd(h1), even(h2), odd(h2))
            res.at[j][pl.ds(r, 16), :] = jnp.concatenate(resident, axis=1).astype(BF16)
            rest.insert(0, alone)
        return tuple(jnp.concatenate(a, axis=0).astype(BF16) for a in zip(*rest))

    def wo_blocks(views, j, c, r, pace):
        raw, res, rest = views
        b11, b12, b21, b22 = [
            raw[pl.ds(j * 256 + half + r, 16), _tile(2 * c + h)].astype(F32)
            for half in (0, 128) for h in range(2)]
        resident, alone = _weight_blocks(pace(b11), b12, b21, b22)
        res.at[c][pl.ds(j * 128 + r, 16), :] = jnp.concatenate(resident, axis=1).astype(BF16)
        rest.at[c][pl.ds(j * 128 + r, 16), :] = jnp.concatenate(alone, axis=1).astype(BF16)

    def router_scores(x_v, s, half, scores, pace):
        xs = [x_v[s, 16 * half:16 * half + 16, _tile(t)].astype(F32) for t in range(DM // 128)]
        r = _row_dot([pace(xs[0])] + xs[1:], wr_v[...].astype(F32))
        for i in range(2):
            scores = jnp.where(lane == 4 * s + 2 * half + i, r[8 * i:8 * i + 8], scores)
        return scores

    def select_tokens(scores):
        keys = []
        for h, r in enumerate(scores):
            r = r.astype(BF16).astype(F32)
            bits = pltpu.bitcast(jnp.where(r == 0.0, 0.0, r), I32) >> 16
            order = jnp.where(r != r, 0, jnp.where(bits < 0, ~bits, bits + 0x8000))
            token = (h * 128 + lane) * 8 + sub
            keys.append(pltpu.bitcast((1 << 29) + (order << 11) + (SEQ - 1 - token), F32))
        tiles = [zero] * (DM // 128)
        for n in range(TOPK):
            top = jnp.max(jnp.maximum(keys[0], keys[1]), axis=0, keepdims=True)
            top = jnp.max(top, axis=1, keepdims=True)
            keys = [jnp.where(k == top, 0.0, k) for k in keys]
            low = pltpu.bitcast(jnp.broadcast_to(top, (8, 128)), I32)[0, 0] & (SEQ - 1)
            token = SEQ - 1 - low
            chosen[n] = token
            rows = xbuf[token >> 5, _rows(token & 24, 8), :].astype(F32)
            rows = pltpu.roll(rows, (n - token) & 7, 0)
            tiles = [jnp.where(sub == n, rows[:, _tile(t)], z) for t, z in enumerate(tiles)]
        r, g = [jax.nn.sigmoid(_row_dot(tiles, v[...].astype(F32))) for v in (wr_v, gw_v)]
        return jnp.concatenate(tiles, axis=1), jnp.broadcast_to(r * (1.0 - g), (8, 128))

    def qkv_chunk(w, c, group, groups, never, extra=None):
        pairs = pl.ds(w * NPAIR + 4 * group, 4 * groups)
        raw = stage32.at[w, pl.ds(group, groups)]
        res, sums = wres.at[pairs, _rows(c * 128, 128)], dbuf.at[pairs]
        alone = qkv_blocks(raw, res, 0)
        for j in range(4 * groups):
            ahead = qkv_blocks(raw, res, j + 1) if j + 1 < 4 * groups else None
            for r in range(0, SROWS, ROWS_P0):
                rows = pl.ds(r, ROWS_P0)
                ops = [xl.at[c][rows, _tile(t)] for t in range(3)]
                if ahead is not None:
                    n = 128 - 16 * min((r + ROWS_P0) * 8 // SROWS + 1, 8)
                    ops[0] = jnp.concatenate(
                        [jnp.where(never, ahead[0][n:n + 16], ops[0][:16]), ops[0][16:]], axis=0)
                m1, m6, m7 = [_mm(ops[t], alone[t]) for t in range(3)]
                for t, d in enumerate((m1 + m7, m1 + m6)):
                    if not isinstance(c, int):
                        d = d + jnp.where(c > 0, sums[j, rows, _tile(t)], 0.0)
                    elif c > 0:
                        d = d + sums[j, rows, _tile(t)]
                    sums[j, rows, _tile(t)] = d
                if extra is not None:
                    extra((j * SROWS + r) // ROWS_P0, m1)
            alone = ahead

    x_first.start()
    w_start(0, 0, sem_g)
    w_start(1, 0)
    w_start(2, 0)
    x_first.wait()
    for cp in [x_second, x_rest] + small:
        cp.start()
    x_blocks(0)

    def first(g, carry):
        pltpu.make_async_copy(staged.at[0, g], staged.at[0, g], sem_g.at[g]).wait()
        qkv_chunk(0, 0, g, 1, g < 0)
        return carry

    lax.fori_loop(0, NGROUP, first, 0)
    w_start(0, 1)

    def early(i, carry):
        c, w = carry
        w_wait(w)

        @pl.when(i == 3)
        def _():
            x_second.wait()

        @pl.when(i == 6)
        def _():
            x_right(0).wait()
            x_right(1).wait()

        @pl.when((i == 2) | (i == 3))
        def _():
            x_right(jnp.clip(i - 2, 0, 1)).start()

        @pl.when(i >= 4)
        def _():
            wo_copy(jnp.maximum(i - 4, 0)).start()

        @pl.when(w == 0)
        def _():
            x_blocks(c)

        qkv_chunk(w, c, 0, NGROUP, i < 0)
        for n in range(3):
            @pl.when(w == n)
            def _():
                w_start(n, c + 1)

        return jnp.where(w == 2, c + 1, c), jnp.where(w == 2, 0, w + 1)

    lax.fori_loop(1, 3 * (NC - 1), early, (0, 1))

    for cp in [x_rest, wo_copy(0)] + small:
        cp.wait()
    wo_copy(5, 1).start()
    ff_start(0)
    x_blocks(NC - 1)

    def wo_views(first, pairs):
        return (wo_raw.at[_window(first, pairs, 256)], wores.at[:, _window(first, pairs, 128)],
                woalone.at[:, _window(first, pairs, 128)])

    def last(w, carry):
        scores, fresh = carry[0], [zero]
        w_wait(w)
        wo_copy(jnp.minimum(w + 1, 2) + w).wait()

        @pl.when(w == 1)
        def _():
            wo_copy(2).wait()

        x_v = xbuf.at[_rows(jnp.minimum(w, 1) * (NSEG // 2), NSEG // 2)]
        wo_todo = [(j, c, r) for j in range(5) for c in range(NC) for r in range(0, 128, 16)]
        slots = (NPAIR * SROWS - 128) // ROWS_P0
        views = wo_views(5 * w, 5)

        def extra(n, m):
            pace = lambda z: jnp.where(w < 0, m[:z.shape[0]], z)
            for item in wo_todo[len(wo_todo) * n // slots:len(wo_todo) * (n + 1) // slots]:
                wo_blocks(views, *item, pace)
            for g in range(NSEG * n // slots, min(NSEG * (n + 1) // slots, NSEG)):
                fresh[0] = router_scores(x_v, g // 2, g % 2, fresh[0], pace)

        picked = select_tokens(scores)
        qkv_chunk(w, NC - 1, 0, NGROUP, w < 0, extra)
        return (jnp.where(w == 0, fresh[0], scores[0]), fresh[0]), picked

    _, (xsel, weight) = _repeat(
        3, last, ((zero, zero), (jnp.zeros((8, DM), F32), zero)), UNROLL_LAST)

    wo_copy(5, 1).wait()
    ff_wait(0)
    for c in range(NC):
        for r in range(0, 128, 16):
            wo_blocks(wo_views(NPAIR - 1, 1), 0, c, r, lambda z: z)

    qi = lax.broadcasted_iota(I32, (MEM + SEG, MEM + SEG), 0)
    ki = lax.broadcasted_iota(I32, (MEM + SEG, MEM + SEG), 1)
    visible = (qi < MEM) | (qi >= ki)

    def attend(q, k):
        sc = lax.dot_general(q, k, (((1,), (1,)), ((), ())), preferred_element_type=F32)
        if EXP2:
            sc = jnp.where(visible, sc * (HD ** -0.5 * LOG2E), -1000000000.0 * LOG2E)
            e = jnp.exp2(sc - jnp.max(sc, axis=1, keepdims=True))
        else:
            sc = jnp.where(visible, sc * HD ** -0.5, -1000000000.0)
            e = jnp.exp(sc - jnp.max(sc, axis=1, keepdims=True))
        total = jnp.sum(e, axis=1, keepdims=True)
        inv = pltpu.reciprocal(total, approx=True)
        return e, inv * (2.0 - total * inv)

    def segment(views, s, mem, held, filler, never, ready):
        x_v, sums, ops_out, mix, gates = views
        r8, r32 = pl.ds(s * 8, 8), pl.ds(s * SEG, SEG)
        xs = [jnp.where(never, 1.0, x_v[s, :, _tile(t)].astype(F32)) for t in range(DM // 128)]
        for c in range(NC):
            ops = _resident_lhs(mem[2 * c], mem[2 * c + 1], xs[2 * c], xs[2 * c + 1])
            for t in range(4):
                lhs.at[t][:, _tile(c)] = ops[t]
        g = jnp.broadcast_to(jax.nn.sigmoid(_row_dot(xs, gw_v[...].astype(F32))), (SEG, 128))
        gates[pl.ds(s * 16, 16), :] = g[16:32]

        def products(w, j, k):
            m = {t: _mm(lhs.at[t][:, k], wres.at[w * NPAIR + j][k, _tile(t)]) for t in TPERM}
            return [m[t] for t in range(4)]

        due = []

        def on_time(z):
            for _ in range(min(len(due), PER)):
                z = jnp.where(never, due.pop(0), z)
            return z

        def project(w, j, head=None):
            u = w * NPAIR + j
            if head is None:
                m2, m4, m3, m5 = products(w, j, slice(0, NC * 128))
            else:
                m2, m4, m3, m5 = [b + a for a, b in zip(head, products(w, j, _tile(NC - 1)))]
            left, right = m2 + m4, m3 + m5
            c11 = m4[8:16] - m5[8:16] + on_time(sums[u, r8, _tile(0)])
            c22 = m3[8:16] - m2[8:16] + on_time(sums[u, r8, _tile(1)])
            return (jnp.concatenate([left[0:8], left[16:32], c11, left[8:16]], axis=0),
                    jnp.concatenate([right[0:8], right[16:32], right[8:16], c22], axis=0))

        keep = {}

        def values(j, p, v):
            oe, oo = [_mm(e * inv, vh) if NORM else _mm(e, vh) * inv for (e, inv), vh in zip(p, v)]
            ops = _resident_lhs(oe[0:8], oo[0:8], oe[8:40], oo[8:40])
            for t in range(4):
                olhs.at[t][:, _tile(j)] = ops[t]
            if PACE & 1:
                ready.extend((oe + oo)[n:n + 8] for n in range(0, MEM + SEG, 8))
            alone = _alone_lhs(oe[24:32], oo[24:32], oe[32:40], oo[32:40])
            if PACE & 2:
                ready.extend(alone)
            if held is None:
                keep[j] = alone
            else:
                for t in range(3):
                    ops_out.at[t][pl.ds((s - 1) * 8, 16), _tile(j)] = jnp.concatenate(
                        [held[j][t], alone[t]], axis=0).astype(BF16)

        def out_proj(c, j0, j1):
            k = slice(j0 * 128, j1 * 128)
            m = {t: _mm(olhs.at[t][:, k], wores.at[c][k, _tile(t)]) for t in OPERM}
            return [m[t] for t in range(4)]

        new_mem = [None] * (2 * NC)

        acc = {}

        def out_part(c, j0, j1):
            m2, m4, m3, m5 = out_proj(c, j0, j1)
            new = [m2 + m4, m3 + m5, m4[8:16] - m5[8:16], m3[8:16] - m2[8:16]]
            acc[c] = [a + b for a, b in zip(acc[c], new)] if c in acc else new

        def out_done(c):
            left, right, c11, c22 = acc[c]
            new_mem[2 * c], new_mem[2 * c + 1] = left[0:8], right[0:8]
            parts = ((left[16:32], c11, left[8:16]), (right[16:32], right[8:16], c22))
            for t, a in zip((2 * c, 2 * c + 1), parts):
                z = g * jnp.concatenate(a, axis=0) + (1.0 - g) * x_v[s, :, _tile(t)].astype(F32)
                mix[r32, _tile(t)] = z
                if PACE & 4:
                    ready.extend(z[n:n + 8] for n in range(0, SEG, 8))

        first = [("qkv".index(op.lower()), int(op.isupper()))
                 for op in ORDER if op in "qkvQKV"][:2]
        heads = {wj: products(*wj, slice(0, (NC - 1) * 128)) for wj in first if s or FIRST0}
        got = {}
        for pair in range(0, NPAIR, 2):
            due.extend(ready)
            ready.clear()
            for op in ORDER:
                j = pair + op.isupper()
                if op in "qkvQKV":
                    w = "qkv".index(op.lower())
                    got[w, j] = project(w, j, heads.get((w, j)))
                    if KV16 >> w & 1:
                        got[w, j] = [z.astype(BF16) for z in got[w, j]]
                elif op in "sS":
                    got["p", j] = [attend(q, k) for q, k in zip(got[0, j], got[1, j])]
                elif op in "pP" and pair > 0:
                    values(j - 2, got["p", j - 2], got[2, j - 2])
                elif op == "f" and pair // 2 in SLOTS:
                    filler(SLOTS.index(pair // 2) + 1)
        out_part(0, 0, SPLIT)
        for j in (NPAIR - 2, NPAIR - 1):
            values(j, got["p", j], got[2, j])
        out_part(1, 0, SPLIT)
        for c in range(NC):
            out_part(c, SPLIT if c < 2 else 0, NPAIR)
            out_done(c)
        return new_mem, keep or None

    def trip(i, carry):
        mem, y = list(carry[0]), list(carry[1])

        f = jnp.minimum(i, NFP - 1)

        @pl.when(i + 1 < NFP)
        def _():
            ff_start(jnp.minimum(i + 1, NFP - 1))

        weights, hidden = ffw.at[f & 1], {}

        def ff_in(m):
            def fill(n):
                if n <= 4:
                    u, k = 2 * m + (n - 1) // 2, (n - 1) % 2 * 512
                    part = _mm(xsel[:, k:k + 512], weights[pl.ds(u * DM + k, 512), :])
                    hidden[u] = part if k == 0 else part + hidden[u]
            return fill

        def ff_out(n):
            if n <= 4:
                act = jnp.concatenate(
                    [jax.nn.silu(hidden[h]) * hidden[2 + h] for h in range(2)], axis=1)
                for t in (2 * n - 2, 2 * n - 1):
                    part = _mm(act, weights[pl.ds(4 * DM + t * 256, 256), :])
                    y[t] = y[t] + jnp.where(i < NFP, part, 0.0)

        views = (xbuf.at[_rows(i * UNROLL, UNROLL)], dbuf.at[:, _rows(i * UNROLL * 8, UNROLL * 8)],
                 oalone.at[:, _rows(i * UNROLL * 8, UNROLL * 8)],
                 apart.at[_rows(i * UNROLL * SEG, UNROLL * SEG)],
                 gate.at[_rows(i * UNROLL * 16, UNROLL * 16)])
        held, ready = None, []
        for s, fill in enumerate((lambda n: None, ff_in(0), ff_in(1), ff_out)):
            mem, held = segment(views, s, mem, held, fill, i < 0, ready)

        @pl.when(i + 1 < NFP)
        def _():
            ff_wait(i + 1)

        return tuple(mem), tuple(y)

    mem0 = tuple(mem_v[:, _tile(t)].astype(F32) for t in range(DM // 128))
    _, y = lax.fori_loop(0, NSEG // UNROLL, trip, (mem0, (zero,) * (DM // 128)))
    y = jnp.concatenate([part * weight for part in y], axis=1)
    for n in range(TOPK):
        apart[pl.ds(chosen[n], 1), :] += y[n:n + 1]

    def finish(n, carry):
        ops = oalone.at[:, _rows(n * SEG_FIN * 8, SEG_FIN * 8)]
        mix = apart.at[_rows(n * SEG_FIN * SEG, SEG_FIN * SEG)]
        gates = gate.at[_rows(n * SEG_FIN * 16, SEG_FIN * 16)]
        outs = out_v.at[_rows(n * SEG_FIN * SEG, SEG_FIN * SEG)]
        done = []
        for c in range(NC):
            for r in range(0, SEG_FIN * 8, ROWS_FIN):
                left = [ops.at[t][pl.ds(r, ROWS_FIN), :] for t in range(3)]
                if done:
                    late = jnp.concatenate(done[::len(done) // (2 * NPAIR)], axis=1)
                    for t, part in ((2, late[:, :NPAIR * 128]), (1, late[:, NPAIR * 128:])):
                        left[t] = jnp.concatenate(
                            [jnp.where(n < 0, part, left[t][:16]), left[t][16:]], axis=0)
                done = []
                m1, m7, m6 = [_mm(left[t], woalone.at[c][:, _tile(t)]) for t in (0, 2, 1)]
                d11, d22 = m1 + m7, m1 + m6
                for i in range(ROWS_FIN // 8):
                    s = r // 8 + i
                    r32 = pl.ds(s * SEG, SEG)
                    g = gates[pl.ds(s * 16, 16), :]
                    zl, zr = mix[r32, _tile(2 * c)], mix[r32, _tile(2 * c + 1)]
                    zl = [zl[0:16], zl[16:24] + g[0:8] * d11[8 * i:8 * i + 8], zl[24:32]]
                    zr = [zr[0:24], zr[24:32] + g[8:16] * d22[8 * i:8 * i + 8]]
                    for t, z in ((2 * c, zl), (2 * c + 1, zr)):
                        z = jnp.concatenate(z, axis=0).astype(BF16)
                        outs[r32, _tile(t)] = z
                        done += [z[16:], z[:16]]
                sl = (_window(n * SEG_FIN + r // 8, ROWS_FIN // 8, SEG), pl.ds(c * 256, 256))
                pltpu.make_async_copy(out_v.at[sl], out_hbm.at[sl], sem_out).start()
        return carry

    _repeat(NSEG // SEG_FIN, finish, 0, UNROLL_FIN)
    pltpu.make_async_copy(out_v, out_hbm, sem_out).wait()


def _by_head_group(w):
    return w.reshape(DM, HEADS // 8, 8, HD).transpose(0, 2, 1, 3).reshape(DM * 8, HEADS // 8 * HD)


@functools.partial(jax.jit, static_argnames=("A_seg_len",))
def pallas_gated_mix__memory_aug_recurrent_mem_tr__moe_arch_mod__prompt_kernel(
    A_x: jax.Array,
    A_mem0: jax.Array,
    A_Wq: jax.Array,
    A_Wk: jax.Array,
    A_Wv: jax.Array,
    A_Wo: jax.Array,
    A_seg_len: int,
    B_x: jax.Array,
    B_w_r: jax.Array,
    B_w_gate: jax.Array,
    B_w_up: jax.Array,
    B_w_down: jax.Array,
    gate_w: jax.Array,
):
    del B_x
    assert A_seg_len == SEG and A_x.shape == (1, SEQ, DM) and A_mem0.shape == (1, MEM, DM)
    assert A_Wq.shape == (DM, HEADS, HD) and B_w_gate.shape == (DM, FF)

    hbm = pl.BlockSpec(memory_space=pl.ANY)
    out = pl.pallas_call(
        _kernel,
        out_shape=jax.ShapeDtypeStruct((SEQ, DM), BF16),
        in_specs=[hbm] * 11,
        out_specs=hbm,
        scratch_shapes=[
            pltpu.VMEM((48, 128), BF16),
            pltpu.VMEM((NSEG, SEG, DM), BF16),
            pltpu.VMEM((MEM, DM), BF16),
            pltpu.VMEM((3, NGROUP, 2048 + 64, HD), BF16),
            pltpu.VMEM((HEADS * HD, DM), BF16),
            pltpu.VMEM((NC, SROWS // 2, 3 * 128), U32),
            pltpu.VMEM((3 * NPAIR, 256, 4 * 128), U32),
            pltpu.VMEM((NC, NPAIR * 64, 4 * 128), U32),
            pltpu.VMEM((NC, NPAIR * 64, 3 * 128), U32),
            pltpu.VMEM((3 * NPAIR, SROWS, 2 * 128), F32),
            pltpu.VMEM((4, 16, NC * 128), U32),
            pltpu.VMEM((4, 16, NPAIR * 128), U32),
            pltpu.VMEM((3, SROWS // 2, NPAIR * 128), U32),
            pltpu.VMEM((SEQ, DM), F32),
            pltpu.VMEM((SEQ // 2, 128), F32),
            pltpu.VMEM((2, 6 * DM, 128), BF16),
            pltpu.VMEM((SEQ, DM), BF16),
            pltpu.SMEM((TOPK,), I32),
            pltpu.SemaphoreType.DMA((3,)),
            pltpu.SemaphoreType.DMA((NGROUP,)),
            pltpu.SemaphoreType.DMA((NC + 1,)),
            pltpu.SemaphoreType.DMA((6,)),
            pltpu.SemaphoreType.DMA((3,)),
            pltpu.SemaphoreType.DMA((2,)),
            pltpu.SemaphoreType.DMA,
        ],
        compiler_params=pltpu.CompilerParams(
            vmem_limit_bytes=126 * 1024 * 1024, disable_bounds_checks=True, flags=FLAGS),
    )(
        A_x.reshape(NSEG, SEG, DM),
        A_mem0.reshape(MEM, DM),
        _by_head_group(A_Wq),
        _by_head_group(A_Wk),
        _by_head_group(A_Wv),
        A_Wo.reshape(HEADS * HD, DM),
        B_w_r.reshape(8, 128),
        B_w_gate,
        B_w_up,
        B_w_down,
        gate_w.reshape(8, 128),
    )
    return out.reshape(1, SEQ, DM)
```

```python
import functools

import jax
import jax.numpy as jnp
import numpy as np
from jax import lax
from jax.experimental import pallas as pl
from jax.experimental.pallas import tpu as pltpu

F32, BF16, U32, I32 = jnp.float32, jnp.bfloat16, jnp.uint32, jnp.int32

SEQ, DM, HEADS, HD = 2048, 1024, 32, 128
MEM, SEG, TOPK, FF = 8, 32, 8, 3584
NSEG = SEQ // SEG
NT = DM // 128
NC = NT // 2
NPAIR = HEADS // 2
NGROUP = HEADS // 8
NFP = FF // 256
SROWS = NSEG * 8
ROWS = 64
UNROLL = 4
SEG_OUT = 32
Q, K, V = 0, 1, 2


def _mm(a, b):
    return jnp.dot(a, b, preferred_element_type=F32)


def _tile(i):
    return slice(i * 128, (i + 1) * 128)


def _window(first, count, unit):
    start = first * unit
    return pl.ds(start if isinstance(start, int) else pl.multiple_of(start, unit), count * unit)


def _block(n, size):
    return _window(n, 1, size)


def _weight_blocks(b11, b12, b21, b22):
    resident = [b11, b21 - b11, b12 - b22, b22]
    alone = [b11 + b22, b11 + b12, b21 + b22]
    return resident, alone


def _resident_lhs(m1, m2, z1, z2):
    ms, zs = m1 + m2, z1 + z2
    parts = ((ms, zs[24:32], zs[0:16]), (m2, z2[24:32], z2[0:16]),
             (m1, z1[16:24], z1[0:16]), (ms, zs[16:24], zs[0:16]))
    return [jnp.concatenate(p, axis=0).astype(BF16) for p in parts]


def _alone_lhs(a11, a12, a21, a22):
    return [a11 + a22, a21 - a11, a12 - a22]


def _row_dot(tiles, w_ref):
    w = w_ref[...].astype(F32)
    acc = tiles[0] * w[0:1]
    for t in range(1, NT):
        acc = acc + tiles[t] * w[t:t + 1]
    return jnp.sum(acc, axis=1, keepdims=True)


def _kernel(x_hbm, mem_hbm, wq_hbm, wk_hbm, wv_hbm, wo_hbm, wr_hbm, wg_hbm,
            wu_hbm, wd_hbm, gw_hbm, out_hbm,
            vecs, xbuf, mem_v, stage, wo_raw, xl_u, wres_u, wores_u, woalone_u,
            dbuf, lhs_u, olhs_u, oalone_u, mixed, gate, ffw, out_v, chosen,
            sem_w, sem_g, sem_x, sem_o, sem_s, sem_f, sem_out):
    xl = xl_u.bitcast(BF16)
    wres = wres_u.bitcast(BF16)
    wores = wores_u.bitcast(BF16)
    woalone = woalone_u.bitcast(BF16)
    lhs = lhs_u.bitcast(BF16)
    olhs = olhs_u.bitcast(BF16)
    oalone = oalone_u.bitcast(BF16)
    stage32 = stage.bitcast(U32)

    wr_v, gw_v = vecs.at[0:8], vecs.at[16:24]
    zero = jnp.zeros((8, 128), F32)
    lane = lax.broadcasted_iota(I32, (8, 128), 1)
    sub = lax.broadcasted_iota(I32, (8, 128), 0)

    staged = stage.at[:, :, pl.ds(0, 2048)]

    def w_start(w, c, sems=None):
        for g in range(NGROUP):
            pltpu.make_async_copy(
                (wq_hbm, wk_hbm, wv_hbm)[w].at[_block(c, 2048), _tile(g)],
                staged.at[w, g], sem_w.at[w] if sems is None else sems.at[g]).start()

    def w_wait(w):
        pltpu.make_async_copy(staged.at[w], staged.at[w], sem_w.at[w]).wait()

    def x_copy(n, segs, rows, cols):
        return pltpu.make_async_copy(
            x_hbm.at[segs, rows, cols], xbuf.at[segs, rows, cols], sem_x.at[n])

    every = slice(None)
    x_first = x_copy(0, every, pl.ds(16, 16), pl.ds(0, 256))
    x_rest = x_copy(1, every, pl.ds(0, 16), pl.ds(0, 256))
    x_second = x_copy(2, every, every, pl.ds(256, 256))

    def x_right(h):
        return x_copy(3 + h, _block(h, NSEG // 2), every, pl.ds(512, 512))

    def wo_copy(p, pairs=3):
        rows = _window(3 * p, pairs, 2 * HD)
        return pltpu.make_async_copy(wo_hbm.at[rows], wo_raw.at[rows], sem_o.at[p])

    def ff_start(f):
        dst, sem = ffw.at[f & 1], sem_f.at[f & 1]
        for h in range(2):
            for n, src in enumerate((wg_hbm, wu_hbm)):
                pltpu.make_async_copy(src.at[:, _block(f * 2 + h, 128)],
                                      dst.at[_block(2 * n + h, DM)], sem).start()
        for t in range(NT):
            pltpu.make_async_copy(wd_hbm.at[_block(f, 256), _tile(t)],
                                  dst.at[pl.ds(4 * DM + t * 256, 256)], sem).start()

    def ff_wait(f):
        pltpu.make_async_copy(ffw.at[f & 1], ffw.at[f & 1], sem_f.at[f & 1]).wait()

    small = [pltpu.make_async_copy(src, dst, sem_s.at[n]) for n, (src, dst) in enumerate(
        ((mem_hbm, mem_v), (wr_hbm, wr_v), (gw_hbm, gw_v)))]

    def x_blocks(c):
        src, dst = xbuf.at[:, :, _block(c, 256)], xl.at[c]
        for n in range(NSEG // 2):
            got = []
            for s in (2 * n, 2 * n + 1):
                z1, z2 = [src[s, 16:32, _tile(h)].astype(F32) for h in range(2)]
                got.append(_alone_lhs(z1[0:8], z2[0:8], z1[8:16], z2[8:16]))
            for t in range(3):
                dst[pl.ds(n * 16, 16), _tile(t)] = jnp.concatenate(
                    [got[0][t], got[1][t]], axis=0).astype(BF16)

    def qkv_blocks(raw, res, j):
        raw = raw.at[j // 4]
        even = lambda z: pltpu.bitcast(z << 16, F32)
        odd = lambda z: pltpu.bitcast(z & np.uint32(0xFFFF0000), F32)
        rest = []
        for r in range(112, -16, -16):
            h1 = raw[pl.ds(4 * r + j % 4, 16, stride=4), :]
            h2 = raw[pl.ds(4 * (128 + r) + j % 4, 16, stride=4), :]
            resident, alone = _weight_blocks(even(h1), odd(h1), even(h2), odd(h2))
            res.at[j][pl.ds(r, 16), :] = jnp.concatenate(resident, axis=1).astype(BF16)
            rest.insert(0, alone)
        return tuple(jnp.concatenate(a, axis=0).astype(BF16) for a in zip(*rest))

    def wo_views(first, pairs):
        return (wo_raw.at[_window(first, pairs, 2 * HD)], wores.at[:, _window(first, pairs, HD)],
                woalone.at[:, _window(first, pairs, HD)])

    def wo_blocks(views, j, c, r, pace):
        raw, res, rest = views
        b11, b12, b21, b22 = [
            raw[pl.ds((2 * j + head) * HD + r, 16), _tile(2 * c + h)].astype(F32)
            for head in range(2) for h in range(2)]
        resident, alone = _weight_blocks(pace(b11), b12, b21, b22)
        res.at[c][pl.ds(j * HD + r, 16), :] = jnp.concatenate(resident, axis=1).astype(BF16)
        rest.at[c][pl.ds(j * HD + r, 16), :] = jnp.concatenate(alone, axis=1).astype(BF16)

    def router_scores(x_v, n, scores, pace):
        rows = pl.ds(16 * (n % 2), 16)
        xs = [x_v[n // 2, rows, _tile(t)].astype(F32) for t in range(NT)]
        r = _row_dot([pace(xs[0])] + xs[1:], wr_v)
        for i in range(2):
            scores = jnp.where(lane == 2 * n + i, r[8 * i:8 * i + 8], scores)
        return scores

    def select_tokens(scores):
        keys = []
        for h, r in enumerate(scores):
            r = r.astype(BF16).astype(F32)
            bits = pltpu.bitcast(jnp.where(r == 0.0, 0.0, r), I32) >> 16
            order = jnp.where(r != r, 0, jnp.where(bits < 0, ~bits, bits + 0x8000))
            token = (h * 128 + lane) * 8 + sub
            keys.append(pltpu.bitcast((1 << 29) + (order << 11) + (SEQ - 1 - token), F32))
        tiles = [zero] * NT
        for n in range(TOPK):
            top = jnp.max(jnp.maximum(keys[0], keys[1]), axis=0, keepdims=True)
            top = jnp.max(top, axis=1, keepdims=True)
            keys = [jnp.where(k == top, 0.0, k) for k in keys]
            low = pltpu.bitcast(jnp.broadcast_to(top, (8, 128)), I32)[0, 0] & (SEQ - 1)
            token = SEQ - 1 - low
            chosen[n] = token
            rows = xbuf[token >> 5, pl.ds(pl.multiple_of(token & 24, 8), 8), :].astype(F32)
            rows = pltpu.roll(rows, (n - token) & 7, 0)
            tiles = [jnp.where(sub == n, rows[:, _tile(t)], z) for t, z in enumerate(tiles)]
        r, g = [jax.nn.sigmoid(_row_dot(tiles, v)) for v in (wr_v, gw_v)]
        return jnp.concatenate(tiles, axis=1), jnp.broadcast_to(r * (1.0 - g), (8, 128))

    def qkv_chunk(w, c, group, groups, never, extra=None):
        pairs = pl.ds(w * NPAIR + 4 * group, 4 * groups)
        raw = stage32.at[w, pl.ds(group, groups)]
        res, sums = wres.at[pairs, _block(c, 128)], dbuf.at[pairs]
        alone = qkv_blocks(raw, res, 0)
        for j in range(4 * groups):
            ahead = qkv_blocks(raw, res, j + 1) if j + 1 < 4 * groups else None
            for n in range(SROWS // ROWS):
                rows = _block(n, ROWS)
                ops = [xl.at[c][rows, _tile(t)] for t in range(3)]
                if ahead is not None:
                    r = 128 - 16 * min(n + 2, 8)
                    ops[0] = jnp.concatenate(
                        [jnp.where(never, ahead[0][r:r + 16], ops[0][:16]), ops[0][16:]], axis=0)
                m1, m6, m7 = [_mm(ops[t], alone[t]) for t in range(3)]
                for t, d in enumerate((m1 + m7, m1 + m6)):
                    if not isinstance(c, int):
                        d = d + jnp.where(c > 0, sums[j, rows, _tile(t)], 0.0)
                    elif c > 0:
                        d = d + sums[j, rows, _tile(t)]
                    sums[j, rows, _tile(t)] = d
                if extra is not None:
                    extra(j * (SROWS // ROWS) + n, m1)
            alone = ahead

    x_first.start()
    w_start(Q, 0, sem_g)
    w_start(K, 0)
    w_start(V, 0)
    x_first.wait()
    for cp in [x_second, x_rest] + small:
        cp.start()
    x_blocks(0)

    def first(g, carry):
        pltpu.make_async_copy(staged.at[Q, g], staged.at[Q, g], sem_g.at[g]).wait()
        qkv_chunk(Q, 0, g, 1, g < 0)
        return carry

    lax.fori_loop(0, NGROUP, first, 0)
    w_start(Q, 1)

    def early(i, carry):
        c, w = carry
        w_wait(w)

        @pl.when(i == 3)
        def _():
            x_second.wait()

        @pl.when(i == 6)
        def _():
            x_right(0).wait()
            x_right(1).wait()

        @pl.when((i == 2) | (i == 3))
        def _():
            x_right(jnp.clip(i - 2, 0, 1)).start()

        @pl.when(i >= 4)
        def _():
            wo_copy(jnp.maximum(i - 4, 0)).start()

        @pl.when(w == 0)
        def _():
            x_blocks(c)

        qkv_chunk(w, c, 0, NGROUP, i < 0)
        for n in (Q, K, V):
            @pl.when(w == n)
            def _():
                w_start(n, c + 1)

        return jnp.where(w == V, c + 1, c), jnp.where(w == V, Q, w + 1)

    lax.fori_loop(1, 3 * (NC - 1), early, (0, K))

    for cp in [x_rest, wo_copy(0)] + small:
        cp.wait()
    wo_copy(5, 1).start()
    ff_start(0)
    x_blocks(NC - 1)

    def last(w, carry):
        scores, fresh = carry[0], [zero]
        w_wait(w)
        wo_copy(jnp.minimum(w + 1, 2) + w).wait()

        @pl.when(w == 1)
        def _():
            wo_copy(2).wait()

        x_v = xbuf.at[_block(jnp.minimum(w, 1), NSEG // 2)]
        todo = [(j, c, r) for j in range(5) for c in range(NC) for r in range(0, HD, 16)]
        slots = NPAIR * SROWS // ROWS - 2
        views = wo_views(5 * w, 5)

        def extra(n, m):
            pace = lambda z: jnp.where(w < 0, m[:16], z)
            for item in todo[len(todo) * n // slots:len(todo) * (n + 1) // slots]:
                wo_blocks(views, *item, pace)
            for g in range(NSEG * n // slots, min(NSEG * (n + 1) // slots, NSEG)):
                fresh[0] = router_scores(x_v, g, fresh[0], pace)

        picked = select_tokens(scores)
        qkv_chunk(w, NC - 1, 0, NGROUP, w < 0, extra)
        return (jnp.where(w == 0, fresh[0], scores[0]), fresh[0]), picked

    _, (xsel, weight) = lax.fori_loop(
        0, 3, last, ((zero, zero), (jnp.zeros((TOPK, DM), F32), zero)))

    wo_copy(5, 1).wait()
    ff_wait(0)
    for c in range(NC):
        for r in range(0, HD, 16):
            wo_blocks(wo_views(NPAIR - 1, 1), 0, c, r, lambda z: z)

    qi = lax.broadcasted_iota(I32, (MEM + SEG, MEM + SEG), 0)
    ki = lax.broadcasted_iota(I32, (MEM + SEG, MEM + SEG), 1)
    visible = (qi < MEM) | (qi >= ki)

    def attend(q, k):
        sc = lax.dot_general(q, k, (((1,), (1,)), ((), ())), preferred_element_type=F32)
        sc = jnp.where(visible, sc * HD ** -0.5, -1000000000.0)
        e = jnp.exp(sc - jnp.max(sc, axis=1, keepdims=True))
        total = jnp.sum(e, axis=1, keepdims=True)
        inv = pltpu.reciprocal(total, approx=True)
        return e, inv * (2.0 - total * inv)

    def segment(views, s, mem, held, due, filler, never):
        x_v, sums, ops_out, mix, gates = views
        r8, r32 = _block(s, 8), _block(s, SEG)
        xs = [jnp.where(never, 1.0, x_v[s, :, _tile(t)].astype(F32)) for t in range(NT)]
        for c in range(NC):
            ops = _resident_lhs(mem[2 * c], mem[2 * c + 1], xs[2 * c], xs[2 * c + 1])
            for t in range(4):
                lhs.at[t][:, _tile(c)] = ops[t]
        g = jnp.broadcast_to(jax.nn.sigmoid(_row_dot(xs, gw_v)), (SEG, 128))
        gates[_block(s, 16), :] = g[16:32]

        def on_time(z):
            for _ in range(min(len(due), 3)):
                z = jnp.where(never, due.pop(0), z)
            return z

        def products(w, j, k):
            m = {t: _mm(lhs.at[t][:, k], wres.at[w * NPAIR + j][k, _tile(t)]) for t in (2, 3, 0, 1)}
            return [m[t] for t in range(4)]

        def project(w, j, head=None):
            if head is None:
                m2, m4, m3, m5 = products(w, j, slice(0, NC * 128))
            else:
                m2, m4, m3, m5 = [b + a for a, b in zip(head, products(w, j, _tile(NC - 1)))]
            left, right = m2 + m4, m3 + m5
            c11 = m4[8:16] - m5[8:16] + on_time(sums[w * NPAIR + j, r8, _tile(0)])
            c22 = m3[8:16] - m2[8:16] + on_time(sums[w * NPAIR + j, r8, _tile(1)])
            both = (jnp.concatenate([left[0:8], left[16:32], c11, left[8:16]], axis=0),
                    jnp.concatenate([right[0:8], right[16:32], right[8:16], c22], axis=0))
            return both if w == Q else [z.astype(BF16) for z in both]

        keep, acc, new_mem, results = {}, {}, [], []

        def values(j, p, v):
            oe, oo = [_mm(e * inv, vh) for (e, inv), vh in zip(p, v)]
            ops = _resident_lhs(oe[0:8], oo[0:8], oe[8:40], oo[8:40])
            for t in range(4):
                olhs.at[t][:, _tile(j)] = ops[t]
            alone = _alone_lhs(oe[24:32], oo[24:32], oe[32:40], oo[32:40])
            if held is None:
                keep[j] = alone
            else:
                for t in range(3):
                    ops_out.at[t][pl.ds((s - 1) * 8, 16), _tile(j)] = jnp.concatenate(
                        [held[j][t], alone[t]], axis=0).astype(BF16)

        def out_part(c, j0, j1):
            k = slice(j0 * HD, j1 * HD)
            m4, m2, m3, m5 = [
                _mm(olhs.at[t][:, k], wores.at[c][k, _tile(t)]) for t in (1, 0, 2, 3)]
            new = [m2 + m4, m3 + m5, m4[8:16] - m5[8:16], m3[8:16] - m2[8:16]]
            acc[c] = [a + b for a, b in zip(acc[c], new)] if c in acc else new

        def out_done(c):
            left, right, c11, c22 = acc[c]
            new_mem.extend((left[0:8], right[0:8]))
            parts = ((left[16:32], c11, left[8:16]), (right[16:32], right[8:16], c22))
            for t, a in zip((2 * c, 2 * c + 1), parts):
                z = g * jnp.concatenate(a, axis=0) + (1.0 - g) * x_v[s, :, _tile(t)].astype(F32)
                mix[r32, _tile(t)] = z
                results.extend(z[n:n + 8] for n in range(0, SEG, 8))

        heads = {j: products(K, j, slice(0, (NC - 1) * 128)) for j in range(2)}
        pending = []
        for j in range(0, NPAIR, 2):
            k0, k1 = project(K, j, heads.get(j)), project(K, j + 1, heads.get(j + 1))
            filler(j // 2)
            for item in pending:
                values(*item)
            q0, q1 = project(Q, j), project(Q, j + 1)
            v0 = project(V, j)
            p0 = [attend(q, k) for q, k in zip(q0, k0)]
            p1 = [attend(q, k) for q, k in zip(q1, k1)]
            pending = [(j, p0, v0), (j + 1, p1, project(V, j + 1))]
        split = 10
        out_part(0, 0, split)
        for item in pending:
            values(*item)
        out_part(1, 0, split)
        for c in range(NC):
            out_part(c, split if c < 2 else 0, NPAIR)
            out_done(c)
        return new_mem, keep or None, results

    def trip(i, carry):
        mem, y = list(carry[0]), list(carry[1])

        @pl.when(i + 1 < NFP)
        def _():
            ff_start(jnp.minimum(i + 1, NFP - 1))

        weights, hidden = ffw.at[jnp.minimum(i, NFP - 1) & 1], {}
        slot = {1: 0, 2: 1, 4: 2, 6: 3}

        def ff_in(m):
            def fill(n):
                if n in slot:
                    u, k = 2 * m + slot[n] // 2, slot[n] % 2 * 512
                    part = _mm(xsel[:, k:k + 512], weights[pl.ds(u * DM + k, 512), :])
                    hidden[u] = part if k == 0 else part + hidden[u]
            return fill

        def ff_out(n):
            if n in slot:
                act = jnp.concatenate(
                    [jax.nn.silu(hidden[h]) * hidden[2 + h] for h in range(2)], axis=1)
                for t in (2 * slot[n], 2 * slot[n] + 1):
                    part = _mm(act, weights[pl.ds(4 * DM + t * 256, 256), :])
                    y[t] = y[t] + jnp.where(i < NFP, part, 0.0)

        views = (xbuf.at[_block(i, UNROLL)], dbuf.at[:, _block(i, UNROLL * 8)],
                 oalone.at[:, _block(i, UNROLL * 8)], mixed.at[_block(i, UNROLL * SEG)],
                 gate.at[_block(i, UNROLL * 16)])
        held, due = None, []
        for s, fill in enumerate((lambda n: None, ff_in(0), ff_in(1), ff_out)):
            mem, held, due = segment(views, s, mem, held, due, fill, i < 0)

        @pl.when(i + 1 < NFP)
        def _():
            ff_wait(i + 1)

        return tuple(mem), tuple(y)

    mem0 = tuple(mem_v[:, _tile(t)].astype(F32) for t in range(NT))
    _, y = lax.fori_loop(0, NSEG // UNROLL, trip, (mem0, (zero,) * NT))
    y = jnp.concatenate([part * weight for part in y], axis=1)
    for n in range(TOPK):
        mixed[pl.ds(chosen[n], 1), :] += y[n:n + 1]

    def finish(n, carry):
        ops = oalone.at[:, _block(n, SEG_OUT * 8)]
        mix = mixed.at[_block(n, SEG_OUT * SEG)]
        gates = gate.at[_block(n, SEG_OUT * 16)]
        outs = out_v.at[_block(n, SEG_OUT * SEG)]
        done = []
        for c in range(NC):
            for r in range(0, SEG_OUT * 8, ROWS):
                left = [ops.at[t][pl.ds(r, ROWS), :] for t in range(3)]
                if done:
                    late = jnp.concatenate(done, axis=1)
                    for t, part in ((2, late[:, :NPAIR * HD]), (1, late[:, NPAIR * HD:])):
                        left[t] = jnp.concatenate(
                            [jnp.where(n < 0, part, left[t][:16]), left[t][16:]], axis=0)
                done = []
                m1, m7, m6 = [_mm(left[t], woalone.at[c][:, _tile(t)]) for t in (0, 2, 1)]
                d11, d22 = m1 + m7, m1 + m6
                for i in range(ROWS // 8):
                    s = r // 8 + i
                    g = gates[_block(s, 16), :]
                    zl, zr = [mix[_block(s, SEG), _tile(2 * c + h)] for h in range(2)]
                    zl = [zl[0:16], zl[16:24] + g[0:8] * d11[8 * i:8 * i + 8], zl[24:32]]
                    zr = [zr[0:24], zr[24:32] + g[8:16] * d22[8 * i:8 * i + 8]]
                    for h, z in enumerate((zl, zr)):
                        z = jnp.concatenate(z, axis=0).astype(BF16)
                        outs[_block(s, SEG), _tile(2 * c + h)] = z
                        done += [z[16:], z[:16]]
                where = (_window(n * SEG_OUT + r // 8, ROWS // 8, SEG), _block(c, 256))
                pltpu.make_async_copy(out_v.at[where], out_hbm.at[where], sem_out).start()
        return carry

    lax.fori_loop(0, NSEG // SEG_OUT, finish, 0)
    pltpu.make_async_copy(out_v, out_hbm, sem_out).wait()


def _by_head_group(w):
    return w.reshape(DM, NGROUP, 8, HD).transpose(0, 2, 1, 3).reshape(DM * 8, NGROUP * HD)


@functools.partial(jax.jit, static_argnames=("A_seg_len",))
def pallas_gated_mix__memory_aug_recurrent_mem_tr__moe_arch_mod__prompt_kernel(
    A_x: jax.Array,
    A_mem0: jax.Array,
    A_Wq: jax.Array,
    A_Wk: jax.Array,
    A_Wv: jax.Array,
    A_Wo: jax.Array,
    A_seg_len: int,
    B_x: jax.Array,
    B_w_r: jax.Array,
    B_w_gate: jax.Array,
    B_w_up: jax.Array,
    B_w_down: jax.Array,
    gate_w: jax.Array,
):
    del B_x
    assert A_seg_len == SEG and A_x.shape == (1, SEQ, DM) and A_mem0.shape == (1, MEM, DM)
    assert A_Wq.shape == (DM, HEADS, HD) and B_w_gate.shape == (DM, FF)

    hbm = pl.BlockSpec(memory_space=pl.ANY)
    out = pl.pallas_call(
        _kernel,
        out_shape=jax.ShapeDtypeStruct((SEQ, DM), BF16),
        in_specs=[hbm] * 11,
        out_specs=hbm,
        scratch_shapes=[
            pltpu.VMEM((48, 128), BF16),
            pltpu.VMEM((NSEG, SEG, DM), BF16),
            pltpu.VMEM((MEM, DM), BF16),
            pltpu.VMEM((3, NGROUP, 2048 + 64, HD), BF16),
            pltpu.VMEM((HEADS * HD, DM), BF16),
            pltpu.VMEM((NC, SROWS // 2, 3 * 128), U32),
            pltpu.VMEM((3 * NPAIR, NC * 64, 4 * 128), U32),
            pltpu.VMEM((NC, NPAIR * 64, 4 * 128), U32),
            pltpu.VMEM((NC, NPAIR * 64, 3 * 128), U32),
            pltpu.VMEM((3 * NPAIR, SROWS, 2 * 128), F32),
            pltpu.VMEM((4, 16, NC * 128), U32),
            pltpu.VMEM((4, 16, NPAIR * HD), U32),
            pltpu.VMEM((3, SROWS // 2, NPAIR * HD), U32),
            pltpu.VMEM((SEQ, DM), F32),
            pltpu.VMEM((SEQ // 2, 128), F32),
            pltpu.VMEM((2, 6 * DM, 128), BF16),
            pltpu.VMEM((SEQ, DM), BF16),
            pltpu.SMEM((TOPK,), I32),
            pltpu.SemaphoreType.DMA((3,)),
            pltpu.SemaphoreType.DMA((NGROUP,)),
            pltpu.SemaphoreType.DMA((5,)),
            pltpu.SemaphoreType.DMA((6,)),
            pltpu.SemaphoreType.DMA((3,)),
            pltpu.SemaphoreType.DMA((2,)),
            pltpu.SemaphoreType.DMA,
        ],
        compiler_params=pltpu.CompilerParams(
            vmem_limit_bytes=126 * 1024 * 1024, disable_bounds_checks=True),
    )(
        A_x.reshape(NSEG, SEG, DM),
        A_mem0.reshape(MEM, DM),
        _by_head_group(A_Wq),
        _by_head_group(A_Wk),
        _by_head_group(A_Wv),
        A_Wo.reshape(HEADS * HD, DM),
        B_w_r.reshape(8, 128),
        B_w_gate,
        B_w_up,
        B_w_down,
        gate_w.reshape(8, 128),
    )
    return out.reshape(1, SEQ, DM)
```

```python
import functools

import jax
import jax.numpy as jnp
import numpy as np
from jax import lax
from jax.experimental import pallas as pl
from jax.experimental.pallas import tpu as pltpu

F32, BF16, U32, I32 = jnp.float32, jnp.bfloat16, jnp.uint32, jnp.int32

SEQ, DM, HEADS, HD = 2048, 1024, 32, 128
MEM, SEG, TOPK, FF = 8, 32, 8, 3584
NSEG = SEQ // SEG
NT = DM // 128
NC = NT // 2
NPAIR = HEADS // 2
NGROUP = HEADS // 8
NFP = FF // 256
SROWS = NSEG * 8
ROWS = 64
UNROLL = 4
SEG_OUT = 32
Q, K, V = 0, 1, 2


def _mm(a, b):
    return jnp.dot(a, b, preferred_element_type=F32)


def _tile(i):
    return slice(i * 128, (i + 1) * 128)


def _window(first, count, unit):
    start = first * unit
    return pl.ds(start if isinstance(start, int) else pl.multiple_of(start, unit), count * unit)


def _block(n, size):
    return _window(n, 1, size)


def _weight_blocks(b11, b12, b21, b22):
    resident = [b11, b21 - b11, b12 - b22, b22]
    alone = [b11 + b22, b11 + b12, b21 + b22]
    return resident, alone


def _resident_lhs(m1, m2, z1, z2):
    ms, zs = m1 + m2, z1 + z2
    parts = ((ms, zs[24:32], zs[0:16]), (m2, z2[24:32], z2[0:16]),
             (m1, z1[16:24], z1[0:16]), (ms, zs[16:24], zs[0:16]))
    return [jnp.concatenate(p, axis=0).astype(BF16) for p in parts]


def _alone_lhs(a11, a12, a21, a22):
    return [a11 + a22, a21 - a11, a12 - a22]


def _row_dot(tiles, w_ref):
    w = w_ref[...].astype(F32)
    acc = tiles[0] * w[0:1]
    for t in range(1, NT):
        acc = acc + tiles[t] * w[t:t + 1]
    return jnp.sum(acc, axis=1, keepdims=True)


def _kernel(x_hbm, mem_hbm, wq_hbm, wk_hbm, wv_hbm, wo_hbm, wr_hbm, wg_hbm,
            wu_hbm, wd_hbm, gw_hbm, out_hbm,
            vecs, xbuf, mem_v, stage, wo_raw, xl_u, wres_u, wores_u, woalone_u,
            dbuf, lhs_u, olhs_u, oalone_u, mixed, gate, ffw, out_v, chosen,
            sem_w, sem_g, sem_x, sem_o, sem_s, sem_f, sem_out):
    xl = xl_u.bitcast(BF16)
    wres = wres_u.bitcast(BF16)
    wores = wores_u.bitcast(BF16)
    woalone = woalone_u.bitcast(BF16)
    lhs = lhs_u.bitcast(BF16)
    olhs = olhs_u.bitcast(BF16)
    oalone = oalone_u.bitcast(BF16)
    stage32 = stage.bitcast(U32)

    wr_v, gw_v = vecs.at[0:8], vecs.at[16:24]
    zero = jnp.zeros((8, 128), F32)
    lane = lax.broadcasted_iota(I32, (8, 128), 1)
    sub = lax.broadcasted_iota(I32, (8, 128), 0)

    staged = stage.at[:, :, pl.ds(0, 2048)]

    def w_start(w, c, sems=None):
        for g in range(NGROUP):
            pltpu.make_async_copy(
                (wq_hbm, wk_hbm, wv_hbm)[w].at[_block(c, 2048), _tile(g)],
                staged.at[w, g], sem_w.at[w] if sems is None else sems.at[g]).start()

    def w_wait(w):
        pltpu.make_async_copy(staged.at[w], staged.at[w], sem_w.at[w]).wait()

    def x_copy(n, segs, rows, cols):
        return pltpu.make_async_copy(
            x_hbm.at[segs, rows, cols], xbuf.at[segs, rows, cols], sem_x.at[n])

    every = slice(None)
    x_first = x_copy(0, every, pl.ds(16, 16), pl.ds(0, 256))
    x_rest = x_copy(1, every, pl.ds(0, 16), pl.ds(0, 256))
    x_second = x_copy(2, every, every, pl.ds(256, 256))

    def x_right(h):
        return x_copy(3 + h, _block(h, NSEG // 2), every, pl.ds(512, 512))

    def wo_copy(p, first=None, pairs=3):
        rows = _window(3 * p if first is None else first, pairs, 2 * HD)
        return pltpu.make_async_copy(wo_hbm.at[rows], wo_raw.at[rows], sem_o.at[p])

    wo_late, wo_last = wo_copy(4, 12, 2), wo_copy(5, 14, 2)

    def ff_start(f):
        dst, sem = ffw.at[f & 1], sem_f.at[f & 1]
        for h in range(2):
            for n, src in enumerate((wg_hbm, wu_hbm)):
                pltpu.make_async_copy(src.at[:, _block(f * 2 + h, 128)],
                                      dst.at[_block(2 * n + h, DM)], sem).start()
        for t in range(NT):
            pltpu.make_async_copy(wd_hbm.at[_block(f, 256), _tile(t)],
                                  dst.at[pl.ds(4 * DM + t * 256, 256)], sem).start()

    def ff_wait(f):
        pltpu.make_async_copy(ffw.at[f & 1], ffw.at[f & 1], sem_f.at[f & 1]).wait()

    small = [pltpu.make_async_copy(src, dst, sem_s.at[n]) for n, (src, dst) in enumerate(
        ((mem_hbm, mem_v), (wr_hbm, wr_v), (gw_hbm, gw_v)))]

    def x_blocks(c):
        src, dst = xbuf.at[:, :, _block(c, 256)], xl.at[c]
        for n in range(NSEG // 2):
            got = []
            for s in (2 * n, 2 * n + 1):
                z1, z2 = [src[s, 16:32, _tile(h)].astype(F32) for h in range(2)]
                got.append(_alone_lhs(z1[0:8], z2[0:8], z1[8:16], z2[8:16]))
            for t in range(3):
                dst[pl.ds(n * 16, 16), _tile(t)] = jnp.concatenate(
                    [got[0][t], got[1][t]], axis=0).astype(BF16)

    def qkv_blocks(raw, res, j):
        raw = raw.at[j // 4]
        even = lambda z: pltpu.bitcast(z << 16, F32)
        odd = lambda z: pltpu.bitcast(z & np.uint32(0xFFFF0000), F32)
        rest = []
        for r in range(112, -16, -16):
            h1 = raw[pl.ds(4 * r + j % 4, 16, stride=4), :]
            h2 = raw[pl.ds(4 * (128 + r) + j % 4, 16, stride=4), :]
            resident, alone = _weight_blocks(even(h1), odd(h1), even(h2), odd(h2))
            res.at[j][pl.ds(r, 16), :] = jnp.concatenate(resident, axis=1).astype(BF16)
            rest.insert(0, alone)
        return tuple(jnp.concatenate(a, axis=0).astype(BF16) for a in zip(*rest))

    def wo_views(first, pairs):
        return (wo_raw.at[_window(first, pairs, 2 * HD)], wores.at[:, _window(first, pairs, HD)],
                woalone.at[:, _window(first, pairs, HD)])

    def wo_blocks(views, j, c, r, pace):
        raw, res, rest = views
        b11, b12, b21, b22 = [
            raw[pl.ds((2 * j + head) * HD + r, 16), _tile(2 * c + h)].astype(F32)
            for head in range(2) for h in range(2)]
        resident, alone = _weight_blocks(pace(b11), b12, b21, b22)
        res.at[c][pl.ds(j * HD + r, 16), :] = jnp.concatenate(resident, axis=1).astype(BF16)
        rest.at[c][pl.ds(j * HD + r, 16), :] = jnp.concatenate(alone, axis=1).astype(BF16)

    def router_scores(x_v, n, scores, pace):
        rows = pl.ds(16 * (n % 2), 16)
        xs = [x_v[n // 2, rows, _tile(t)].astype(F32) for t in range(NT)]
        r = _row_dot([pace(xs[0])] + xs[1:], wr_v)
        for i in range(2):
            scores = jnp.where(lane == 2 * n + i, r[8 * i:8 * i + 8], scores)
        return scores

    def select_tokens(scores):
        keys = []
        for h, r in enumerate(scores):
            r = r.astype(BF16).astype(F32)
            bits = pltpu.bitcast(jnp.where(r == 0.0, 0.0, r), I32) >> 16
            order = jnp.where(r != r, 0, jnp.where(bits < 0, ~bits, bits + 0x8000))
            token = (h * 128 + lane) * 8 + sub
            keys.append(pltpu.bitcast((1 << 29) + (order << 11) + (SEQ - 1 - token), F32))
        tiles = [zero] * NT
        for n in range(TOPK):
            top = jnp.max(jnp.maximum(keys[0], keys[1]), axis=0, keepdims=True)
            top = jnp.max(top, axis=1, keepdims=True)
            keys = [jnp.where(k == top, 0.0, k) for k in keys]
            low = pltpu.bitcast(jnp.broadcast_to(top, (8, 128)), I32)[0, 0] & (SEQ - 1)
            token = SEQ - 1 - low
            chosen[n] = token
            rows = xbuf[token >> 5, pl.ds(pl.multiple_of(token & 24, 8), 8), :].astype(F32)
            rows = pltpu.roll(rows, (n - token) & 7, 0)
            tiles = [jnp.where(sub == n, rows[:, _tile(t)], z) for t, z in enumerate(tiles)]
        r, g = [jax.nn.sigmoid(_row_dot(tiles, v)) for v in (wr_v, gw_v)]
        return jnp.concatenate(tiles, axis=1), jnp.broadcast_to(r * (1.0 - g), (8, 128))

    def qkv_chunk(w, c, group, groups, never, extra=None):
        pairs = pl.ds(w * NPAIR + 4 * group, 4 * groups)
        raw = stage32.at[w, pl.ds(group, groups)]
        res, sums = wres.at[pairs, _block(c, 128)], dbuf.at[pairs]
        alone = qkv_blocks(raw, res, 0)
        for j in range(4 * groups):
            ahead = qkv_blocks(raw, res, j + 1) if j + 1 < 4 * groups else None
            for n in range(SROWS // ROWS):
                rows = _block(n, ROWS)
                ops = [xl.at[c][rows, _tile(t)] for t in range(3)]
                if ahead is not None:
                    r = 128 - 16 * min(n + 2, 8)
                    ops[0] = jnp.concatenate(
                        [jnp.where(never, ahead[0][r:r + 16], ops[0][:16]), ops[0][16:]], axis=0)
                m1, m6, m7 = [_mm(ops[t], alone[t]) for t in range(3)]
                for t, d in enumerate((m1 + m7, m1 + m6)):
                    if not isinstance(c, int):
                        d = d + jnp.where(c > 0, sums[j, rows, _tile(t)], 0.0)
                    elif c > 0:
                        d = d + sums[j, rows, _tile(t)]
                    sums[j, rows, _tile(t)] = d
                if extra is not None:
                    extra(j * (SROWS // ROWS) + n, m1)
            alone = ahead

    x_first.start()
    w_start(Q, 0, sem_g)
    w_start(K, 0)
    w_start(V, 0)
    x_first.wait()
    for cp in [x_second, x_rest] + small:
        cp.start()
    x_blocks(0)

    def first(g, carry):
        pltpu.make_async_copy(staged.at[Q, g], staged.at[Q, g], sem_g.at[g]).wait()
        qkv_chunk(Q, 0, g, 1, g < 0)
        return carry

    lax.fori_loop(0, NGROUP, first, 0)
    w_start(Q, 1)

    def early(i, carry):
        c, w = carry
        w_wait(w)

        @pl.when(i == 3)
        def _():
            x_second.wait()

        @pl.when(i == 6)
        def _():
            x_right(0).wait()
            x_right(1).wait()

        @pl.when((i == 2) | (i == 3))
        def _():
            x_right(jnp.clip(i - 2, 0, 1)).start()

        @pl.when((i >= 4) & (i < 8))
        def _():
            wo_copy(jnp.clip(i - 4, 0, 3)).start()

        @pl.when(i == 8)
        def _():
            wo_late.start()

        @pl.when(w == 0)
        def _():
            x_blocks(c)

        qkv_chunk(w, c, 0, NGROUP, i < 0)
        for n in (Q, K, V):
            @pl.when(w == n)
            def _():
                w_start(n, c + 1)

        return jnp.where(w == V, c + 1, c), jnp.where(w == V, Q, w + 1)

    lax.fori_loop(1, 3 * (NC - 1), early, (0, K))

    for cp in [x_rest, wo_copy(0), wo_copy(1)] + small:
        cp.wait()
    wo_last.start()
    ff_start(0)
    x_blocks(NC - 1)

    def last(w, carry):
        scores, fresh = carry[0], [zero]
        w_wait(w)

        @pl.when(w == 1)
        def _():
            wo_copy(2).wait()
            wo_copy(3).wait()

        @pl.when(w == 2)
        def _():
            wo_late.wait()

        x_v = xbuf.at[_block(jnp.minimum(w, 1), NSEG // 2)]
        todo = [(j, c, r) for j in range(5) for c in range(NC) for r in range(0, HD, 16)]
        slots = NPAIR * SROWS // ROWS - 2
        views = wo_views(jnp.minimum(5 * w, 9), 5)

        def extra(n, m):
            pace = lambda z: jnp.where(w < 0, m[:16], z)
            for item in todo[len(todo) * n // slots:len(todo) * (n + 1) // slots]:
                wo_blocks(views, *item, pace)
            for g in range(NSEG * n // slots, min(NSEG * (n + 1) // slots, NSEG)):
                fresh[0] = router_scores(x_v, g, fresh[0], pace)

        picked = select_tokens(scores)
        qkv_chunk(w, NC - 1, 0, NGROUP, w < 0, extra)
        return (jnp.where(w == 0, fresh[0], scores[0]), fresh[0]), picked

    _, (xsel, weight) = lax.fori_loop(
        0, 3, last, ((zero, zero), (jnp.zeros((TOPK, DM), F32), zero)))

    wo_last.wait()
    ff_wait(0)
    for j in range(2):
        for c in range(NC):
            for r in range(0, HD, 16):
                wo_blocks(wo_views(NPAIR - 2, 2), j, c, r, lambda z: z)

    qi = lax.broadcasted_iota(I32, (MEM + SEG, MEM + SEG), 0)
    ki = lax.broadcasted_iota(I32, (MEM + SEG, MEM + SEG), 1)
    visible = (qi < MEM) | (qi >= ki)

    def attend(q, k):
        sc = lax.dot_general(q, k, (((1,), (1,)), ((), ())), preferred_element_type=F32)
        sc = jnp.where(visible, sc * HD ** -0.5, -1000000000.0)
        e = jnp.exp(sc - jnp.max(sc, axis=1, keepdims=True))
        total = jnp.sum(e, axis=1, keepdims=True)
        inv = pltpu.reciprocal(total, approx=True)
        return e, inv * (2.0 - total * inv)

    def segment(views, s, mem, held, due, filler, never):
        x_v, sums, ops_out, mix, gates = views
        r8, r32 = _block(s, 8), _block(s, SEG)
        xs = [jnp.where(never, 1.0, x_v[s, :, _tile(t)].astype(F32)) for t in range(NT)]
        for c in range(NC):
            ops = _resident_lhs(mem[2 * c], mem[2 * c + 1], xs[2 * c], xs[2 * c + 1])
            for t in range(4):
                lhs.at[t][:, _tile(c)] = ops[t]
        g = jnp.broadcast_to(jax.nn.sigmoid(_row_dot(xs, gw_v)), (SEG, 128))
        gates[_block(s, 16), :] = g[16:32]

        def on_time(z):
            for _ in range(min(len(due), 3)):
                z = jnp.where(never, due.pop(0), z)
            return z

        def products(w, j, k):
            m = {t: _mm(lhs.at[t][:, k], wres.at[w * NPAIR + j][k, _tile(t)]) for t in (2, 3, 0, 1)}
            return [m[t] for t in range(4)]

        def project(w, j, head=None):
            if head is None:
                m2, m4, m3, m5 = products(w, j, slice(0, NC * 128))
            else:
                m2, m4, m3, m5 = [b + a for a, b in zip(head, products(w, j, _tile(NC - 1)))]
            left, right = m2 + m4, m3 + m5
            c11 = m4[8:16] - m5[8:16] + on_time(sums[w * NPAIR + j, r8, _tile(0)])
            c22 = m3[8:16] - m2[8:16] + on_time(sums[w * NPAIR + j, r8, _tile(1)])
            both = (jnp.concatenate([left[0:8], left[16:32], c11, left[8:16]], axis=0),
                    jnp.concatenate([right[0:8], right[16:32], right[8:16], c22], axis=0))
            return both if w == Q else [z.astype(BF16) for z in both]

        keep, acc, new_mem, results = {}, {}, [], []

        def values(j, p, v):
            oe, oo = [_mm(e * inv, vh) for (e, inv), vh in zip(p, v)]
            ops = _resident_lhs(oe[0:8], oo[0:8], oe[8:40], oo[8:40])
            for t in range(4):
                olhs.at[t][:, _tile(j)] = ops[t]
            alone = _alone_lhs(oe[24:32], oo[24:32], oe[32:40], oo[32:40])
            if held is None:
                keep[j] = alone
            else:
                for t in range(3):
                    ops_out.at[t][pl.ds((s - 1) * 8, 16), _tile(j)] = jnp.concatenate(
                        [held[j][t], alone[t]], axis=0).astype(BF16)

        def out_part(c, j0, j1):
            k = slice(j0 * HD, j1 * HD)
            m4, m2, m3, m5 = [
                _mm(olhs.at[t][:, k], wores.at[c][k, _tile(t)]) for t in (1, 0, 2, 3)]
            new = [m2 + m4, m3 + m5, m4[8:16] - m5[8:16], m3[8:16] - m2[8:16]]
            acc[c] = [a + b for a, b in zip(acc[c], new)] if c in acc else new

        def out_done(c):
            left, right, c11, c22 = acc[c]
            new_mem.extend((left[0:8], right[0:8]))
            parts = ((left[16:32], c11, left[8:16]), (right[16:32], right[8:16], c22))
            for t, a in zip((2 * c, 2 * c + 1), parts):
                z = g * jnp.concatenate(a, axis=0) + (1.0 - g) * x_v[s, :, _tile(t)].astype(F32)
                mix[r32, _tile(t)] = z
                results.extend(z[n:n + 8] for n in range(0, SEG, 8))

        heads = {j: products(K, j, slice(0, (NC - 1) * 128)) for j in range(2)}
        pending = []
        for j in range(0, NPAIR, 2):
            k0, k1 = project(K, j, heads.get(j)), project(K, j + 1, heads.get(j + 1))
            filler(j // 2)
            for item in pending:
                values(*item)
            q0, q1 = project(Q, j), project(Q, j + 1)
            v0 = project(V, j)
            p0 = [attend(q, k) for q, k in zip(q0, k0)]
            p1 = [attend(q, k) for q, k in zip(q1, k1)]
            pending = [(j, p0, v0), (j + 1, p1, project(V, j + 1))]
        split = 10
        out_part(0, 0, split)
        for item in pending:
            values(*item)
        out_part(1, 0, split)
        for c in range(NC):
            out_part(c, split if c < 2 else 0, NPAIR)
            out_done(c)
        return new_mem, keep or None, results

    def trip(i, carry):
        mem, y = list(carry[0]), list(carry[1])

        @pl.when(i + 1 < NFP)
        def _():
            ff_start(jnp.minimum(i + 1, NFP - 1))

        weights, hidden = ffw.at[jnp.minimum(i, NFP - 1) & 1], {}
        slot = {1: 0, 2: 1, 4: 2, 6: 3}

        def ff_in(m):
            def fill(n):
                if n in slot:
                    u, k = 2 * m + slot[n] // 2, slot[n] % 2 * 512
                    part = _mm(xsel[:, k:k + 512], weights[pl.ds(u * DM + k, 512), :])
                    hidden[u] = part if k == 0 else part + hidden[u]
            return fill

        def ff_out(n):
            if n in slot:
                act = jnp.concatenate(
                    [jax.nn.silu(hidden[h]) * hidden[2 + h] for h in range(2)], axis=1)
                for t in (2 * slot[n], 2 * slot[n] + 1):
                    part = _mm(act, weights[pl.ds(4 * DM + t * 256, 256), :])
                    y[t] = y[t] + jnp.where(i < NFP, part, 0.0)

        views = (xbuf.at[_block(i, UNROLL)], dbuf.at[:, _block(i, UNROLL * 8)],
                 oalone.at[:, _block(i, UNROLL * 8)], mixed.at[_block(i, UNROLL * SEG)],
                 gate.at[_block(i, UNROLL * 16)])
        held, due = None, []
        for s, fill in enumerate((lambda n: None, ff_in(0), ff_in(1), ff_out)):
            mem, held, due = segment(views, s, mem, held, due, fill, i < 0)

        @pl.when(i + 1 < NFP)
        def _():
            ff_wait(i + 1)

        return tuple(mem), tuple(y)

    mem0 = tuple(mem_v[:, _tile(t)].astype(F32) for t in range(NT))
    _, y = lax.fori_loop(0, NSEG // UNROLL, trip, (mem0, (zero,) * NT))
    y = jnp.concatenate([part * weight for part in y], axis=1)
    for n in range(TOPK):
        mixed[pl.ds(chosen[n], 1), :] += y[n:n + 1]

    def finish(n, carry):
        ops = oalone.at[:, _block(n, SEG_OUT * 8)]
        mix = mixed.at[_block(n, SEG_OUT * SEG)]
        gates = gate.at[_block(n, SEG_OUT * 16)]
        outs = out_v.at[_block(n, SEG_OUT * SEG)]
        done = []
        for c in range(NC):
            for r in range(0, SEG_OUT * 8, ROWS):
                left = [ops.at[t][pl.ds(r, ROWS), :] for t in range(3)]
                if done:
                    late = jnp.concatenate(done, axis=1)
                    for t, part in ((2, late[:, :NPAIR * HD]), (1, late[:, NPAIR * HD:])):
                        left[t] = jnp.concatenate(
                            [jnp.where(n < 0, part, left[t][:16]), left[t][16:]], axis=0)
                done = []
                m1, m7, m6 = [_mm(left[t], woalone.at[c][:, _tile(t)]) for t in (0, 2, 1)]
                d11, d22 = m1 + m7, m1 + m6
                for i in range(ROWS // 8):
                    s = r // 8 + i
                    g = gates[_block(s, 16), :]
                    zl, zr = [mix[_block(s, SEG), _tile(2 * c + h)] for h in range(2)]
                    zl = [zl[0:16], zl[16:24] + g[0:8] * d11[8 * i:8 * i + 8], zl[24:32]]
                    zr = [zr[0:24], zr[24:32] + g[8:16] * d22[8 * i:8 * i + 8]]
                    for h, z in enumerate((zl, zr)):
                        z = jnp.concatenate(z, axis=0).astype(BF16)
                        outs[_block(s, SEG), _tile(2 * c + h)] = z
                        done += [z[16:], z[:16]]
                where = (_window(n * SEG_OUT + r // 8, ROWS // 8, SEG), _block(c, 256))
                pltpu.make_async_copy(out_v.at[where], out_hbm.at[where], sem_out).start()
        return carry

    lax.fori_loop(0, NSEG // SEG_OUT, finish, 0)
    pltpu.make_async_copy(out_v, out_hbm, sem_out).wait()


def _by_head_group(w):
    return w.reshape(DM, NGROUP, 8, HD).transpose(0, 2, 1, 3).reshape(DM * 8, NGROUP * HD)


@functools.partial(jax.jit, static_argnames=("A_seg_len",))
def pallas_gated_mix__memory_aug_recurrent_mem_tr__moe_arch_mod__prompt_kernel(
    A_x: jax.Array,
    A_mem0: jax.Array,
    A_Wq: jax.Array,
    A_Wk: jax.Array,
    A_Wv: jax.Array,
    A_Wo: jax.Array,
    A_seg_len: int,
    B_x: jax.Array,
    B_w_r: jax.Array,
    B_w_gate: jax.Array,
    B_w_up: jax.Array,
    B_w_down: jax.Array,
    gate_w: jax.Array,
):
    del B_x
    assert A_seg_len == SEG and A_x.shape == (1, SEQ, DM) and A_mem0.shape == (1, MEM, DM)
    assert A_Wq.shape == (DM, HEADS, HD) and B_w_gate.shape == (DM, FF)

    hbm = pl.BlockSpec(memory_space=pl.ANY)
    out = pl.pallas_call(
        _kernel,
        out_shape=jax.ShapeDtypeStruct((SEQ, DM), BF16),
        in_specs=[hbm] * 11,
        out_specs=hbm,
        scratch_shapes=[
            pltpu.VMEM((48, 128), BF16),
            pltpu.VMEM((NSEG, SEG, DM), BF16),
            pltpu.VMEM((MEM, DM), BF16),
            pltpu.VMEM((3, NGROUP, 2048 + 64, HD), BF16),
            pltpu.VMEM((HEADS * HD, DM), BF16),
            pltpu.VMEM((NC, SROWS // 2, 3 * 128), U32),
            pltpu.VMEM((3 * NPAIR, NC * 64, 4 * 128), U32),
            pltpu.VMEM((NC, NPAIR * 64, 4 * 128), U32),
            pltpu.VMEM((NC, NPAIR * 64, 3 * 128), U32),
            pltpu.VMEM((3 * NPAIR, SROWS, 2 * 128), F32),
            pltpu.VMEM((4, 16, NC * 128), U32),
            pltpu.VMEM((4, 16, NPAIR * HD), U32),
            pltpu.VMEM((3, SROWS // 2, NPAIR * HD), U32),
            pltpu.VMEM((SEQ, DM), F32),
            pltpu.VMEM((SEQ // 2, 128), F32),
            pltpu.VMEM((2, 6 * DM, 128), BF16),
            pltpu.VMEM((SEQ, DM), BF16),
            pltpu.SMEM((TOPK,), I32),
            pltpu.SemaphoreType.DMA((3,)),
            pltpu.SemaphoreType.DMA((NGROUP,)),
            pltpu.SemaphoreType.DMA((5,)),
            pltpu.SemaphoreType.DMA((6,)),
            pltpu.SemaphoreType.DMA((3,)),
            pltpu.SemaphoreType.DMA((2,)),
            pltpu.SemaphoreType.DMA,
        ],
        compiler_params=pltpu.CompilerParams(
            vmem_limit_bytes=112 * 1024 * 1024, disable_bounds_checks=True),
    )(
        A_x.reshape(NSEG, SEG, DM),
        A_mem0.reshape(MEM, DM),
        _by_head_group(A_Wq),
        _by_head_group(A_Wk),
        _by_head_group(A_Wv),
        A_Wo.reshape(HEADS * HD, DM),
        B_w_r.reshape(8, 128),
        B_w_gate,
        B_w_up,
        B_w_down,
        gate_w.reshape(8, 128),
    )
    return out.reshape(1, SEQ, DM)
```
